```python
import os as _os
_os.environ.setdefault("JAX_PLATFORMS", "cpu")
import jax
import jax.numpy as jnp

def _softmax(x, axis=-1):
    return jax.nn.softmax(x, axis=axis)
def _gelu(x):
    return jax.nn.gelu(x, approximate=True)
def _silu(x):
    return jax.nn.silu(x)
def _sigmoid(x):
    return jax.nn.sigmoid(x)
def _layernorm(x, axis=-1, eps=1e-5):
    m = jnp.mean(x, axis=axis, keepdims=True)
    v = jnp.var(x, axis=axis, keepdims=True)
    return (x - m) / jnp.sqrt(v + eps)
def _scatter_add(tgt, idx, src, axis=0):
    return tgt.at[idx].add(src)
def _segment_sum(src, seg, n):
    return jax.ops.segment_sum(src, seg, n)
class _Rng:
    def __init__(self, key):
        self._k = key
    def _next(self):
        self._k, sub = jax.random.split(self._k)
        return sub
    def normal(self, shape):
        return jax.random.normal(self._next(), shape, dtype=jnp.bfloat16)
    def randint(self, lo, hi, shape):
        return jax.random.randint(self._next(), shape, lo, hi, dtype=jnp.int32)
    def uniform(self, shape, lo=0.0, hi=1.0):
        return jax.random.uniform(self._next(), shape, jnp.bfloat16, lo, hi)
    def permutation(self, n):
        return jax.random.permutation(self._next(), n)


kernel_name = 'gated_mix__sliding_block__sliding_local_dilated__prompt'

def setup_inputs():
    _rng = _Rng(jax.random.key(int.from_bytes(__import__("os").urandom(4), "little")))
    _w = (lambda a: (lambda t: t.astype(jnp.bfloat16) if jnp.issubdtype(t.dtype, jnp.floating) else t)(jnp.asarray(a)))
    def _A_setup():
        B, S, D = 1, 2048, 640
        return {
            "x": _w((lambda *s: _rng.normal(s) * 0.05)(B, S, D)),
            "wqkv": _w((lambda *s: _rng.normal(s) * 0.8)(D, 3 * D)),
            "wo": _w((lambda *s: _rng.normal(s) * 0.05)(D, D)),
        }
    _A_in = _A_setup()

    def _B_setup():
        B, S, D = 1, 2048, 640
        return {
            "x": _w((lambda *s: _rng.normal(s) * 0.05)(B, S, D)),
            "wqkv": _w((lambda *s: _rng.normal(s) * 0.8)(D, 3 * D)),
            "wo": _w((lambda *s: _rng.normal(s) * 0.05)(D, D)),
        }
    _B_in = _B_setup()

    return {
        "A_x": _A_in["x"],
        "A_wqkv": _A_in["wqkv"],
        "A_wo": _A_in["wo"],
        "B_x": _B_in["x"],
        "B_wqkv": _B_in["wqkv"],
        "B_wo": _B_in["wo"],
        "gate_w": _w((lambda *s: _rng.normal(s) * 0.05)(640) * 16.0),
    }

def reference(A_x, A_wqkv, A_wo, B_x, B_wqkv, B_wo, gate_w):
    def _A_ref(x, wqkv, wo):
        B, S, D = x.shape
        H = 32; Dh = D // H; W = 256
        qkv = (lambda x, *d: x.transpose(*d))((x @ wqkv).reshape(B, S, 3, H, Dh), 2, 0, 3, 1, 4)
        q, k, v = qkv[0], qkv[1], qkv[2]
        scores = jnp.einsum("bhqd,bhkd->bhqk", q, k) * (Dh ** -0.5)
        idx = jnp.arange(S)
        mask = (idx[:, None] - idx[None, :] >= 0) & (idx[:, None] - idx[None, :] < W)
        scores = jnp.where(mask[None, None], scores, -1e9)
        p = _softmax(scores, axis=-1)
        o = jnp.einsum("bhqk,bhkd->bhqd", p, v)
        return (lambda x, *d: x.transpose(*d))(o, 0, 2, 1, 3).reshape(B, S, D) @ wo

    def _B_ref(x, wqkv, wo):
        B, S, D = x.shape
        H = 32; Dh = D // H
        W, dil = 8, 2
        qkv = (lambda x, *d: x.transpose(*d))((x @ wqkv).reshape(B, S, 3, H, Dh), 2, 0, 3, 1, 4)
        q, k, v = qkv[0], qkv[1], qkv[2]
        scale = Dh ** -0.5
        pos = jnp.arange(S)
        off = jnp.arange(W) * dil
        idx = pos[:, None] - off[None, :]
        mask = idx >= 0
        idx_c = jnp.where(mask, idx, 0).reshape(-1)
        kg = k[:, :, idx_c, :].reshape(B, H, S, W, Dh)
        vg = v[:, :, idx_c, :].reshape(B, H, S, W, Dh)
        logits = jnp.einsum("bhsd,bhswd->bhsw", q, kg) * scale
        logits = jnp.where(mask[None, None, :, :], logits, -1e9)
        attn = _softmax(logits, axis=-1)
        o = jnp.einsum("bhsw,bhswd->bhsd", attn, vg)
        return (lambda x, *d: x.transpose(*d))(o, 0, 2, 1, 3).reshape(B, S, D) @ wo

    x = A_x
    g = _sigmoid((x * gate_w).sum(-1, keepdims=True))
    a = _A_ref(x, A_wqkv, A_wo)
    b = _B_ref(x, B_wqkv, B_wo)
    return g * a + (1 - g) * b
```

```python
import functools
import math

import jax
import jax.numpy as jnp
from jax import lax
import jax.experimental.pallas as pl
import jax.experimental.pallas.tpu as pltpu

S = 2048
D = 640
H = 32
DH = 20
WIN = 256
NG = 8
LT = D // 128
BW = 8
HALO = 16

QSCALE = (DH ** -0.5) * math.log2(math.e)
NEG_BITS = 0xCE80CE80
ONE_BITS = 0x3F803F80

_NT = (((1,), (1,)), ((), ()))


def _u32(x):
    return pltpu.bitcast(x, jnp.uint32)


def _bf16(x):
    return pltpu.bitcast(x, jnp.bfloat16)


def _pack_shuffled(p):
    R, C = p.shape
    p3 = p.reshape(R // 16, 16, C)
    w = pltpu.pack_elementwise([p3[:, :8, :], p3[:, 8:, :]], packed_dtype=jnp.bfloat16)
    return w.reshape(R // 2, C).astype(jnp.uint32)


def _lane_range_mask(shape, lo, n):
    lane = lax.broadcasted_iota(jnp.int32, shape, 1)
    lo = lo % 128
    if lo + n <= 128:
        return (lane >= lo) & (lane < lo + n)
    return (lane >= lo) | (lane < lo + n - 128)


def make_kernel(TB):
    NQB = TB // 128

    def kernel(x_ref, wa_ref, woa_ref, wb_ref, wob_ref, gw_ref, o_ref,
               wvt_ref, wbt_ref, wobp_ref, kg_ref, vtp_ref, qg_ref, qkvb_ref,
               ot_ref, oa_ref, ob_ref, tmp_ref, bacc_ref):
        step = pl.program_id(0)

        @pl.when(step == 0)
        def _prep():
            for kt in range(LT):
                blk = wa_ref[kt * 128:(kt + 1) * 128, 2 * D:3 * D].astype(jnp.float32)
                wvt_ref[:, kt * 128:(kt + 1) * 128] = blk.T.astype(jnp.bfloat16)
            for kt in range(LT):
                for p in range(3):
                    blk = wb_ref[kt * 128:(kt + 1) * 128, p * D:(p + 1) * D].astype(jnp.float32)
                    tmp_ref[...] = blk.T
                    for d in range(DH):
                        rows = tmp_ref[pl.ds(d, H, stride=DH), :]
                        wbt_ref[p * D + d * H:p * D + (d + 1) * H, kt * 128:(kt + 1) * 128] = rows.astype(jnp.bfloat16)
            for lt in range(LT):
                tmp_ref[...] = wob_ref[:, lt * 128:(lt + 1) * 128].astype(jnp.float32)
                for d in range(DH):
                    rows = tmp_ref[pl.ds(d, H, stride=DH), :]
                    wobp_ref[d * H:(d + 1) * H, lt * 128:(lt + 1) * 128] = rows.astype(jnp.bfloat16)
            for g in range(NG):
                xl = (80 * g + 100) % 128
                lane = lax.broadcasted_iota(jnp.int32, (WIN // 2, 128), 1)
                kg_ref[g, 0:WIN // 2, :] = jnp.where(lane == xl, jnp.uint32(ONE_BITS), jnp.uint32(0))
            vtp_ref[0:2] = jnp.zeros((2, H * 16, 128), jnp.uint32)
            qkvb_ref[:, 0:HALO, :] = jnp.zeros((3 * LT, HALO, 128), jnp.float32)

        xb = x_ref[...]
        xf = xb.astype(jnp.float32)
        row0 = pl.multiple_of(step * TB, TB)
        row0h = pl.multiple_of(step * (TB // 2), TB // 2)

        qkvb = lax.dot_general(xb, wbt_ref[...], _NT, preferred_element_type=jnp.float32)
        for l in range(3 * LT):
            t = qkvb[:, l * 128:(l + 1) * 128]
            if l < LT:
                t = t * QSCALE
            qkvb_ref[l, HALO:HALO + TB, :] = t

        qk = jnp.dot(xb, wa_ref[:, 0:2 * D], preferred_element_type=jnp.float32)
        qt = [_u32((qk[:, l * 128:(l + 1) * 128] * QSCALE).astype(jnp.bfloat16)) for l in range(LT)]
        kt_ = [_u32(qk[:, D + l * 128:D + (l + 1) * 128].astype(jnp.bfloat16)) for l in range(LT)]
        shp = (TB // 2, 128)
        for g in range(NG):
            lo, hi = 80 * g, 80 * g + 80
            t0, t1 = lo // 128, (hi - 1) // 128
            if t0 == t1:
                m = _lane_range_mask(shp, lo, 80)
                kgv = jnp.where(m, kt_[t0], jnp.uint32(0))
                qgv = qt[t0]
            else:
                n0 = 128 * t1 - lo
                m0 = _lane_range_mask(shp, lo, n0)
                m1 = _lane_range_mask(shp, 0, 80 - n0)
                kgv = jnp.where(m0, kt_[t0], jnp.where(m1, kt_[t1], jnp.uint32(0)))
                qgv = jnp.where(m0, qt[t0], qt[t1])
            kg_ref[g, pl.ds(WIN // 2 + row0h, TB // 2), :] = kgv
            qg_ref[g] = qgv

        xs = _bf16(_pack_shuffled(xf))
        vt = lax.dot_general(wvt_ref[...], xs, _NT, preferred_element_type=jnp.float32)
        vtu = _u32(vt.astype(jnp.bfloat16))
        for qb in range(NQB):
            tile = 2 + step * NQB + qb
            for h in range(H):
                o = (4 * h) % 16
                ws = (20 * h - o) // 2
                win = vtu[ws:ws + 16, qb * 128:(qb + 1) * 128]
                r = lax.broadcasted_iota(jnp.int32, (16, 128), 0)
                keep = (r >= o // 2) & (r < o // 2 + 10)
                vtp_ref[tile, 16 * h:16 * h + 16, :] = jnp.where(keep, win, jnp.uint32(ONE_BITS))

        RB = 16
        for rb in range(TB // RB):
            r0 = HALO + rb * RB
            q = [qkvb_ref[l, r0:r0 + RB, :] for l in range(LT)]
            logits = []
            for w in range(BW):
                t = None
                for l in range(LT):
                    pr = q[l] * qkvb_ref[LT + l, r0 - 2 * w:r0 - 2 * w + RB, :]
                    t = pr if t is None else t + pr
                t = t + pltpu.roll(t, 64, 1)
                t = t + pltpu.roll(t, 32, 1)
                if rb == 0 and w > 0:
                    pos = row0 + lax.broadcasted_iota(jnp.int32, (RB, 128), 0)
                    t = jnp.where(pos >= 2 * w, t, -1e9)
                logits.append(t)
            m = functools.reduce(jnp.maximum, logits)
            e = [jnp.exp2(t - m) for t in logits]
            den = functools.reduce(jnp.add, e)
            rinv = 1.0 / den
            for l in range(LT):
                acc = None
                for w in range(BW):
                    pr = e[w] * qkvb_ref[2 * LT + l, r0 - 2 * w:r0 - 2 * w + RB, :]
                    acc = pr if acc is None else acc + pr
                ob_ref[rb * RB:(rb + 1) * RB, l * 128:(l + 1) * 128] = (acc * rinv).astype(jnp.bfloat16)
        qkvb_ref[LT:, 0:HALO, :] = qkvb_ref[LT:, TB:TB + HALO, :]

        z = jnp.sum(xf * gw_ref[...].astype(jnp.float32), axis=-1, keepdims=True)
        gate = 1.0 / (1.0 + jnp.exp(-z))

        def bproj():
            b = jnp.dot(ob_ref[...], wobp_ref[...], preferred_element_type=jnp.float32)
            bacc_ref[...] = (1.0 - gate) * b

        rr = lax.broadcasted_iota(jnp.int32, (32, 128), 0)
        ll = lax.broadcasted_iota(jnp.int32, (32, 128), 1)
        tri = rr > (ll & 31)
        l16 = lax.broadcasted_iota(jnp.int32, (16, 128), 1)
        b0 = (l16 & 32) == 0
        b1 = (l16 & 64) == 0
        zero16 = jnp.zeros((16, 128), jnp.uint32)

        def qk_stage(qb, g):
            xl = (80 * g + 100) % 128
            cst = jnp.where(l16 == xl, jnp.uint32(NEG_BITS), jnp.uint32(0))
            hm = [_lane_range_mask((16, 128), 80 * g + 20 * hh, 20) for hh in range(4)]
            out = []
            for j in range(4):
                qj = qg_ref[g, qb * 64 + j * 16:qb * 64 + (j + 1) * 16, :]
                wt = jnp.concatenate([jnp.where(hm[c ^ j], qj, cst) for c in range(4)], axis=0)
                kwin = kg_ref[g, pl.ds(pl.multiple_of(row0h + qb * 64 + 16 * j, 16), 144), :]
                s = lax.dot_general(_bf16(kwin), _bf16(wt), _NT, preferred_element_type=jnp.float32)
                dg = jnp.where(tri, s[0:32], s[256:288])
                sm = s[32:256]
                m = jnp.maximum(jnp.max(dg, axis=0, keepdims=True), jnp.max(sm, axis=0, keepdims=True))
                out.append((dg, sm, m))
            return out

        def pv_stage(qb, g, sc):
            P = []
            for j in range(4):
                dg, sm, m = sc[j]
                pd = jnp.exp2(dg - m)
                pm = jnp.exp2(sm - m)
                pa = jnp.where(tri, pd, 0.0)
                pc = jnp.where(tri, 0.0, pd)
                P.append(jnp.concatenate([_pack_shuffled(pa), _pack_shuffled(pm), _pack_shuffled(pc)], axis=0))
            Wh = [[], [], [], []]
            for kb in range(12):
                src = []
                for j in range(4):
                    if j <= kb <= j + 8:
                        src.append(P[j][(kb - j) * 16:(kb - j + 1) * 16])
                    else:
                        src.append(None)

                def sel(m, a, b):
                    if a is None and b is None:
                        return None
                    return jnp.where(m, zero16 if a is None else a, zero16 if b is None else b)
                t0 = sel(b0, src[0], src[1])
                t1 = sel(b0, src[1], src[0])
                t2 = sel(b0, src[2], src[3])
                t3 = sel(b0, src[3], src[2])
                Wh[0].append(sel(b1, t0, t2))
                Wh[2].append(sel(b1, t2, t0))
                Wh[1].append(sel(b1, t1, t3))
                Wh[3].append(sel(b1, t3, t1))
            res = []
            for hh in range(4):
                h = 4 * g + hh
                w = _bf16(jnp.concatenate(Wh[hh], axis=0))
                acc = None
                for a in range(3):
                    v = _bf16(vtp_ref[step * NQB + qb + a, 16 * h:16 * h + 16, :])
                    d = jnp.dot(v, w[a * 128:(a + 1) * 128], preferred_element_type=jnp.float32)
                    acc = d if acc is None else acc + d
                den = acc[24:32] if hh < 2 else acc[0:8]
                rinv = 1.0 / den
                res.append((acc, rinv))
            r8 = lax.broadcasted_iota(jnp.int32, (8, 128), 0) < 4

            def piece(hh, v):
                return res[hh][0][8 * v:8 * v + 8] * res[hh][1]
            blk = [piece(0, 0), piece(0, 1), jnp.where(r8, piece(0, 2), piece(1, 0)), piece(1, 1), piece(1, 2),
                   piece(2, 1), piece(2, 2), jnp.where(r8, piece(2, 3), piece(3, 1)), piece(3, 2), piece(3, 3)]
            ot_ref[qb, 80 * g:80 * g + 80, :] = jnp.concatenate(blk, axis=0)

        def finish(qb):
            for l in range(LT):
                z = ot_ref[qb, l * 128:(l + 1) * 128, :].T
                zu = _u32(z.astype(jnp.bfloat16))
                hd = (l * 128 + l16) // DH
                h0 = (hd & 1) == 0
                h1 = (hd & 2) == 0
                zc = [zu[16 * c:16 * c + 16] for c in range(4)]
                t0 = jnp.where(h0, zc[0], zc[1])
                t1 = jnp.where(h0, zc[1], zc[0])
                t2 = jnp.where(h0, zc[2], zc[3])
                t3 = jnp.where(h0, zc[3], zc[2])
                oj = [jnp.where(h1, t0, t2), jnp.where(h1, t1, t3), jnp.where(h1, t2, t0), jnp.where(h1, t3, t1)]
                oa_ref[qb * 64:(qb + 1) * 64, l * 128:(l + 1) * 128] = jnp.concatenate(oj, axis=0)

        def aproj(qb):
            rows = slice(qb * 128, (qb + 1) * 128)
            a = jnp.dot(_bf16(oa_ref[qb * 64:(qb + 1) * 64, :]), woa_ref[...], preferred_element_type=jnp.float32)
            o_ref[rows, :] = (gate[rows] * a + bacc_ref[rows, :]).astype(o_ref.dtype)

        chunks = [(qb, g) for qb in range(NQB) for g in range(NG)]
        sc = qk_stage(*chunks[0])
        for n, (qb, g) in enumerate(chunks):
            if n + 1 < len(chunks):
                nxt = qk_stage(*chunks[n + 1])
            else:
                bproj()
            pv_stage(qb, g, sc)
            sc = nxt
            if g == NG - 1:
                finish(qb)
        for qb in range(NQB):
            aproj(qb)

    return kernel


def build(TB=256):
    kernel = make_kernel(TB)
    full = lambda shape: pl.BlockSpec(shape, lambda i: (0,) * len(shape))

    @jax.jit
    def f(A_x, A_wqkv, A_wo, B_x, B_wqkv, B_wo, gate_w):
        x = A_x.reshape(S, D)
        gw = gate_w.reshape(1, D)
        out = pl.pallas_call(
            kernel,
            grid=(S // TB,),
            in_specs=[
                pl.BlockSpec((TB, D), lambda i: (i, 0)),
                full((D, 3 * D)), full((D, D)), full((D, 3 * D)), full((D, D)), full((1, D)),
            ],
            out_specs=pl.BlockSpec((TB, D), lambda i: (i, 0)),
            out_shape=jax.ShapeDtypeStruct((S, D), jnp.bfloat16),
            scratch_shapes=[
                pltpu.VMEM((D, D), jnp.bfloat16),
                pltpu.VMEM((3 * D, D), jnp.bfloat16),
                pltpu.VMEM((D, D), jnp.bfloat16),
                pltpu.VMEM((NG, (WIN + S) // 2, 128), jnp.uint32),
                pltpu.VMEM((2 + S // 128, H * 16, 128), jnp.uint32),
                pltpu.VMEM((NG, TB // 2, 128), jnp.uint32),
                pltpu.VMEM((3 * LT, HALO + TB, 128), jnp.float32),
                pltpu.VMEM((TB // 128, D, 128), jnp.float32),
                pltpu.VMEM((TB // 2, D), jnp.uint32),
                pltpu.VMEM((TB, D), jnp.bfloat16),
                pltpu.VMEM((D, 128), jnp.float32),
                pltpu.VMEM((TB, D), jnp.float32),
            ],
            compiler_params=pltpu.CompilerParams(
                dimension_semantics=("arbitrary",),
                vmem_limit_bytes=100 * 1024 * 1024,
            ),
        )(x, A_wqkv, A_wo, B_wqkv, B_wo, gw)
        return out.reshape(1, S, D)
    return f


_impl = build()


@jax.jit
def pallas_gated_mix__sliding_block__sliding_local_dilated__prompt_kernel(
    A_x: jax.Array,
    A_wqkv: jax.Array,
    A_wo: jax.Array,
    B_x: jax.Array,
    B_wqkv: jax.Array,
    B_wo: jax.Array,
    gate_w: jax.Array,
):
    return _impl(A_x, A_wqkv, A_wo, B_x, B_wqkv, B_wo, gate_w)
```

```python
import functools
import math

import jax
import jax.numpy as jnp
from jax import lax
import jax.experimental.pallas as pl
import jax.experimental.pallas.tpu as pltpu

S = 2048
D = 640
H = 32
DH = 20
WIN = 256
NG = 8
LT = D // 128
BW = 8
HALO = 16
TB = 256
NT = S // TB
NQB = TB // 128
RB = 16

QSCALE = (DH ** -0.5) * math.log2(math.e)
ONE_BITS = 0x3F803F80
NEG = -1e30

_NT = (((1,), (1,)), ((), ()))


def _u32(x):
    return pltpu.bitcast(x, jnp.uint32)


def _bf16(x):
    return pltpu.bitcast(x, jnp.bfloat16)


def _pack2(a, b):
    return pltpu.pack_elementwise([a, b], packed_dtype=jnp.bfloat16).astype(jnp.uint32)


def _pack_shuffled(p):
    R, C = p.shape
    p3 = p.reshape(R // 16, 16, C)
    w = pltpu.pack_elementwise([p3[:, :8, :], p3[:, 8:, :]], packed_dtype=jnp.bfloat16)
    return w.reshape(R // 2, C).astype(jnp.uint32)


def _fold(v):
    u = _u32(v)
    R, C = u.shape
    parts = [u[r:r + 16, c:c + 128] for r in range(0, R, 16) for c in range(0, C, 128)]
    while len(parts) > 1:
        parts = [parts[i] | parts[i + 1] if i + 1 < len(parts) else parts[i] for i in range(0, len(parts), 2)]
    return parts[0]


def _lane_range_mask(shape, lo, n):
    lane = lax.broadcasted_iota(jnp.int32, shape, 1)
    lo = lo % 128
    if lo + n <= 128:
        return (lane >= lo) & (lane < lo + n)
    return (lane >= lo) | (lane < lo + n - 128)


def make_kernel(order0, order1, nrun=NT, pace=None, bchain=0, bsync=0, bforce=None, joint=True, bchain0=0, pace0=None, pace1=None, rot0=1, poff0=1):

    def kernel(x_hbm, wa_hbm, woa_hbm, wb_hbm, wob_hbm, gw_hbm, o_hbm,
               x_ref, wa_ref, woa_ref, wb_ref, wob_ref, gw_ref, o_ref,
               wvt_ref, wqt_ref, wbt_ref, wobp_ref, kg_ref, vtp_ref, qr_ref, qkvb_ref,
               ot_ref, oa_ref, ob_ref, tmps_ref, tmpu_ref, bacc_ref, z_ref,
               wsem):

        sems = {}
        sts = {}

        cur = {"deps": ()}
        wanted = {d for it in order0 if len(it) > 3 for d in it[3]}

        def want(t, key):
            return isinstance(t, int) and (t, key) in wanted

        def sem_of(key):
            return wsem.at[sems.setdefault(key, len(sems))]

        def wcopy(key):
            i, kt = key if isinstance(key, tuple) else (key, None)
            r = slice(None) if kt is None else slice(kt * 128, (kt + 1) * 128)
            sem = sem_of(key)
            if i == 20:
                return pltpu.make_async_copy(z_ref.at[1], z_ref.at[0], sem)
            if i < 3:
                return pltpu.make_async_copy(wa_hbm.at[r, i * D:(i + 1) * D], wa_ref.at[r, i * D:(i + 1) * D], sem)
            if i < 6:
                p = i - 3
                return pltpu.make_async_copy(wb_hbm.at[r, p * D:(p + 1) * D], wb_ref.at[r, p * D:(p + 1) * D], sem)
            if i == 6:
                return pltpu.make_async_copy(wob_hbm, wob_ref, sem)
            if i == 7:
                return pltpu.make_async_copy(woa_hbm, woa_ref, sem)
            return pltpu.make_async_copy(gw_hbm, gw_ref, sem)

        def rows(t):
            if isinstance(t, int):
                return pl.ds(t * TB, TB)
            return pl.ds(pl.multiple_of(t * TB, TB), TB)

        def xcopy(t):
            sem = sem_of("x1") if (isinstance(t, int) and t == 1) else sem_of("x")
            return pltpu.make_async_copy(x_hbm.at[rows(t), :], x_ref.at[rows(t), :], sem)

        def ocopy(t):
            return pltpu.make_async_copy(o_ref.at[rows(t), :], o_hbm.at[rows(t), :], sem_of("o"))

        rr = lax.broadcasted_iota(jnp.int32, (32, 128), 0)
        ll = lax.broadcasted_iota(jnp.int32, (32, 128), 1)
        tri = rr > (ll & 31)
        l16 = lax.broadcasted_iota(jnp.int32, (16, 128), 1)
        b0 = (l16 & 32) == 0
        b1 = (l16 & 64) == 0
        zero16 = jnp.zeros((16, 128), jnp.uint32)
        chunks = [(qb, g) for qb in range(NQB) for g in range(NG)]
        hcls = ((lax.broadcasted_iota(jnp.int32, (40, 128), 1) >> 5)
                - lax.broadcasted_iota(jnp.int32, (40, 128), 0) // 10) & 3

        def tile_fns(t, slot=0):
            first = isinstance(t, int) and t == 0
            st = {}
            if isinstance(t, int):
                sts[t] = st
            q0 = HALO + slot * TB

            def opaque(rows=8):
                o = z_ref[0] != 0
                return o if rows == 8 else jnp.concatenate([o] * (rows // 8), axis=0)

            def dep_on(u, r0=0, c0=0):
                deps = cur["deps"]
                if not deps:
                    return u
                blk = u[r0:r0 + 16, c0:c0 + 128]
                for b, key in deps:
                    blk = jnp.where(opaque(16), _u32(sts[b][key]), blk)
                R, C = u.shape
                mid = [u[r0:r0 + 16, :c0]] * (c0 > 0) + [blk] + [u[r0:r0 + 16, c0 + 128:]] * (c0 + 128 < C)
                mid = jnp.concatenate(mid, axis=1) if len(mid) > 1 else blk
                full = [u[:r0]] * (r0 > 0) + [mid] + [u[r0 + 16:]] * (r0 + 16 < R)
                return jnp.concatenate(full, axis=0) if len(full) > 1 else mid

            def hoff(base, mult):
                if isinstance(t, int):
                    return t * (TB // 2) + base
                return pl.multiple_of(t * (TB // 2) + base, mult)

            def PREP(key):
                i, kt = key if isinstance(key, tuple) else (key, None)
                kts = range(LT) if kt is None else [kt]
                outs = []
                if i in (0, 2):
                    dst = wvt_ref if i == 2 else wqt_ref
                    tmp_ref = tmps_ref.at[i // 2]
                    for kt in kts:
                        blk = wa_ref[kt * 128:(kt + 1) * 128, i * D:(i + 1) * D].astype(jnp.float32)
                        tmp_ref[kt] = blk.T
                        for par in range(2):
                            a = tmp_ref[kt, pl.ds(par, D // 4, stride=4), :]
                            b = tmp_ref[kt, pl.ds(par + 2, D // 4, stride=4), :]
                            outs.append(_pack2(a, b))
                            dst[par * (D // 4):(par + 1) * (D // 4), kt * 128:(kt + 1) * 128] = outs[-1]
                elif i < 6:
                    p = i - 3
                    tmp_ref = tmps_ref.at[2 + p]
                    for kt in kts:
                        blk = wb_ref[kt * 128:(kt + 1) * 128, p * D:(p + 1) * D].astype(jnp.float32)
                        tmp_ref[kt] = blk.T
                        for d in range(DH):
                            ev = tmp_ref[kt, pl.ds(d, H // 2, stride=2 * DH), :]
                            od = tmp_ref[kt, pl.ds(d + DH, H // 2, stride=2 * DH), :]
                            outs.append(_pack2(ev, od))
                            r0 = (p * D + d * H) // 2
                            wbt_ref[r0:r0 + H // 2, kt * 128:(kt + 1) * 128] = outs[-1]
                else:
                    for lt in range(LT):
                        tmpu_ref[lt] = _u32(wob_ref[:, lt * 128:(lt + 1) * 128])
                        for d2 in range(DH // 2):
                            ev = tmpu_ref[lt, pl.ds(d2, H // 2, stride=DH), :]
                            od = tmpu_ref[lt, pl.ds(d2 + DH // 2, H // 2, stride=DH), :]
                            lo = (ev & jnp.uint32(0xFFFF)) | (od << 16)
                            hi = (ev >> 16) | (od & jnp.uint32(0xFFFF0000))
                            outs.append(jnp.concatenate([lo, hi], axis=0))
                            wobp_ref[d2 * H:(d2 + 1) * H, lt * 128:(lt + 1) * 128] = outs[-1]
                if want(t, ("PREP", key)):
                    st["PREP", key] = _fold(jnp.concatenate([_fold(o) for o in outs], axis=0))

            def WW(i):
                wcopy(i).wait()

            def WS(i):
                wcopy(i).start()

            def XW(_):
                xcopy(t).wait()

            def XS(k):
                if isinstance(t, int):
                    if t + k < nrun:
                        xcopy(t + k).start()
                else:
                    @pl.when(t + 1 < nrun)
                    def _():
                        xcopy(t + 1).start()

            def xdep():
                xb = x_ref[rows(t), :]
                return _bf16(dep_on(_u32(xb))) if cur["deps"] else xb

            def PB(ps):
                xb = x_ref[rows(t), :]
                lo, hi = ps[:2]
                w = wbt_ref[lo * D // 2:hi * D // 2, :]
                if cur["deps"]:
                    nt, kt = ps[2:] if len(ps) > 2 else (LT - 1, 0)
                    w = dep_on(w, 64 * nt, 128 * kt)
                qkvb = lax.dot_general(xb, _bf16(w), _NT, preferred_element_type=jnp.float32)
                for l in range((hi - lo) * LT):
                    v = qkvb[:, l * 128:(l + 1) * 128]
                    if lo * LT + l < LT:
                        v = v * QSCALE
                    qkvb_ref[lo * LT + l, q0:q0 + TB, :] = v

            def groups(tiles, zero):
                shp = (TB // 2, 128)
                out = []
                for g in range(NG):
                    lo, hi = 80 * g, 80 * g + 80
                    t0, t1 = lo // 128, (hi - 1) // 128
                    if t0 == t1:
                        v = tiles[t0]
                        if zero:
                            v = jnp.where(_lane_range_mask(shp, lo, 80), v, jnp.uint32(0))
                    else:
                        n0 = 128 * t1 - lo
                        m0 = _lane_range_mask(shp, lo, n0)
                        v = tiles[t1]
                        if zero:
                            v = jnp.where(_lane_range_mask(shp, 0, 80 - n0), v, jnp.uint32(0))
                        v = jnp.where(m0, tiles[t0], v)
                    out.append(v)
                return out

            def PK(_):
                xb = xdep()
                k = jnp.dot(xb, wa_ref[:, D:2 * D], preferred_element_type=jnp.float32)
                kt_ = [_u32(k[:, l * 128:(l + 1) * 128].astype(jnp.bfloat16)) for l in range(LT)]
                for g, v in enumerate(groups(kt_, False)):
                    kg_ref[g, pl.ds(hoff(0, TB // 2), TB // 2), :] = v

            def QT(_):
                xb = x_ref[rows(t), :]
                qt = lax.dot_general(_bf16(dep_on(wqt_ref[...])), xb, _NT, preferred_element_type=jnp.float32) * QSCALE
                qtu = _pack2(qt[:D // 2], qt[D // 2:])
                s8 = lax.broadcasted_iota(jnp.int32, (8, 128), 0)
                for qb in range(NQB):
                    for g in range(NG):
                        blk = []
                        for v in range(5):
                            u = qtu[40 * g + 8 * v:40 * g + 8 * v + 8, qb * 128:(qb + 1) * 128]
                            lo, hi = (16 * v) // DH, (16 * v + 15) // DH
                            rl = lambda r: pltpu.roll(u, 32 * r, 1) if r else u
                            if lo == hi:
                                blk.append(rl(lo))
                            else:
                                blk.append(jnp.where(s8 < (DH * hi - 16 * v) // 2, rl(lo), rl(hi)))
                        qr_ref[slot * NQB + qb, 40 * g:40 * g + 40, :] = jnp.concatenate(blk, axis=0)

            def VT(_):
                xf = x_ref[rows(t), :].astype(jnp.float32)
                xs = _bf16(_pack_shuffled(xf))
                vt = lax.dot_general(_bf16(dep_on(wvt_ref[...])), xs, _NT, preferred_element_type=jnp.float32)
                vtu = _pack2(vt[:D // 2], vt[D // 2:])
                r = lax.broadcasted_iota(jnp.int32, (16, 128), 0)
                for qb in range(NQB):
                    tile = t * NQB + qb
                    for h in range(H):
                        o = (4 * h) % 16
                        ws = (20 * h - o) // 2
                        win = vtu[ws:ws + 16, qb * 128:(qb + 1) * 128]
                        keep = (r >= o // 2) & (r < o // 2 + 10)
                        vtp_ref[tile, 16 * h:16 * h + 16, :] = jnp.where(keep, win, jnp.uint32(ONE_BITS))

            def BV(rbs):
                if first and rbs[0] == 0:
                    qkvb_ref[LT:, 0:HALO, :] = jnp.zeros((2 * LT, HALO, 128), jnp.float32)
                for rb in range(*rbs):
                    r0 = q0 + rb * RB
                    q = [qkvb_ref[l, r0:r0 + RB, :] for l in range(LT)]
                    bc = bchain0 if first else bchain
                    if rb == rbs[0] and cur["deps"]:
                        q = [pltpu.bitcast(dep_on(_u32(v)), jnp.float32) for v in q]
                    if bc and rb >= bc:
                        dep = st["bv", rb - bc]
                        q = [jnp.where(opaque(RB), dep, v) for v in q]
                    logits = []
                    for w in range(BW):
                        s = None
                        for l in range(LT):
                            pr = q[l] * qkvb_ref[LT + l, r0 - 2 * w:r0 - 2 * w + RB, :]
                            s = pr if s is None else s + pr
                        s = s + pltpu.roll(s, 64, 1)
                        s = s + pltpu.roll(s, 32, 1)
                        if first and rb * RB < 2 * w:
                            pos = rb * RB + lax.broadcasted_iota(jnp.int32, (RB, 128), 0)
                            s = jnp.where(pos >= 2 * w, s, NEG)
                        logits.append(s)
                    m = functools.reduce(jnp.maximum, logits)
                    e = [jnp.exp2(s - m) for s in logits]
                    den = functools.reduce(jnp.add, e)
                    rinv = 1.0 / den
                    for l in range(LT):
                        acc = None
                        for w in range(BW):
                            pr = e[w] * qkvb_ref[2 * LT + l, r0 - 2 * w:r0 - 2 * w + RB, :]
                            acc = pr if acc is None else acc + pr
                        acc = acc * rinv
                        ob_ref[slot, rb * RB:(rb + 1) * RB, l * 128:(l + 1) * 128] = acc.astype(jnp.bfloat16)
                        st["bv", rb] = [rinv, acc, m, logits[0], logits[4]][bsync]
                        st["bvl"] = acc
                if rbs[1] == TB // RB and not (first and joint):
                    qkvb_ref[LT:, 0:HALO, :] = qkvb_ref[LT:, q0 + TB - HALO:q0 + TB, :]

            def GATE(_):
                xf = x_ref[rows(t), :].astype(jnp.float32)
                gw = gw_ref[...].astype(jnp.float32).reshape(1, D)
                z = jnp.sum(xf * gw, axis=-1, keepdims=True)
                st["gate"] = 1.0 / (1.0 + jnp.exp(-z))
                if want(t, "GATE"):
                    st["GATE"] = _fold(jnp.broadcast_to(st["gate"], (TB, 128)))

            def BP(_):
                ob = ob_ref[slot]
                ob = _bf16(dep_on(_u32(ob))) if cur["deps"] else ob
                b = jnp.dot(ob, _bf16(wobp_ref[...]), preferred_element_type=jnp.float32)
                b = (1.0 - st["gate"]) * b
                if "a_done" in st:
                    b = (b + bacc_ref[slot]).astype(o_ref.dtype)
                    o_ref[rows(t), :] = b
                else:
                    st["b_done"] = True
                    bacc_ref[slot] = b
                if want(t, "BP"):
                    st["BP"] = _fold(b)

            def max4(b):
                return jnp.maximum(jnp.maximum(b[0:8], b[8:16]), jnp.maximum(b[16:24], b[24:32]))

            def QK(n):
                qb, g = chunks[n]
                qr = qr_ref[slot * NQB + qb, 40 * g:40 * g + 40, :]
                if isinstance(t, int):
                    qr = dep_on(qr)
                elif bforce is not None and n == bforce:
                    qr = jnp.concatenate([jnp.where(opaque(RB), _u32(st["bvl"]), qr[0:RB]), qr[RB:]], axis=0)
                zero24 = jnp.zeros((24, 128), jnp.uint32)
                out = [None] * 4
                for j in ([(jj + rot0 * n) % 4 for jj in range(4)] if first else range(4)):
                    J = 4 * qb + j
                    wq = jnp.concatenate([jnp.where(hcls == j, qr, jnp.uint32(0)), zero24], axis=0)
                    sh = (40 * g) % 64
                    wt = jnp.concatenate([wq[64 - sh:], wq[:64 - sh]], axis=0) if sh else wq
                    blocks = [None] * 8
                    if first:
                        kwin = kg_ref[g, 0:16 * (J + 1), :]
                        s = jnp.dot(_bf16(kwin), _bf16(wt), preferred_element_type=jnp.float32)
                        blocks[0] = jnp.where(tri, NEG, s[32 * J:32 * J + 32])
                        for i in range(J):
                            blocks[8 - J + i] = s[32 * i:32 * i + 32]
                    else:
                        base = hoff(16 * J - WIN // 2, 16)
                        kwin = jnp.concatenate([kg_ref[g, pl.ds(base, 16), :],
                                                kg_ref[g, pl.ds(base + 128, 16), :],
                                                kg_ref[g, pl.ds(base + 16, 112), :]], axis=0)
                        s = jnp.dot(_bf16(kwin), _bf16(wt), preferred_element_type=jnp.float32)
                        blocks[0] = jnp.where(tri, s[0:32], s[32:64])
                        for i in range(1, 8):
                            blocks[i] = s[32 * i + 32:32 * i + 64]
                    run = []
                    for b in blocks:
                        if b is not None:
                            run.append(max4(b) if not run else jnp.maximum(run[-1], max4(b)))
                    m = jnp.broadcast_to(jnp.max(run[-1], axis=0, keepdims=True), (8, 128))
                    out[j] = (blocks, run, m)
                st["s", n] = out

            def PV(n):
                qb, g = chunks[n]
                sc = st.pop(("s", n))
                pc = pace0 if first else (pace1 if isinstance(t, int) and pace1 is not None else pace)
                off = poff0 if first else 1
                nxt = st.get(("s", n + off)) if pc is not None else None
                if first and nxt is not None:
                    nxt = [nxt[(j + rot0 * off) % 4] for j in range(4)]
                a0 = (2 - qb) if first else 0
                pcs = [None] * 4
                Wh = [[], [], [], []]

                def prob(j, kk):
                    blocks, _, m = sc[j]
                    if first:
                        i = (kk + j - 4 * a0 + 1 if kk else 0) - pc if nxt is not None else -1
                    else:
                        i = kk + j - pc if nxt is not None else -1
                    if i >= 0:
                        m = jnp.where(opaque(), nxt[j][1][min(i, len(nxt[j][1]) - 1)], m)
                    return jnp.exp2(blocks[kk] - jnp.concatenate([m] * 4, axis=0))

                def sel(m, a, b):
                    if a is None and b is None:
                        return None
                    return jnp.where(m, zero16 if a is None else a, zero16 if b is None else b)

                if first:
                    for j in range(4):
                        pcs[j] = _pack_shuffled(jnp.where(tri, 0.0, prob(j, 0)))
                for kb in range(4 * a0, 12):
                    src = []
                    for j in range(4):
                        kk = kb - j
                        if kk == 0:
                            pd = prob(j, 0)
                            src.append(_pack_shuffled(jnp.where(tri, pd, 0.0)))
                            pcs[j] = _pack_shuffled(jnp.where(tri, 0.0, pd))
                        elif 0 < kk < 8:
                            src.append(_pack_shuffled(prob(j, kk)))
                        elif kk == 8:
                            src.append(pcs[j])
                        else:
                            src.append(None)
                    inn = [src[(-i) % 4] for i in range(4)]
                    tt = [sel(b0, inn[r], inn[(r - 1) % 4]) for r in range(4)]
                    for r in range(4):
                        Wh[r].append(sel(b1, tt[r], tt[(r - 2) % 4]))
                accs = [None] * 4
                for a in range(a0, 3):
                    for hh in range(4):
                        h = 4 * g + hh
                        w = _bf16(jnp.concatenate(Wh[hh][4 * (a - a0):4 * (a - a0) + 4], axis=0))
                        v = _bf16(vtp_ref[t * NQB + qb + a - 2, 16 * h:16 * h + 16, :])
                        d = jnp.dot(v, w, preferred_element_type=jnp.float32)
                        accs[hh] = d if accs[hh] is None else accs[hh] + d
                res = [(accs[hh], 1.0 / (accs[hh][24:32] if hh < 2 else accs[hh][0:8])) for hh in range(4)]
                r8 = lax.broadcasted_iota(jnp.int32, (8, 128), 0) < 4

                def piece(hh, v):
                    return res[hh][0][8 * v:8 * v + 8] * res[hh][1]
                blk = [piece(0, 0), piece(0, 1), jnp.where(r8, piece(0, 2), piece(1, 0)), piece(1, 1), piece(1, 2),
                       piece(2, 1), piece(2, 2), jnp.where(r8, piece(2, 3), piece(3, 1)), piece(3, 2), piece(3, 3)]
                ot_ref[slot * NQB + qb, 80 * g:80 * g + 80, :] = jnp.concatenate(blk, axis=0)
                st["PV", n] = jnp.concatenate(blk[8:10], axis=0)

            def FIN(qb):
                for l in range(LT):
                    z = ot_ref[slot * NQB + qb, l * 128:(l + 1) * 128, :].T
                    zu = _u32(z.astype(jnp.bfloat16))
                    hd = (l * 128 + l16) // DH
                    h0 = (hd & 1) == 0
                    h1 = (hd & 2) == 0
                    zc = [zu[16 * c:16 * c + 16] for c in range(4)]
                    tt = [jnp.where(h0, zc[j], zc[(j + 1) % 4]) for j in range(4)]
                    oj = [jnp.where(h1, tt[j], tt[(j + 2) % 4]) for j in range(4)]
                    oa_ref[slot, qb * 64:(qb + 1) * 64, l * 128:(l + 1) * 128] = jnp.concatenate(oj, axis=0)

            def AP(qb):
                r = slice(qb * 128, (qb + 1) * 128)
                a = jnp.dot(_bf16(dep_on(oa_ref[slot, qb * 64:(qb + 1) * 64, :])), woa_ref[...], preferred_element_type=jnp.float32)
                if isinstance(t, int):
                    dst = pl.ds(t * TB + qb * 128, 128)
                else:
                    dst = pl.ds(pl.multiple_of(t * TB + qb * 128, 128), 128)
                if "b_done" in st:
                    a = (st["gate"][r] * a + bacc_ref[slot, r, :]).astype(o_ref.dtype)
                    o_ref[dst, :] = a
                else:
                    st["a_done"] = True
                    a = st["gate"][r] * a
                    bacc_ref[slot, r, :] = a
                if want(t, "AP%d" % qb):
                    st["AP%d" % qb] = _fold(a)

            def OS(_):
                ocopy(t).start()

            def SPIN(n):
                acc = lax.fori_loop(0, n, lambda i, a: a * 1.0001 + 1.0, jnp.zeros((8, 128), jnp.float32))
                bacc_ref[0, 0:8, 0:128] = acc

            fns = dict(PREP=PREP, WW=WW, WS=WS, XW=XW, XS=XS, PB=PB, PK=PK, QT=QT, VT=VT, BV=BV, GATE=GATE, BP=BP,
                       QK=QK, PV=PV, FIN=FIN, AP=AP, OS=OS, SPIN=SPIN)
            return fns

        z_ref[1] = jnp.zeros((8, 128), jnp.int32)
        fs = [tile_fns(0, 0), tile_fns(1, 1)]
        for it in order0:
            cur["deps"] = it[3] if len(it) > 3 else ()
            fs[it[2] if len(it) > 2 else 0][it[0]](it[1])
        cur["deps"] = ()

        def loop_body(t, c):
            fns = tile_fns(t)
            for name, arg in order1:
                fns[name](arg)
            return c
        t1 = 2 if joint else 1
        if nrun > t1:
            lax.fori_loop(t1, nrun, loop_body, 0)
        for t in range(nrun):
            ocopy(t).wait()

    return kernel


def attn_order(lo=0, hi=NQB * NG, extra=None, last=("BP", 0), first=True, depth=1):
    extra = extra or {}
    nch = NQB * NG
    order = [("QK", lo + i) for i in range(depth)] if first else []
    for n in range(lo, hi):
        if n + depth < nch:
            order.append(("QK", n + depth))
        elif last and n == nch - 1:
            order.append(last)
        order += extra.get(n, [])
        order.append(("PV", n))
        if n % NG == NG - 1:
            order.append(("FIN", n // NG))
    return order


def orders(v0=0, depth=1, v1=0, p=None):
    NRB = TB // RB
    order1 = [("XW", 0), ("XS", 1), ("PB", (0, 3)), ("PK", 0), ("QT", 0), ("VT", 0), ("BV", (0, NRB)), ("GATE", 0)]
    if v1 == 0:
        order1 += attn_order(depth=depth) + [("AP", 0), ("AP", 1), ("OS", 0)]
    elif v1 == 1:
        order1 += [("BP", 0)] + attn_order(depth=depth, last=("AP", 0)) + [("AP", 1), ("OS", 0)]
    elif v1 == 3:
        order1 += attn_order(depth=depth, last=None, extra={14: [("BP", 0)]}) + [("AP", 0), ("AP", 1), ("OS", 0)]
    elif v1 == 2:
        order1 += [("BP", 0)] + attn_order(depth=depth, last=None, extra={14: [("AP", 0)]}) + [("AP", 1), ("OS", 0)]
    def T(items, tile):
        return [(n, a, tile) for n, a in items]

    B = (0, NRB)
    att0 = attn_order(depth=2, last=None)
    if v0 == 0:
        order0 = [("WS", 20), ("XS", 0), ("WS", 1), ("XS", 1), ("WS", 8)] + [("WS", i) for i in (3, 4, 5, 2, 0, 6, 7)]
        order0 += [("XW", 0), ("WW", 1), ("XS", 2), ("PK", 0),
                   ("XW", 0, 1), ("WW", 8), ("WW", 20), ("WW", 3), ("PREP", 3), ("PK", 0, 1), ("GATE", 0), ("GATE", 0, 1),
                   ("WW", 4), ("PREP", 4), ("PB", (0, 1)), ("PB", (0, 1), 1),
                   ("WW", 5), ("WW", 2), ("PREP", 5), ("PREP", 2), ("PB", (1, 2)), ("PB", (1, 2), 1),
                   ("WW", 0), ("WW", 6), ("WW", 7),
                   ("PREP", 0), ("PREP", 6), ("PB", (2, 3)), ("PB", (2, 3), 1), ("VT", 0), ("QT", 0), ("VT", 0, 1), ("QT", 0, 1),
                   ("BV", B), ("BV", B, 1)]
        order0 += att0 + [("BP", 0)]
        order0 += T(attn_order(depth=depth, last=None, extra={14: [("BP", 0)]}), 1)
        i = order0.index(("PV", 1, 1))
        order0[i:i] = [("AP", 0), ("AP", 1), ("OS", 0)]
        order0 += T([("AP", 0), ("AP", 1), ("OS", 0)], 1)
    if v0 == 1:
        order0 = [("WS", 20), ("XS", 0), ("WS", 1), ("XS", 1), ("WS", 8)] + [("WS", i) for i in (3, 4, 5, 2, 0, 6, 7)]
        order0 += [("XW", 0), ("WW", 1), ("XS", 2), ("PK", 0),
                   ("XW", 0, 1), ("WW", 8), ("WW", 20), ("WW", 3), ("PREP", 3), ("PK", 0, 1), ("GATE", 0), ("GATE", 0, 1),
                   ("PB", (0, 1)),
                   ("WW", 4), ("PREP", 4), ("PB", (0, 1), 1), ("PB", (1, 2)),
                   ("WW", 5), ("WW", 2), ("WW", 0), ("PREP", 5), ("PB", (1, 2), 1), ("PB", (2, 3)), ("PREP", 2), ("PB", (2, 3), 1),
                   ("BV", B), ("BV", B, 1),
                   ("PREP", 0), ("VT", 0), ("QT", 0), ("VT", 0, 1), ("QT", 0, 1)]
        order0 += att0 + [("WW", 6), ("WW", 7), ("PREP", 6), ("AP", 0), ("AP", 1), ("BP", 0), ("OS", 0)]
        order0 += T(attn_order(depth=depth, last=None, extra={14: [("BP", 0)]}), 1)
        order0 += T([("AP", 0), ("AP", 1), ("OS", 0)], 1)
    if v0 in (2, 3):
        order0 = [("WS", 20), ("XS", 0), ("WS", 1), ("XS", 1), ("WS", 8)] + [("WS", i) for i in (3, 4, 5, 2, 0, 6, 7)]
        order0 += [("XW", 0), ("WW", 1), ("XS", 2), ("PK", 0),
                   ("XW", 0, 1), ("WW", 8), ("WW", 20), ("WW", 3), ("PREP", 3), ("PK", 0, 1),
                   ("PB", (0, 1)),
                   ("WW", 4), ("PREP", 4), ("PB", (0, 1), 1), ("PB", (1, 2)),
                   ("WW", 5), ("WW", 2), ("WW", 0), ("PREP", 5), ("PB", (1, 2), 1), ("PB", (2, 3)), ("PREP", 2), ("PB", (2, 3), 1),
                   ("BV", B),
                   ("PREP", 0), ("VT", 0), ("QT", 0)]
        if v0 == 2:
            order0 += att0
            order0 += [("WW", 6), ("WW", 7), ("PREP", 6), ("VT", 0, 1)]
        else:
            order0 += attn_order(depth=2, last=None, extra={14: [("VT", 0, 1)]})[:-1]
            order0 += [("WW", 6), ("WW", 7), ("PREP", 6), ("FIN", 1)]
        order0 += [("QT", 0, 1), ("BV", B, 1), ("GATE", 0), ("GATE", 0, 1),
                   ("AP", 0), ("AP", 1), ("BP", 0), ("OS", 0)]
        order0 += T(attn_order(depth=depth, last=None, extra={14: [("BP", 0)]}), 1)
        order0 += T([("AP", 0), ("AP", 1), ("OS", 0)], 1)
    def addep(order, item, deps):
        i = order.index(item)
        order[i] = (item[0], item[1], item[2] if len(item) > 2 else 0, deps)

    if v0 == 4:
        order0 = [("WS", 20), ("XS", 0), ("WS", 1), ("XS", 1), ("WS", 8)] + [("WS", i) for i in (3, 4, 5, 2, 0, 6, 7)]
        order0 += [("XW", 0), ("WW", 1), ("XS", 2), ("PK", 0),
                   ("XW", 0, 1), ("WW", 8), ("WW", 20), ("WW", 3), ("PREP", 3), ("PK", 0, 1),
                   ("PB", (0, 1)),
                   ("WW", 4), ("PREP", 4), ("PB", (0, 1), 1), ("PB", (1, 2)),
                   ("WW", 5), ("WW", 2), ("PREP", 5), ("PB", (1, 2), 1), ("GATE", 0), ("GATE", 0, 1), ("PREP", 2), ("PB", (2, 3)),
                   ("VT", 0, 0, [(0, "GATE"), (1, "GATE")]),
                   ("WW", 0), ("WW", 6), ("WW", 7),
                   ("PREP", 0), ("PREP", 6), ("BV", B), ("PB", (2, 3), 1), ("VT", 0, 1, [(0, ("PREP", 6))]), ("QT", 0)]
        order0 += attn_order(depth=2, last=None, extra={14: [("QT", 0, 1)]})
        addep(order0, ("QK", 2), [(0, "bvl")])
        order0 += [("BV", B, 1), ("BP", 0), ("AP", 0), ("AP", 1), ("OS", 0)]
        order0 += T(attn_order(depth=depth, last=None, extra={14: [("BP", 0)]}), 1)
        addep(order0, ("QK", 2, 1), [(1, "bvl")])
        addep(order0, ("QK", 3, 1), [(0, "AP0"), (0, "AP1")])
        order0 += T([("AP", 0), ("AP", 1), ("OS", 0)], 1)
    if v0 in (5, 6):
        order0 = [("WS", 20), ("XS", 0), ("WS", 1), ("XS", 1), ("WS", 8)] + [("WS", i) for i in (3, 4, 6, 5, 2, 0, 7)]
        order0 += [("XW", 0), ("WW", 1), ("XS", 2), ("PK", 0),
                   ("XW", 0, 1), ("WW", 8), ("WW", 20), ("WW", 3), ("PREP", 3), ("PK", 0, 1), ("GATE", 0), ("GATE", 0, 1),
                   ("PB", (0, 1), 0, [(0, "GATE"), (1, "GATE")]),
                   ("WW", 4), ("WW", 6), ("PREP", 4), ("PB", (0, 1), 1), ("PREP", 6), ("PB", (1, 2), 0, [(0, ("PREP", 6))]),
                   ("WW", 5), ("WW", 2), ("PREP", 5), ("PB", (1, 2), 1), ("PREP", 2), ("PB", (2, 3), 0, [(0, ("PREP", 2))]),
                   ("WW", 0), ("WW", 7),
                   ("PREP", 0), ("BV", B), ("PB", (2, 3), 1), ("VT", 0)]
        p = dict(dict(f0=2, s1=12, f1=2, fa=3, d0=2, x0=14), **(p or {}))
        if v0 == 5:
            order0 += [("QT", 0), ("VT", 0, 1)]
            order0 += attn_order(depth=p["d0"], last=None, extra={p["x0"]: [("QT", 0, 1)]})
        else:
            order0 += [("QT", 0)]
            order0 += attn_order(depth=2, last=None, extra={14: [("QT", 0, 1)]}) + [("VT", 0, 1)]
        p = dict(dict(f0=2, s1=12, f1=2, fa=3), **(p or {}))
        addep(order0, ("QK", p["f0"]), [(0, "bvl")])
        order0 += [("BV", B, 1, [(0, ("PV", p["s1"]))] if p["s1"] is not None else []), ("BP", 0), ("AP", 0), ("AP", 1), ("OS", 0)]
        order0 += T(attn_order(depth=depth, last=None, extra={14: [("BP", 0)]}), 1)
        if p["f1"] == p["fa"]:
            addep(order0, ("QK", p["f1"], 1), [(1, "bvl"), (0, "AP0"), (0, "AP1")])
        else:
            addep(order0, ("QK", p["f1"], 1), [(1, "bvl")])
            if p["fa"] is not None:
                addep(order0, ("QK", p["fa"], 1), [(0, "AP0"), (0, "AP1")])
        order0 += T([("AP", 0), ("AP", 1), ("OS", 0)], 1)
    return order0, order1


def build(v0=0, nrun=NT, cut=None, pace=None, depth=1, v1=0, p=None, **kw):
    o0, o1 = orders(v0, depth, v1, p)
    if cut is not None:
        print(o0[cut - 3:cut])
        o0 = o0[:cut] + [("SPIN", 3000)] + [o for o in o0[cut:] if o[0] in ("WW", "XW", "OS")]
    kernel = make_kernel(o0, o1, nrun=nrun, pace=pace, **kw)
    anyspec = pl.BlockSpec(memory_space=pl.ANY)

    @jax.jit
    def f(A_x, A_wqkv, A_wo, B_x, B_wqkv, B_wo, gate_w):
        x = A_x.reshape(S, D)
        out = pl.pallas_call(
            kernel,
            in_specs=[anyspec] * 6,
            out_specs=anyspec,
            out_shape=jax.ShapeDtypeStruct((S, D), jnp.bfloat16),
            scratch_shapes=[
                pltpu.VMEM((S, D), jnp.bfloat16),
                pltpu.VMEM((D, 3 * D), jnp.bfloat16),
                pltpu.VMEM((D, D), jnp.bfloat16),
                pltpu.VMEM((D, 3 * D), jnp.bfloat16),
                pltpu.VMEM((D, D), jnp.bfloat16),
                pltpu.VMEM((D,), jnp.bfloat16),
                pltpu.VMEM((S, D), jnp.bfloat16),
                pltpu.VMEM((D // 2, D), jnp.uint32),
                pltpu.VMEM((D // 2, D), jnp.uint32),
                pltpu.VMEM((3 * D // 2, D), jnp.uint32),
                pltpu.VMEM((D // 2, D), jnp.uint32),
                pltpu.VMEM((NG, S // 2, 128), jnp.uint32),
                pltpu.VMEM((S // 128, H * 16, 128), jnp.uint32),
                pltpu.VMEM((2 * NQB, D // 2, 128), jnp.uint32),
                pltpu.VMEM((3 * LT, HALO + 2 * TB, 128), jnp.float32),
                pltpu.VMEM((2 * NQB, D, 128), jnp.float32),
                pltpu.VMEM((2, TB // 2, D), jnp.uint32),
                pltpu.VMEM((2, TB, D), jnp.bfloat16),
                pltpu.VMEM((5, LT, D, 128), jnp.float32),
                pltpu.VMEM((LT, D // 2, 128), jnp.uint32),
                pltpu.VMEM((2, TB, D), jnp.float32),
                pltpu.VMEM((2, 8, 128), jnp.int32),
                pltpu.SemaphoreType.DMA((32,)),
            ],
            compiler_params=pltpu.CompilerParams(
                vmem_limit_bytes=100 * 1024 * 1024,
            ),
        )(x, A_wqkv, A_wo, B_wqkv, B_wo, gate_w)
        return out.reshape(1, S, D)
    return f


_impl = build(v0=5, pace=3, depth=2, v1=3, bchain=1, bforce=2, bchain0=1, pace1=1, p=dict(s1=11))


@jax.jit
def pallas_gated_mix__sliding_block__sliding_local_dilated__prompt_kernel(
    A_x: jax.Array,
    A_wqkv: jax.Array,
    A_wo: jax.Array,
    B_x: jax.Array,
    B_wqkv: jax.Array,
    B_wo: jax.Array,
    gate_w: jax.Array,
):
    return _impl(A_x, A_wqkv, A_wo, B_x, B_wqkv, B_wo, gate_w)
```

```python
import functools
import math

import jax
import jax.numpy as jnp
from jax import lax
import jax.experimental.pallas as pl
import jax.experimental.pallas.tpu as pltpu

S = 2048
D = 640
H = 32
DH = 20
WIN = 256
NG = 8
LT = D // 128
BW = 8
HALO = 16
TB = 256
NT = S // TB
NQB = TB // 128
RB = 16

QSCALE = (DH ** -0.5) * math.log2(math.e)
ONE_BITS = 0x3F803F80
NEG = -1e30

_NT = (((1,), (1,)), ((), ()))


def _u32(x):
    return pltpu.bitcast(x, jnp.uint32)


def _bf16(x):
    return pltpu.bitcast(x, jnp.bfloat16)


def _pack2(a, b):
    return pltpu.pack_elementwise([a, b], packed_dtype=jnp.bfloat16).astype(jnp.uint32)


def _pack_shuffled(p):
    R, C = p.shape
    p3 = p.reshape(R // 16, 16, C)
    w = pltpu.pack_elementwise([p3[:, :8, :], p3[:, 8:, :]], packed_dtype=jnp.bfloat16)
    return w.reshape(R // 2, C).astype(jnp.uint32)


def _fold(v):
    u = _u32(v)
    R, C = u.shape
    parts = [u[r:r + 16, c:c + 128] for r in range(0, R, 16) for c in range(0, C, 128)]
    while len(parts) > 1:
        parts = [parts[i] | parts[i + 1] if i + 1 < len(parts) else parts[i] for i in range(0, len(parts), 2)]
    return parts[0]


def _lane_range_mask(shape, lo, n):
    lane = lax.broadcasted_iota(jnp.int32, shape, 1)
    lo = lo % 128
    if lo + n <= 128:
        return (lane >= lo) & (lane < lo + n)
    return (lane >= lo) | (lane < lo + n - 128)


def make_kernel(order0, order1, nrun=NT, pace=None, bchain=0, bsync=0, bforce=None, joint=True, bchain0=0, pace0=None, pace1=None, rot0=1, poff0=1, pchain=(4, 5, 6), ech={}, ech0={}, semmap={}):

    def kernel(x_hbm, wa_hbm, woa_hbm, wb_hbm, wob_hbm, gw_hbm, o_hbm,
               x_ref, wa_ref, woa_ref, wb_ref, wob_ref, gw_ref, o_ref,
               wvt_ref, wqt_ref, wbt_ref, wobp_ref, kg_ref, vtp_ref, qr_ref, qkvb_ref,
               ot_ref, oa_ref, ob_ref, tmps_ref, tmpu_ref, bacc_ref, z_ref,
               wsem):

        sems = {}
        sts = {}

        cur = {"deps": ()}
        wanted = {d for it in order0 + order1 if len(it) > 3 for d in it[3]}

        def want(t, key):
            return (t if isinstance(t, int) else "L", key) in wanted

        def sem_of(key):
            key = semmap.get(key, key)
            return wsem.at[sems.setdefault(key, len(sems))]

        def wcopy(key):
            i, kt = key if isinstance(key, tuple) else (key, None)
            r = slice(None) if kt is None else slice(kt * 128, (kt + 1) * 128)
            sem = sem_of(key)
            if i == 20:
                return pltpu.make_async_copy(z_ref.at[1], z_ref.at[0], sem)
            if i == 32:
                return pltpu.make_async_copy(x_hbm.at[TB:2 * TB, :], x_ref.at[TB:2 * TB, :], sem)
            if i == 31:
                return pltpu.make_async_copy(x_hbm.at[2 * TB:, :], x_ref.at[2 * TB:, :], sem)
            if i == 30:
                return pltpu.make_async_copy(x_hbm.at[r, :], x_ref.at[r, :], sem)
            if i < 3:
                return pltpu.make_async_copy(wa_hbm.at[r, i * D:(i + 1) * D], wa_ref.at[r, i * D:(i + 1) * D], sem)
            if i < 6:
                p = i - 3
                return pltpu.make_async_copy(wb_hbm.at[r, p * D:(p + 1) * D], wb_ref.at[r, p * D:(p + 1) * D], sem)
            if i == 6:
                return pltpu.make_async_copy(wob_hbm, wob_ref, sem)
            if i == 7:
                return pltpu.make_async_copy(woa_hbm, woa_ref, sem)
            return pltpu.make_async_copy(gw_hbm, gw_ref, sem)

        def rows(t):
            if isinstance(t, int):
                return pl.ds(t * TB, TB)
            return pl.ds(pl.multiple_of(t * TB, TB), TB)

        def xcopy(t):
            sem = sem_of("x1") if (isinstance(t, int) and t == 1) else sem_of("x")
            return pltpu.make_async_copy(x_hbm.at[rows(t), :], x_ref.at[rows(t), :], sem)

        def ocopy(t, qb):
            r = t * TB + qb * 128
            r = pl.ds(r if isinstance(t, int) else pl.multiple_of(r, 128), 128)
            return pltpu.make_async_copy(o_ref.at[r, :], o_hbm.at[r, :], sem_of("o"))

        nlead = 0
        while order0[nlead][0] == "WS" and order0[nlead][1] != 20:
            wcopy(order0[nlead][1]).start()
            nlead += 1

        rr = lax.broadcasted_iota(jnp.int32, (32, 128), 0)
        ll = lax.broadcasted_iota(jnp.int32, (32, 128), 1)
        tri = rr > (ll & 31)
        l16 = lax.broadcasted_iota(jnp.int32, (16, 128), 1)
        b0 = (l16 & 32) == 0
        b1 = (l16 & 64) == 0
        zero16 = jnp.zeros((16, 128), jnp.uint32)
        chunks = [(qb, g) for qb in range(NQB) for g in range(NG)]
        hcls = ((lax.broadcasted_iota(jnp.int32, (40, 128), 1) >> 5)
                - lax.broadcasted_iota(jnp.int32, (40, 128), 0) // 10) & 3

        def tile_fns(t, slot=0):
            first = isinstance(t, int) and t == 0
            st = {}
            sts[t if isinstance(t, int) else "L"] = st
            q0 = HALO + slot * TB

            def opaque(rows=8):
                o = z_ref[0] != 0
                return o if rows == 8 else jnp.concatenate([o] * (rows // 8), axis=0)

            def dep_on(u, r0=0, c0=0):
                deps = cur["deps"]
                if not deps:
                    return u
                blk = u[r0:r0 + 16, c0:c0 + 128]
                for b, key in deps:
                    blk = jnp.where(opaque(16), _u32(sts[b][key]), blk)
                R, C = u.shape
                mid = [u[r0:r0 + 16, :c0]] * (c0 > 0) + [blk] + [u[r0:r0 + 16, c0 + 128:]] * (c0 + 128 < C)
                mid = jnp.concatenate(mid, axis=1) if len(mid) > 1 else blk
                full = [u[:r0]] * (r0 > 0) + [mid] + [u[r0 + 16:]] * (r0 + 16 < R)
                return jnp.concatenate(full, axis=0) if len(full) > 1 else mid

            def hoff(base, mult):
                if isinstance(t, int):
                    return t * (TB // 2) + base
                return pl.multiple_of(t * (TB // 2) + base, mult)

            def PREP(key):
                i, kt, ph = (key + ("AB",))[:3] if isinstance(key, tuple) else (key, None, "AB")
                kts = range(LT) if kt is None else [kt]
                outs = []
                chain = want(t, ("PREP", key))

                def link(o):
                    if chain and outs:
                        o = jnp.where(opaque(o.shape[0]), outs[-1], o)
                    outs.append(o)

                def xpose(blk):
                    if key in pchain and "T" in st:
                        top = jnp.where(jnp.concatenate([opaque()] * LT, axis=1),
                                        jnp.concatenate([st["T"]] * LT, axis=1), blk[0:8])
                        blk = jnp.concatenate([top, blk[8:]], axis=0)
                    bt = blk.T
                    st["T"] = bt[D - 8:]
                    return bt
                st.pop("T", None)
                if i in (0, 2):
                    dst = wvt_ref if i == 2 else wqt_ref
                    tmp_ref = tmps_ref.at[i // 2]
                    for kt in kts:
                        blk = wa_ref[kt * 128:(kt + 1) * 128, i * D:(i + 1) * D].astype(jnp.float32)
                        tmp_ref[kt] = xpose(blk)
                        for par in range(2):
                            a = tmp_ref[kt, pl.ds(par, D // 4, stride=4), :]
                            b = tmp_ref[kt, pl.ds(par + 2, D // 4, stride=4), :]
                            link(_pack2(a, b))
                            dst[par * (D // 4):(par + 1) * (D // 4), kt * 128:(kt + 1) * 128] = outs[-1]
                elif i < 6:
                    p = i - 3
                    tmp_ref = tmps_ref.at[2 + p]
                    for kt in kts:
                        if "A" in ph:
                            blk = wb_ref[kt * 128:(kt + 1) * 128, p * D:(p + 1) * D].astype(jnp.float32)
                            tmp_ref[kt] = xpose(blk)
                        for d in range(DH) if "B" in ph else ():
                            ev = tmp_ref[kt, pl.ds(d, H // 2, stride=2 * DH), :]
                            od = tmp_ref[kt, pl.ds(d + DH, H // 2, stride=2 * DH), :]
                            link(_pack2(ev, od))
                            r0 = (p * D + d * H) // 2
                            wbt_ref[r0:r0 + H // 2, kt * 128:(kt + 1) * 128] = outs[-1]
                else:
                    for lt in range(LT):
                        u = _u32(wob_ref[:, lt * 128:(lt + 1) * 128])
                        if key in pchain and outs:
                            u = jnp.where(opaque(D // 2), jnp.concatenate([outs[-1]] * (D // 64), axis=0), u)
                        tmpu_ref[lt] = u
                        for d2 in range(DH // 2):
                            ev = tmpu_ref[lt, pl.ds(d2, H // 2, stride=DH), :]
                            od = tmpu_ref[lt, pl.ds(d2 + DH // 2, H // 2, stride=DH), :]
                            lo = (ev & jnp.uint32(0xFFFF)) | (od << 16)
                            hi = (ev >> 16) | (od & jnp.uint32(0xFFFF0000))
                            link(jnp.concatenate([lo, hi], axis=0))
                            wobp_ref[d2 * H:(d2 + 1) * H, lt * 128:(lt + 1) * 128] = outs[-1]
                if want(t, ("PREP", key)):
                    st["PREP", key] = _fold(outs[-1])

            def WW(i):
                wcopy(i).wait()

            def WS(i):
                wcopy(i).start()

            def XW(_):
                xcopy(t).wait()

            def XS(k):
                if isinstance(t, int):
                    if t + k < nrun:
                        xcopy(t + k).start()
                else:
                    @pl.when(t + 1 < nrun)
                    def _():
                        xcopy(t + 1).start()

            def xdep():
                xb = x_ref[rows(t), :]
                return _bf16(dep_on(_u32(xb))) if cur["deps"] else xb

            def PB(ps):
                xb = x_ref[rows(t), :]
                lo, hi = ps[:2]
                w = wbt_ref[lo * D // 2:hi * D // 2, :]
                if cur["deps"]:
                    nt, kt = ps[2:] if len(ps) > 2 else (LT - 1, 0)
                    w = dep_on(w, 64 * nt, 128 * kt)
                qkvb = lax.dot_general(xb, _bf16(w), _NT, preferred_element_type=jnp.float32)
                for l in range((hi - lo) * LT):
                    v = qkvb[:, l * 128:(l + 1) * 128]
                    if lo * LT + l < LT:
                        v = v * QSCALE
                    qkvb_ref[lo * LT + l, q0:q0 + TB, :] = v

            def PBX(a):
                c0, c1, r0, r1 = a[:4]
                xb = x_ref[t * TB + r0:t * TB + r1, :]
                w = wbt_ref[64 * c0:64 * c1, :]
                if cur["deps"]:
                    nt, kt = a[4:] if len(a) > 4 else (c1 - c0 - 1, 0)
                    w = dep_on(w, 64 * nt, 128 * kt)
                qkvb = lax.dot_general(xb, _bf16(w), _NT, preferred_element_type=jnp.float32)
                for l in range(c0, c1):
                    v = qkvb[:, (l - c0) * 128:(l - c0 + 1) * 128]
                    if l < LT:
                        v = v * QSCALE
                    qkvb_ref[l, q0 + r0:q0 + r1, :] = v

            def groups(tiles, zero):
                shp = tiles[0].shape
                out = []
                for g in range(NG):
                    lo, hi = 80 * g, 80 * g + 80
                    t0, t1 = lo // 128, (hi - 1) // 128
                    if t0 == t1:
                        v = tiles[t0]
                        if zero:
                            v = jnp.where(_lane_range_mask(shp, lo, 80), v, jnp.uint32(0))
                    else:
                        n0 = 128 * t1 - lo
                        m0 = _lane_range_mask(shp, lo, n0)
                        v = tiles[t1]
                        if zero:
                            v = jnp.where(_lane_range_mask(shp, 0, 80 - n0), v, jnp.uint32(0))
                        v = jnp.where(m0, tiles[t0], v)
                    out.append(v)
                return out

            def PK(rr_):
                r0, r1 = rr_ or (0, TB)
                xb = x_ref[t * TB + r0:t * TB + r1, :] if rr_ else xdep()
                k = jnp.dot(xb, wa_ref[:, D:2 * D], preferred_element_type=jnp.float32)
                kt_ = [_u32(k[:, l * 128:(l + 1) * 128].astype(jnp.bfloat16)) for l in range(LT)]
                for g, v in enumerate(groups(kt_, False)):
                    kg_ref[g, pl.ds(hoff(r0 // 2, 64), (r1 - r0) // 2), :] = v

            def QT(_):
                xb = x_ref[rows(t), :]
                qt = lax.dot_general(_bf16(dep_on(wqt_ref[...])), xb, _NT, preferred_element_type=jnp.float32) * QSCALE
                qtu = _pack2(qt[:D // 2], qt[D // 2:])
                s8 = lax.broadcasted_iota(jnp.int32, (8, 128), 0)
                for qb in range(NQB):
                    for g in range(NG):
                        blk = []
                        for v in range(5):
                            u = qtu[40 * g + 8 * v:40 * g + 8 * v + 8, qb * 128:(qb + 1) * 128]
                            lo, hi = (16 * v) // DH, (16 * v + 15) // DH
                            rl = lambda r: pltpu.roll(u, 32 * r, 1) if r else u
                            if lo == hi:
                                blk.append(rl(lo))
                            else:
                                blk.append(jnp.where(s8 < (DH * hi - 16 * v) // 2, rl(lo), rl(hi)))
                        qr_ref[slot * NQB + qb, 40 * g:40 * g + 40, :] = jnp.concatenate(blk, axis=0)

            def VT(_):
                xf = x_ref[rows(t), :].astype(jnp.float32)
                xs = _bf16(_pack_shuffled(xf))
                vt = lax.dot_general(_bf16(dep_on(wvt_ref[...])), xs, _NT, preferred_element_type=jnp.float32)
                vtu = _pack2(vt[:D // 2], vt[D // 2:])
                r = lax.broadcasted_iota(jnp.int32, (16, 128), 0)
                for qb in range(NQB):
                    tile = t * NQB + qb
                    for h in range(H):
                        o = (4 * h) % 16
                        ws = (20 * h - o) // 2
                        win = vtu[ws:ws + 16, qb * 128:(qb + 1) * 128]
                        keep = (r >= o // 2) & (r < o // 2 + 10)
                        vtp_ref[tile, 16 * h:16 * h + 16, :] = jnp.where(keep, win, jnp.uint32(ONE_BITS))

            def BV(rbs):
                if first and rbs[0] == 0:
                    qkvb_ref[LT:, 0:HALO, :] = jnp.zeros((2 * LT, HALO, 128), jnp.float32)
                for rb in range(*rbs):
                    r0 = q0 + rb * RB
                    q = [qkvb_ref[l, r0:r0 + RB, :] for l in range(LT)]
                    bc = bchain0 if first else bchain
                    if rb == rbs[0] and cur["deps"]:
                        q = [pltpu.bitcast(dep_on(_u32(v)), jnp.float32) for v in q]
                    if bc and rb >= bc:
                        dep = st["bv", rb - bc]
                        q = [jnp.where(opaque(RB), dep, v) for v in q]
                    logits = []
                    for w in range(BW):
                        s = None
                        for l in range(LT):
                            pr = q[l] * qkvb_ref[LT + l, r0 - 2 * w:r0 - 2 * w + RB, :]
                            s = pr if s is None else s + pr
                        s = s + pltpu.roll(s, 64, 1)
                        s = s + pltpu.roll(s, 32, 1)
                        if first and rb * RB < 2 * w:
                            pos = rb * RB + lax.broadcasted_iota(jnp.int32, (RB, 128), 0)
                            s = jnp.where(pos >= 2 * w, s, NEG)
                        logits.append(s)
                    m = functools.reduce(jnp.maximum, logits)
                    e = [jnp.exp2(s - m) for s in logits]
                    den = functools.reduce(jnp.add, e)
                    rinv = 1.0 / den
                    for l in range(LT):
                        acc = None
                        for w in range(BW):
                            pr = e[w] * qkvb_ref[2 * LT + l, r0 - 2 * w:r0 - 2 * w + RB, :]
                            acc = pr if acc is None else acc + pr
                        acc = acc * rinv
                        ob_ref[slot, rb * RB:(rb + 1) * RB, l * 128:(l + 1) * 128] = acc.astype(jnp.bfloat16)
                        st["bv", rb] = [rinv, acc, m, logits[0], logits[4]][bsync]
                        st["bvl"] = acc
                if rbs[1] == TB // RB and not (first and joint):
                    qkvb_ref[LT:, 0:HALO, :] = qkvb_ref[LT:, q0 + TB - HALO:q0 + TB, :]

            def GATE(_):
                xf = x_ref[rows(t), :].astype(jnp.float32)
                gw = gw_ref[...].astype(jnp.float32).reshape(1, D)
                z = jnp.sum(xf * gw, axis=-1, keepdims=True)
                st["gate"] = 1.0 / (1.0 + jnp.exp(-z))
                if want(t, "GATE"):
                    st["GATE"] = _fold(jnp.broadcast_to(st["gate"], (TB, 128)))

            def BP(_):
                ob = ob_ref[slot]
                ob = _bf16(dep_on(_u32(ob))) if cur["deps"] else ob
                b = jnp.dot(ob, _bf16(wobp_ref[...]), preferred_element_type=jnp.float32)
                b = (1.0 - st["gate"]) * b
                if "a_done" in st:
                    b = (b + bacc_ref[slot]).astype(o_ref.dtype)
                    o_ref[rows(t), :] = b
                else:
                    st["b_done"] = True
                    bacc_ref[slot] = b
                if want(t, "BP"):
                    st["BP"] = _fold(b)

            def max4(b):
                return jnp.maximum(jnp.maximum(b[0:8], b[8:16]), jnp.maximum(b[16:24], b[24:32]))

            def QK(n):
                qb, g = chunks[n]
                qr = qr_ref[slot * NQB + qb, 40 * g:40 * g + 40, :]
                if isinstance(t, int):
                    qr = dep_on(qr)
                elif bforce is not None and n == bforce:
                    qr = jnp.concatenate([jnp.where(opaque(RB), _u32(st["bvl"]), qr[0:RB]), qr[RB:]], axis=0)
                zero24 = jnp.zeros((24, 128), jnp.uint32)
                out = [None] * 4
                for j in ([(jj + rot0 * n) % 4 for jj in range(4)] if first else range(4)):
                    J = 4 * qb + j
                    wq = jnp.concatenate([jnp.where(hcls == j, qr, jnp.uint32(0)), zero24], axis=0)
                    sh = (40 * g) % 64
                    wt = jnp.concatenate([wq[64 - sh:], wq[:64 - sh]], axis=0) if sh else wq
                    blocks = [None] * 8
                    if first:
                        kwin = kg_ref[g, 0:16 * (J + 1), :]
                        s = jnp.dot(_bf16(kwin), _bf16(wt), preferred_element_type=jnp.float32)
                        blocks[0] = jnp.where(tri, NEG, s[32 * J:32 * J + 32])
                        for i in range(J):
                            blocks[8 - J + i] = s[32 * i:32 * i + 32]
                    else:
                        base = hoff(16 * J - WIN // 2, 16)
                        kwin = jnp.concatenate([kg_ref[g, pl.ds(base, 16), :],
                                                kg_ref[g, pl.ds(base + 128, 16), :],
                                                kg_ref[g, pl.ds(base + 16, 112), :]], axis=0)
                        s = jnp.dot(_bf16(kwin), _bf16(wt), preferred_element_type=jnp.float32)
                        blocks[0] = jnp.where(tri, s[0:32], s[32:64])
                        for i in range(1, 8):
                            blocks[i] = s[32 * i + 32:32 * i + 64]
                    run = []
                    for b in blocks:
                        if b is not None:
                            run.append(max4(b) if not run else jnp.maximum(run[-1], max4(b)))
                    m = jnp.broadcast_to(jnp.max(run[-1], axis=0, keepdims=True), (8, 128))
                    out[j] = (blocks, run, m)
                st["s", n] = out

            def PV(n):
                qb, g = chunks[n]
                sc = st.pop(("s", n))
                pc = pace0 if first else (pace1 if isinstance(t, int) and pace1 is not None else pace)
                off = poff0 if first else 1
                nxt = st.get(("s", n + off)) if pc is not None else None
                if first and nxt is not None:
                    nxt = [nxt[(j + rot0 * off) % 4] for j in range(4)]
                a0 = (2 - qb) if first else 0
                pcs = [None] * 4
                Wh = [[], [], [], []]

                hist = []
                ec = (ech0 if first else ech).get(n, 0)

                def prob(j, kk):
                    blocks, _, m = sc[j]
                    if first:
                        i = (kk + j - 4 * a0 + 1 if kk else 0) - pc if nxt is not None else -1
                    else:
                        i = kk + j - pc if nxt is not None else -1
                    if i >= 0:
                        m = jnp.where(opaque(), nxt[j][1][min(i, len(nxt[j][1]) - 1)], m)
                    if ec and len(hist) >= ec:
                        m = jnp.where(opaque(), hist[-ec][24:32], m)
                    hist.append(jnp.exp2(blocks[kk] - jnp.concatenate([m] * 4, axis=0)))
                    return hist[-1]

                def sel(m, a, b):
                    if a is None and b is None:
                        return None
                    return jnp.where(m, zero16 if a is None else a, zero16 if b is None else b)

                if first:
                    for j in range(4):
                        pcs[j] = _pack_shuffled(jnp.where(tri, 0.0, prob(j, 0)))
                for kb in range(4 * a0, 12):
                    src = []
                    for j in range(4):
                        kk = kb - j
                        if kk == 0:
                            pd = prob(j, 0)
                            src.append(_pack_shuffled(jnp.where(tri, pd, 0.0)))
                            pcs[j] = _pack_shuffled(jnp.where(tri, 0.0, pd))
                        elif 0 < kk < 8:
                            src.append(_pack_shuffled(prob(j, kk)))
                        elif kk == 8:
                            src.append(pcs[j])
                        else:
                            src.append(None)
                    inn = [src[(-i) % 4] for i in range(4)]
                    tt = [sel(b0, inn[r], inn[(r - 1) % 4]) for r in range(4)]
                    for r in range(4):
                        Wh[r].append(sel(b1, tt[r], tt[(r - 2) % 4]))
                accs = [None] * 4
                for a in range(a0, 3):
                    for hh in range(4):
                        h = 4 * g + hh
                        w = _bf16(jnp.concatenate(Wh[hh][4 * (a - a0):4 * (a - a0) + 4], axis=0))
                        v = _bf16(vtp_ref[t * NQB + qb + a - 2, 16 * h:16 * h + 16, :])
                        d = jnp.dot(v, w, preferred_element_type=jnp.float32)
                        accs[hh] = d if accs[hh] is None else accs[hh] + d
                res = [(accs[hh], 1.0 / (accs[hh][24:32] if hh < 2 else accs[hh][0:8])) for hh in range(4)]
                r8 = lax.broadcasted_iota(jnp.int32, (8, 128), 0) < 4

                def piece(hh, v):
                    return res[hh][0][8 * v:8 * v + 8] * res[hh][1]
                blk = [piece(0, 0), piece(0, 1), jnp.where(r8, piece(0, 2), piece(1, 0)), piece(1, 1), piece(1, 2),
                       piece(2, 1), piece(2, 2), jnp.where(r8, piece(2, 3), piece(3, 1)), piece(3, 2), piece(3, 3)]
                ot_ref[slot * NQB + qb, 80 * g:80 * g + 80, :] = jnp.concatenate(blk, axis=0)
                st["PV", n] = jnp.concatenate(blk[8:10], axis=0)

            def FIN(qb):
                for l in range(LT):
                    z = ot_ref[slot * NQB + qb, l * 128:(l + 1) * 128, :].T
                    zu = _u32(z.astype(jnp.bfloat16))
                    hd = (l * 128 + l16) // DH
                    h0 = (hd & 1) == 0
                    h1 = (hd & 2) == 0
                    zc = [zu[16 * c:16 * c + 16] for c in range(4)]
                    tt = [jnp.where(h0, zc[j], zc[(j + 1) % 4]) for j in range(4)]
                    oj = [jnp.where(h1, tt[j], tt[(j + 2) % 4]) for j in range(4)]
                    oa_ref[slot, qb * 64:(qb + 1) * 64, l * 128:(l + 1) * 128] = jnp.concatenate(oj, axis=0)

            def AP(qb):
                r = slice(qb * 128, (qb + 1) * 128)
                a = jnp.dot(_bf16(dep_on(oa_ref[slot, qb * 64:(qb + 1) * 64, :])), woa_ref[...], preferred_element_type=jnp.float32)
                if isinstance(t, int):
                    dst = pl.ds(t * TB + qb * 128, 128)
                else:
                    dst = pl.ds(pl.multiple_of(t * TB + qb * 128, 128), 128)
                if "b_done" in st:
                    a = (st["gate"][r] * a + bacc_ref[slot, r, :]).astype(o_ref.dtype)
                    o_ref[dst, :] = a
                else:
                    st["a_done"] = True
                    a = st["gate"][r] * a
                    bacc_ref[slot, r, :] = a
                if want(t, "AP%d" % qb):
                    st["AP%d" % qb] = _fold(a)

            def OS(qbs):
                for qb in (qbs or (0, 1)):
                    ocopy(t, qb).start()

            def SPIN(n):
                acc = lax.fori_loop(0, n, lambda i, a: a * 1.0001 + 1.0, jnp.zeros((8, 128), jnp.float32))
                bacc_ref[0, 0:8, 0:128] = acc

            fns = dict(PBX=PBX, PREP=PREP, WW=WW, WS=WS, XW=XW, XS=XS, PB=PB, PK=PK, QT=QT, VT=VT, BV=BV, GATE=GATE, BP=BP,
                       QK=QK, PV=PV, FIN=FIN, AP=AP, OS=OS, SPIN=SPIN)
            return fns

        z_ref[1] = jnp.zeros((8, 128), jnp.int32)
        fs = [tile_fns(0, 0), tile_fns(1, 1)]
        for it in order0[nlead:]:
            cur["deps"] = it[3] if len(it) > 3 else ()
            fs[it[2] if len(it) > 2 else 0][it[0]](it[1])
        cur["deps"] = ()

        def loop_body(t, c):
            fns = tile_fns(t)
            for it in order1:
                cur["deps"] = it[3] if len(it) > 3 else ()
                fns[it[0]](it[1])
            cur["deps"] = ()
            return c
        t1 = 2 if joint else 1
        if nrun > t1:
            lax.fori_loop(t1, nrun, loop_body, 0)
        for t in range(nrun):
            for qb in range(NQB):
                ocopy(t, qb).wait()

    return kernel


def attn_order(lo=0, hi=NQB * NG, extra=None, last=("BP", 0), first=True, depth=1):
    extra = extra or {}
    nch = NQB * NG
    order = [("QK", lo + i) for i in range(depth)] if first else []
    for n in range(lo, hi):
        if n + depth < nch:
            order.append(("QK", n + depth))
        elif last and n == nch - 1:
            order.append(last)
        order += extra.get(n, [])
        order.append(("PV", n))
        if n % NG == NG - 1:
            order.append(("FIN", n // NG))
    return order


def orders(v0=0, depth=1, v1=0, p=None):
    NRB = TB // RB
    order1 = [("XW", 0), ("XS", 1), ("PB", (0, 3)), ("PK", 0), ("QT", 0), ("VT", 0), ("BV", (0, NRB)), ("GATE", 0)]
    if v1 == 0:
        order1 += attn_order(depth=depth) + [("AP", 0), ("AP", 1), ("OS", 0)]
    elif v1 == 1:
        order1 += [("BP", 0)] + attn_order(depth=depth, last=("AP", 0)) + [("AP", 1), ("OS", 0)]
    elif v1 == 3:
        order1 += attn_order(depth=depth, last=None, extra={14: [("BP", 0)]}) + [("AP", 0), ("AP", 1), ("OS", 0)]
    elif v1 == 4:
        order1 += attn_order(depth=depth, last=None, extra={14: [("BP", 0)]}) + [("AP", 0), ("OS", (0,)), ("AP", 1), ("OS", (1,))]
    elif v1 == 5:
        order1 = [("XW", 0), ("XS", 1), ("GATE", 0), ("PB", (0, 3, (p or {}).get("gn", 8), 0), 0, [("L", "GATE")]), ("PK", 0), ("QT", 0), ("VT", 0), ("BV", (0, NRB))]
        order1 += attn_order(depth=depth, last=None, extra={14: [("BP", 0)]}) + [("AP", 0), ("OS", (0,)), ("AP", 1), ("OS", (1,))]
    elif v1 == 2:
        order1 += [("BP", 0)] + attn_order(depth=depth, last=None, extra={14: [("AP", 0)]}) + [("AP", 1), ("OS", 0)]
    def T(items, tile):
        return [(n, a, tile) for n, a in items]

    B = (0, NRB)
    att0 = attn_order(depth=2, last=None)
    if v0 == 0:
        order0 = [("WS", 20), ("XS", 0), ("WS", 1), ("XS", 1), ("WS", 8)] + [("WS", i) for i in (3, 4, 5, 2, 0, 6, 7)]
        order0 += [("XW", 0), ("WW", 1), ("XS", 2), ("PK", 0),
                   ("XW", 0, 1), ("WW", 8), ("WW", 20), ("WW", 3), ("PREP", 3), ("PK", 0, 1), ("GATE", 0), ("GATE", 0, 1),
                   ("WW", 4), ("PREP", 4), ("PB", (0, 1)), ("PB", (0, 1), 1),
                   ("WW", 5), ("WW", 2), ("PREP", 5), ("PREP", 2), ("PB", (1, 2)), ("PB", (1, 2), 1),
                   ("WW", 0), ("WW", 6), ("WW", 7),
                   ("PREP", 0), ("PREP", 6), ("PB", (2, 3)), ("PB", (2, 3), 1), ("VT", 0), ("QT", 0), ("VT", 0, 1), ("QT", 0, 1),
                   ("BV", B), ("BV", B, 1)]
        order0 += att0 + [("BP", 0)]
        order0 += T(attn_order(depth=depth, last=None, extra={14: [("BP", 0)]}), 1)
        i = order0.index(("PV", 1, 1))
        order0[i:i] = [("AP", 0), ("AP", 1), ("OS", 0)]
        order0 += T([("AP", 0), ("AP", 1), ("OS", 0)], 1)
    if v0 == 1:
        order0 = [("WS", 20), ("XS", 0), ("WS", 1), ("XS", 1), ("WS", 8)] + [("WS", i) for i in (3, 4, 5, 2, 0, 6, 7)]
        order0 += [("XW", 0), ("WW", 1), ("XS", 2), ("PK", 0),
                   ("XW", 0, 1), ("WW", 8), ("WW", 20), ("WW", 3), ("PREP", 3), ("PK", 0, 1), ("GATE", 0), ("GATE", 0, 1),
                   ("PB", (0, 1)),
                   ("WW", 4), ("PREP", 4), ("PB", (0, 1), 1), ("PB", (1, 2)),
                   ("WW", 5), ("WW", 2), ("WW", 0), ("PREP", 5), ("PB", (1, 2), 1), ("PB", (2, 3)), ("PREP", 2), ("PB", (2, 3), 1),
                   ("BV", B), ("BV", B, 1),
                   ("PREP", 0), ("VT", 0), ("QT", 0), ("VT", 0, 1), ("QT", 0, 1)]
        order0 += att0 + [("WW", 6), ("WW", 7), ("PREP", 6), ("AP", 0), ("AP", 1), ("BP", 0), ("OS", 0)]
        order0 += T(attn_order(depth=depth, last=None, extra={14: [("BP", 0)]}), 1)
        order0 += T([("AP", 0), ("AP", 1), ("OS", 0)], 1)
    if v0 in (2, 3):
        order0 = [("WS", 20), ("XS", 0), ("WS", 1), ("XS", 1), ("WS", 8)] + [("WS", i) for i in (3, 4, 5, 2, 0, 6, 7)]
        order0 += [("XW", 0), ("WW", 1), ("XS", 2), ("PK", 0),
                   ("XW", 0, 1), ("WW", 8), ("WW", 20), ("WW", 3), ("PREP", 3), ("PK", 0, 1),
                   ("PB", (0, 1)),
                   ("WW", 4), ("PREP", 4), ("PB", (0, 1), 1), ("PB", (1, 2)),
                   ("WW", 5), ("WW", 2), ("WW", 0), ("PREP", 5), ("PB", (1, 2), 1), ("PB", (2, 3)), ("PREP", 2), ("PB", (2, 3), 1),
                   ("BV", B),
                   ("PREP", 0), ("VT", 0), ("QT", 0)]
        if v0 == 2:
            order0 += att0
            order0 += [("WW", 6), ("WW", 7), ("PREP", 6), ("VT", 0, 1)]
        else:
            order0 += attn_order(depth=2, last=None, extra={14: [("VT", 0, 1)]})[:-1]
            order0 += [("WW", 6), ("WW", 7), ("PREP", 6), ("FIN", 1)]
        order0 += [("QT", 0, 1), ("BV", B, 1), ("GATE", 0), ("GATE", 0, 1),
                   ("AP", 0), ("AP", 1), ("BP", 0), ("OS", 0)]
        order0 += T(attn_order(depth=depth, last=None, extra={14: [("BP", 0)]}), 1)
        order0 += T([("AP", 0), ("AP", 1), ("OS", 0)], 1)
    def addep(order, item, deps):
        i = order.index(item)
        order[i] = (item[0], item[1], item[2] if len(item) > 2 else 0, deps)

    if v0 == 4:
        order0 = [("WS", 20), ("XS", 0), ("WS", 1), ("XS", 1), ("WS", 8)] + [("WS", i) for i in (3, 4, 5, 2, 0, 6, 7)]
        order0 += [("XW", 0), ("WW", 1), ("XS", 2), ("PK", 0),
                   ("XW", 0, 1), ("WW", 8), ("WW", 20), ("WW", 3), ("PREP", 3), ("PK", 0, 1),
                   ("PB", (0, 1)),
                   ("WW", 4), ("PREP", 4), ("PB", (0, 1), 1), ("PB", (1, 2)),
                   ("WW", 5), ("WW", 2), ("PREP", 5), ("PB", (1, 2), 1), ("GATE", 0), ("GATE", 0, 1), ("PREP", 2), ("PB", (2, 3)),
                   ("VT", 0, 0, [(0, "GATE"), (1, "GATE")]),
                   ("WW", 0), ("WW", 6), ("WW", 7),
                   ("PREP", 0), ("PREP", 6), ("BV", B), ("PB", (2, 3), 1), ("VT", 0, 1, [(0, ("PREP", 6))]), ("QT", 0)]
        order0 += attn_order(depth=2, last=None, extra={14: [("QT", 0, 1)]})
        addep(order0, ("QK", 2), [(0, "bvl")])
        order0 += [("BV", B, 1), ("BP", 0), ("AP", 0), ("AP", 1), ("OS", 0)]
        order0 += T(attn_order(depth=depth, last=None, extra={14: [("BP", 0)]}), 1)
        addep(order0, ("QK", 2, 1), [(1, "bvl")])
        addep(order0, ("QK", 3, 1), [(0, "AP0"), (0, "AP1")])
        order0 += T([("AP", 0), ("AP", 1), ("OS", 0)], 1)
    if v0 in (5, 6, 7):
        order0 = [("WS", 20), ("XS", 0), ("WS", 1), ("XS", 1), ("WS", 8)] + [("WS", i) for i in (3, 4, 6, 5, 2, 0, 7)]
        order0 += [("XW", 0), ("WW", 1), ("XS", 2), ("PK", 0),
                   ("XW", 0, 1), ("WW", 8), ("WW", 20), ("WW", 3), ("PREP", 3), ("PK", 0, 1), ("GATE", 0), ("GATE", 0, 1),
                   ("PB", (0, 1), 0, [(0, "GATE"), (1, "GATE")]),
                   ("WW", 4), ("WW", 6), ("PREP", 4), ("PB", (0, 1), 1), ("PREP", 6), ("PB", (1, 2), 0, [(0, ("PREP", 6))]),
                   ("WW", 5), ("WW", 2), ("PREP", 5), ("PB", (1, 2), 1), ("PREP", 2), ("PB", (2, 3), 0, [(0, ("PREP", 2))]),
                   ("WW", 0), ("WW", 7),
                   ("PREP", 0), ("BV", B), ("PB", (2, 3), 1), ("VT", 0)]
        p = dict(dict(f0=2, s1=12, f1=2, fa=3, d0=2, x0=14), **(p or {}))
        if v0 == 7:
            H0, H1 = (0, 128), (128, 256)
            order0 = [("WS", (3, k)) for k in range(LT)] + [("WS", (30, 0)), ("WS", (30, 1)), ("WS", 32), ("WS", 8), ("WS", 1),
                                                            ("WS", 20)]
            late = [(4,), (5, 6), (2, 0, 7), (31,), ()]
            for k in range(LT):
                order0 += [("WW", (3, k))] + [("WS", i) for i in late[k]]
                order0 += [("PREP", (3, k, "A"))] + [("PREP", (3, k - 1, "B"))] * (k > 0)
            order0 += [("WW", (30, 0)), ("PREP", (3, LT - 1, "B")), ("PBX", (0, 4) + H0),
                       ("WW", (30, 1)), ("WW", 32), ("WW", 8), ("WW", 20), ("GATE", 0), ("GATE", 0, 1),
                       ("PBX", (4, 5) + H0), ("PBX", (0, 5) + H1), ("PBX", (0, 5) + H0 + (0, 0), 1, [(0, "GATE")]),
                       ("PBX", (0, 5) + H1 + (0, 0), 1, [(1, "GATE")]),
                       ("WW", 1), ("PK", H0), ("PK", H1),
                       ("WW", 4), ("PREP", 4), ("PK", 0, 1), ("PBX", (5, 8, 0, TB)),
                       ("WW", 5), ("WW", 6), ("PREP", 5), ("PBX", (8, 10, 0, TB)), ("PB", (1, 2), 1), ("PREP", 6),
                       ("PB", (2, 3), 0, [(0, ("PREP", 6))]),
                       ("WW", 2), ("WW", 0), ("WW", 7),
                       ("PREP", 2), ("BV", B), ("PB", (2, 3), 1), ("PREP", 0), ("VT", 0)]
            order0 += [("VT", 0, 1), ("QT", 0)] if p.get("vq") else [("QT", 0), ("VT", 0, 1)]
            order0 += attn_order(depth=p["d0"], last=None, extra={p["x0"]: [("QT", 0, 1)]})
        elif v0 == 5:
            order0 += [("QT", 0), ("VT", 0, 1)]
            order0 += attn_order(depth=p["d0"], last=None, extra={p["x0"]: [("QT", 0, 1)]})
        else:
            order0 += [("QT", 0)]
            order0 += attn_order(depth=2, last=None, extra={14: [("QT", 0, 1)]}) + [("VT", 0, 1)]
        p = dict(dict(f0=2, s1=12, f1=2, fa=3), **(p or {}))
        addep(order0, ("QK", p["f0"]), [(0, "bvl")])
        order0 += [("BV", B, 1, [(0, ("PV", p["s1"]))] if p["s1"] is not None else []), ("BP", 0), ("AP", 0), ("AP", 1), ("OS", 0)]
        order0 += T(attn_order(depth=depth, last=None, extra={14: [("BP", 0)]}), 1)
        if p["f1"] == p["fa"]:
            addep(order0, ("QK", p["f1"], 1), [(1, "bvl"), (0, "AP0"), (0, "AP1")])
        else:
            addep(order0, ("QK", p["f1"], 1), [(1, "bvl")])
            if p["fa"] is not None:
                addep(order0, ("QK", p["fa"], 1), [(0, "AP0"), (0, "AP1")])
        order0 += T([("AP", 0), ("AP", 1), ("OS", 0)], 1)
    return order0, order1


def build(v0=0, nrun=NT, cut=None, pace=None, depth=1, v1=0, p=None, xall=True, **kw):
    o0, o1 = orders(v0, depth, v1, p)
    if cut is not None:
        print(o0[cut - 3:cut])
        o0 = o0[:cut] + [("SPIN", 3000)] + [o for o in o0[cut:] if o[0] in ("WW", "XW", "OS")]
    if xall:
        o0 = [("WS", 31) if it == ("XS", 2) else it for it in o0] + [("WW", 31)]
        o1 = [it for it in o1 if it[0] not in ("XW", "XS")]
    kw["semmap"] = {32: (30, 1), 8: (30, 1), 20: (30, 1), 4: (3, 0), 5: (3, 1), 6: (3, 1), 2: (3, 2), 0: (3, 2), 7: (3, 2),
                    31: (3, 3), "o": (3, 4)}
    kernel = make_kernel(o0, o1, nrun=nrun, pace=pace, **kw)
    anyspec = pl.BlockSpec(memory_space=pl.ANY)

    @jax.jit
    def f(A_x, A_wqkv, A_wo, B_x, B_wqkv, B_wo, gate_w):
        x = A_x.reshape(S, D)
        out = pl.pallas_call(
            kernel,
            in_specs=[anyspec] * 6,
            out_specs=anyspec,
            out_shape=jax.ShapeDtypeStruct((S, D), jnp.bfloat16),
            scratch_shapes=[
                pltpu.VMEM((S, D), jnp.bfloat16),
                pltpu.VMEM((D, 3 * D), jnp.bfloat16),
                pltpu.VMEM((D, D), jnp.bfloat16),
                pltpu.VMEM((D, 3 * D), jnp.bfloat16),
                pltpu.VMEM((D, D), jnp.bfloat16),
                pltpu.VMEM((D,), jnp.bfloat16),
                pltpu.VMEM((S, D), jnp.bfloat16),
                pltpu.VMEM((D // 2, D), jnp.uint32),
                pltpu.VMEM((D // 2, D), jnp.uint32),
                pltpu.VMEM((3 * D // 2, D), jnp.uint32),
                pltpu.VMEM((D // 2, D), jnp.uint32),
                pltpu.VMEM((NG, S // 2, 128), jnp.uint32),
                pltpu.VMEM((S // 128, H * 16, 128), jnp.uint32),
                pltpu.VMEM((2 * NQB, D // 2, 128), jnp.uint32),
                pltpu.VMEM((3 * LT, HALO + 2 * TB, 128), jnp.float32),
                pltpu.VMEM((2 * NQB, D, 128), jnp.float32),
                pltpu.VMEM((2, TB // 2, D), jnp.uint32),
                pltpu.VMEM((2, TB, D), jnp.bfloat16),
                pltpu.VMEM((5, LT, D, 128), jnp.float32),
                pltpu.VMEM((LT, D // 2, 128), jnp.uint32),
                pltpu.VMEM((2, TB, D), jnp.float32),
                pltpu.VMEM((2, 8, 128), jnp.int32),
                pltpu.SemaphoreType.DMA((8,)),
            ],
            compiler_params=pltpu.CompilerParams(
                vmem_limit_bytes=100 * 1024 * 1024,
            ),
        )(x, A_wqkv, A_wo, B_wqkv, B_wo, gate_w)
        return out.reshape(1, S, D)
    return f


_impl = build(v0=7, pace=3, depth=2, v1=4, bchain=1, bforce=2, bchain0=1, pace1=1, p=dict(s1=11, d0=4, x0=12))


@jax.jit
def pallas_gated_mix__sliding_block__sliding_local_dilated__prompt_kernel(
    A_x: jax.Array,
    A_wqkv: jax.Array,
    A_wo: jax.Array,
    B_x: jax.Array,
    B_wqkv: jax.Array,
    B_wo: jax.Array,
    gate_w: jax.Array,
):
    return _impl(A_x, A_wqkv, A_wo, B_x, B_wqkv, B_wo, gate_w)
```

```python
import functools
import math

import jax
import jax.numpy as jnp
from jax import lax
import jax.experimental.pallas as pl
import jax.experimental.pallas.tpu as pltpu

S = 2048
D = 640
H = 32
DH = 20
WIN = 256
NG = 8
LT = D // 128
BW = 8
HALO = 16
TB = 256
NT = S // TB
NQB = TB // 128
RB = 16

QSCALE = (DH ** -0.5) * math.log2(math.e)
ONE_BITS = 0x3F803F80
NEG = -1e30

_NT = (((1,), (1,)), ((), ()))
_NN = (((1,), (0,)), ((), ()))


def _u32(x):
    return pltpu.bitcast(x, jnp.uint32)


def _bf16(x):
    return pltpu.bitcast(x, jnp.bfloat16)


def _pack2(a, b):
    return pltpu.pack_elementwise([a, b], packed_dtype=jnp.bfloat16).astype(jnp.uint32)


def _pack_shuffled(p):
    R, C = p.shape
    p3 = p.reshape(R // 16, 16, C)
    w = pltpu.pack_elementwise([p3[:, :8, :], p3[:, 8:, :]], packed_dtype=jnp.bfloat16)
    return w.reshape(R // 2, C).astype(jnp.uint32)


def _fold(v):
    u = _u32(v)
    R, C = u.shape
    parts = [u[r:r + 16, c:c + 128] for r in range(0, R, 16) for c in range(0, C, 128)]
    while len(parts) > 1:
        parts = [parts[i] | parts[i + 1] if i + 1 < len(parts) else parts[i] for i in range(0, len(parts), 2)]
    return parts[0]


def _lane_range_mask(shape, lo, n):
    lane = lax.broadcasted_iota(jnp.int32, shape, 1)
    lo = lo % 128
    if lo + n <= 128:
        return (lane >= lo) & (lane < lo + n)
    return (lane >= lo) | (lane < lo + n - 128)


def make_kernel(order0, order1, nrun=NT, pace=None, bchain=0, bsync=0, bforce=None, joint=True, bchain0=0, pace0=None, pace1=None, rot0=1, poff0=1, pchain=(4, 5, 6), ech={}, ech0={}, semmap={}, wvf=False, wqf=False, bpace={}, sx=0, wx=0, qchain=0, bpace0=0, pair=False, oshift=False):

    def kernel(x_hbm, wa_hbm, woa_hbm, wb_hbm, wob_hbm, gw_hbm, o_hbm,
               x_ref, wa_ref, woa_ref, wb_ref, wob_ref, gw_ref, o_ref,
               wvt_ref, wqt_ref, wbt_ref, wobp_ref, kg_ref, vtp_ref, qr_ref, qkvb_ref,
               ot_ref, oa_ref, ob_ref, tmps_ref, tmpu_ref, bacc_ref, z_ref, sc_ref, w_ref, pk_ref, obf_ref,
               wsem):

        sems = {}
        sts = {}

        cur = {"deps": ()}
        wanted = {d for it in order0 + order1 if len(it) > 3 for d in it[3]}

        def want(t, key):
            return (t if isinstance(t, int) else "L", key) in wanted

        def sem_of(key):
            key = semmap.get(key, key)
            return wsem.at[sems.setdefault(key, len(sems))]

        def wcopy(key):
            i, kt = key[:2] if isinstance(key, tuple) else (key, None)
            r = slice(None) if kt is None else slice(kt * 128, (key[2] if len(key) > 2 else kt + 1) * 128)
            sem = sem_of(key)
            if i == 20:
                return pltpu.make_async_copy(z_ref.at[1], z_ref.at[0], sem)
            if i == 32:
                return pltpu.make_async_copy(x_hbm.at[TB:2 * TB, :], x_ref.at[TB:2 * TB, :], sem)
            if i == 31:
                return pltpu.make_async_copy(x_hbm.at[2 * TB:, :], x_ref.at[2 * TB:, :], sem)
            if i == 30:
                return pltpu.make_async_copy(x_hbm.at[r, :], x_ref.at[r, :], sem)
            if i < 3:
                return pltpu.make_async_copy(wa_hbm.at[r, i * D:(i + 1) * D], wa_ref.at[r, i * D:(i + 1) * D], sem)
            if i < 6:
                p = i - 3
                return pltpu.make_async_copy(wb_hbm.at[r, p * D:(p + 1) * D], wb_ref.at[r, p * D:(p + 1) * D], sem)
            if i == 6:
                return pltpu.make_async_copy(wob_hbm, wob_ref, sem)
            if i == 7:
                return pltpu.make_async_copy(woa_hbm, woa_ref, sem)
            return pltpu.make_async_copy(gw_hbm, gw_ref, sem)

        def rows(t):
            if isinstance(t, int):
                return pl.ds(t * TB, TB)
            return pl.ds(pl.multiple_of(t * TB, TB), TB)

        def xcopy(t):
            sem = sem_of("x1") if (isinstance(t, int) and t == 1) else sem_of("x")
            return pltpu.make_async_copy(x_hbm.at[rows(t), :], x_ref.at[rows(t), :], sem)

        def ocopy(t, qb, n=1):
            r = t * TB + qb * 128
            r = pl.ds(r if isinstance(t, int) else pl.multiple_of(r, 128), 128 * n)
            return pltpu.make_async_copy(o_ref.at[r, :], o_hbm.at[r, :], sem_of("o"))
        pend = []

        nlead = 0
        while order0[nlead][0] == "WS" and order0[nlead][1] != 20:
            wcopy(order0[nlead][1]).start()
            nlead += 1

        rr = lax.broadcasted_iota(jnp.int32, (32, 128), 0)
        ll = lax.broadcasted_iota(jnp.int32, (32, 128), 1)
        tri = rr > (ll & 31)
        l16 = lax.broadcasted_iota(jnp.int32, (16, 128), 1)
        b0 = (l16 & 32) == 0
        b1 = (l16 & 64) == 0
        zero16 = jnp.zeros((16, 128), jnp.uint32)
        chunks = [(qb, g) for qb in range(NQB) for g in range(NG)]
        hcls = ((lax.broadcasted_iota(jnp.int32, (40, 128), 1) >> 5)
                - lax.broadcasted_iota(jnp.int32, (40, 128), 0) // 10) & 3

        def tile_fns(t, slot=0):
            first = isinstance(t, int) and t == 0
            st = {}
            sts[t if isinstance(t, int) else "L"] = st
            q0 = HALO + slot * TB

            def opaque(rows=8):
                o = z_ref[0] != 0
                return o if rows == 8 else jnp.concatenate([o] * (rows // 8), axis=0)

            def dep_on(u, r0=0, c0=0):
                deps = cur["deps"]
                if not deps:
                    return u
                blk = u[r0:r0 + 16, c0:c0 + 128]
                for b, key in deps:
                    blk = jnp.where(opaque(16), _u32(sts[b][key]), blk)
                R, C = u.shape
                mid = [u[r0:r0 + 16, :c0]] * (c0 > 0) + [blk] + [u[r0:r0 + 16, c0 + 128:]] * (c0 + 128 < C)
                mid = jnp.concatenate(mid, axis=1) if len(mid) > 1 else blk
                full = [u[:r0]] * (r0 > 0) + [mid] + [u[r0 + 16:]] * (r0 + 16 < R)
                return jnp.concatenate(full, axis=0) if len(full) > 1 else mid

            def hoff(base, mult):
                if isinstance(t, int):
                    return t * (TB // 2) + base
                return pl.multiple_of(t * (TB // 2) + base, mult)

            def PREP(key):
                i, kt, ph = (key + ("AB",))[:3] if isinstance(key, tuple) else (key, None, "AB")
                kts = range(LT) if kt is None else [kt]
                outs = []
                chain = want(t, ("PREP", key))

                def link(o):
                    if chain and outs:
                        o = jnp.where(opaque(o.shape[0]), outs[-1], o)
                    outs.append(o)

                def xpose(blk):
                    if key in pchain and "T" in st:
                        top = jnp.where(jnp.concatenate([opaque()] * LT, axis=1),
                                        jnp.concatenate([st["T"]] * LT, axis=1), blk[0:8])
                        blk = jnp.concatenate([top, blk[8:]], axis=0)
                    bt = blk.T
                    st["T"] = bt[D - 8:]
                    return bt
                st.pop("T", None)
                if i in (0, 2):
                    dst = wvt_ref if i == 2 else wqt_ref
                    tmp_ref = tmps_ref.at[i // 2]
                    for kt in kts:
                        blk = wa_ref[kt * 128:(kt + 1) * 128, i * D:(i + 1) * D].astype(jnp.float32)
                        tmp_ref[kt] = xpose(blk)
                        if (i == 2 and wvf) or (i == 0 and wqf):
                            continue
                        if i == 2:
                            a = tmp_ref[kt, pl.ds(0, D // 2, stride=2), :]
                            b = tmp_ref[kt, pl.ds(1, D // 2, stride=2), :]
                            link(_pack2(a, b))
                            dst[:, kt * 128:(kt + 1) * 128] = outs[-1]
                            continue
                        for par in range(2):
                            a = tmp_ref[kt, pl.ds(par, D // 4, stride=4), :]
                            b = tmp_ref[kt, pl.ds(par + 2, D // 4, stride=4), :]
                            link(_pack2(a, b))
                            dst[par * (D // 4):(par + 1) * (D // 4), kt * 128:(kt + 1) * 128] = outs[-1]
                elif i < 6:
                    p = i - 3
                    tmp_ref = tmps_ref.at[2 + p]
                    for kt in kts:
                        if "A" in ph:
                            blk = wb_ref[kt * 128:(kt + 1) * 128, p * D:(p + 1) * D].astype(jnp.float32)
                            tmp_ref[kt] = xpose(blk)
                        for d in range(DH) if "B" in ph else ():
                            ev = tmp_ref[kt, pl.ds(d, H // 2, stride=2 * DH), :]
                            od = tmp_ref[kt, pl.ds(d + DH, H // 2, stride=2 * DH), :]
                            link(_pack2(ev, od))
                            r0 = (p * D + d * H) // 2
                            wbt_ref[r0:r0 + H // 2, kt * 128:(kt + 1) * 128] = outs[-1]
                else:
                    for lt in range(LT):
                        u = _u32(wob_ref[:, lt * 128:(lt + 1) * 128])
                        if key in pchain and outs:
                            u = jnp.where(opaque(D // 2), jnp.concatenate([outs[-1]] * (D // 64), axis=0), u)
                        tmpu_ref[lt] = u
                        for d2 in range(DH // 2):
                            ev = tmpu_ref[lt, pl.ds(d2, H // 2, stride=DH), :]
                            od = tmpu_ref[lt, pl.ds(d2 + DH // 2, H // 2, stride=DH), :]
                            lo = (ev & jnp.uint32(0xFFFF)) | (od << 16)
                            hi = (ev >> 16) | (od & jnp.uint32(0xFFFF0000))
                            link(jnp.concatenate([lo, hi], axis=0))
                            wobp_ref[d2 * H:(d2 + 1) * H, lt * 128:(lt + 1) * 128] = outs[-1]
                if want(t, ("PREP", key)):
                    st["PREP", key] = _fold(outs[-1])

            def WW(i):
                wcopy(i).wait()

            def WS(i):
                wcopy(i).start()

            def XW(_):
                xcopy(t).wait()

            def XS(k):
                if isinstance(t, int):
                    if t + k < nrun:
                        xcopy(t + k).start()
                else:
                    @pl.when(t + 1 < nrun)
                    def _():
                        xcopy(t + 1).start()

            def xdep():
                xb = x_ref[rows(t), :]
                return _bf16(dep_on(_u32(xb))) if cur["deps"] else xb

            def PB(ps):
                xb = x_ref[rows(t), :]
                lo, hi = ps[:2]
                w = wbt_ref[lo * D // 2:hi * D // 2, :]
                if cur["deps"]:
                    nt, kt = ps[2:] if len(ps) > 2 else (LT - 1, 0)
                    w = dep_on(w, 64 * nt, 128 * kt)
                qkvb = lax.dot_general(xb, _bf16(w), _NT, preferred_element_type=jnp.float32)
                for l in range((hi - lo) * LT):
                    v = qkvb[:, l * 128:(l + 1) * 128]
                    if lo * LT + l < LT:
                        v = v * QSCALE
                    qkvb_ref[lo * LT + l, q0:q0 + TB, :] = v

            def PBX(a):
                c0, c1, r0, r1 = a[:4]
                xb = x_ref[pl.ds(t * TB + r0 if isinstance(t, int) else pl.multiple_of(t * TB + r0, 128), r1 - r0), :]
                w = wbt_ref[64 * c0:64 * c1, :]
                if cur["deps"]:
                    nt, kt = a[4:] if len(a) > 4 else (c1 - c0 - 1, 0)
                    w = dep_on(w, 64 * nt, 128 * kt)
                qkvb = lax.dot_general(xb, _bf16(w), _NT, preferred_element_type=jnp.float32)
                for l in range(c0, c1):
                    v = qkvb[:, (l - c0) * 128:(l - c0 + 1) * 128]
                    if l < LT:
                        v = v * QSCALE
                    qkvb_ref[l, q0 + r0:q0 + r1, :] = v

            def groups(tiles, zero):
                shp = tiles[0].shape
                out = []
                for g in range(NG):
                    lo, hi = 80 * g, 80 * g + 80
                    t0, t1 = lo // 128, (hi - 1) // 128
                    if t0 == t1:
                        v = tiles[t0]
                        if zero:
                            v = jnp.where(_lane_range_mask(shp, lo, 80), v, jnp.uint32(0))
                    else:
                        n0 = 128 * t1 - lo
                        m0 = _lane_range_mask(shp, lo, n0)
                        v = tiles[t1]
                        if zero:
                            v = jnp.where(_lane_range_mask(shp, 0, 80 - n0), v, jnp.uint32(0))
                        v = jnp.where(m0, tiles[t0], v)
                    out.append(v)
                return out

            def PK(rr_):
                r0, r1, k0, k1 = (tuple(rr_) + (0, LT))[:4] if rr_ else (0, TB, 0, LT)
                xb = x_ref[t * TB + r0:t * TB + r1, k0 * 128:k1 * 128] if rr_ else xdep()
                if rr_ and cur["deps"]:
                    xb = _bf16(dep_on(_u32(xb)))
                k = jnp.dot(xb, wa_ref[k0 * 128:k1 * 128, D:2 * D], preferred_element_type=jnp.float32)
                if k0 > 0:
                    k = k + pk_ref[t, r0:r1, :]
                if k1 < LT:
                    pk_ref[t, r0:r1, :] = k
                    return
                kt_ = [_u32(k[:, l * 128:(l + 1) * 128].astype(jnp.bfloat16)) for l in range(LT)]
                for g, v in enumerate(groups(kt_, False)):
                    kg_ref[g, pl.ds(hoff(r0 // 2, 32), (r1 - r0) // 2), :] = v

            def QT(_):
                xb = x_ref[rows(t), :]
                if wqf:
                    w = jnp.concatenate([jnp.concatenate([tmps_ref[0, kt, pl.ds(par, D // 2, stride=2), :] for par in range(2)], axis=0)
                                         for kt in range(LT)], axis=1)
                    w = pltpu.bitcast(dep_on(_u32(w)), jnp.float32) if cur["deps"] else w
                else:
                    w = _bf16(dep_on(wqt_ref[...]))
                qt = lax.dot_general(w, xb, _NT, preferred_element_type=jnp.float32) * QSCALE
                qtu = _pack2(qt[:D // 2], qt[D // 2:])
                s8 = lax.broadcasted_iota(jnp.int32, (8, 128), 0)
                for qb in range(NQB):
                    for g in range(NG):
                        blk = []
                        for v in range(5):
                            u = qtu[40 * g + 8 * v:40 * g + 8 * v + 8, qb * 128:(qb + 1) * 128]
                            if qchain and v == 4 and "qc" in st:
                                u = jnp.where(opaque(), st["qc"], u)
                            lo, hi = (16 * v) // DH, (16 * v + 15) // DH
                            rl = lambda r: pltpu.roll(u, 32 * r, 1) if r else u
                            if lo == hi:
                                blk.append(rl(lo))
                            else:
                                blk.append(jnp.where(s8 < (DH * hi - 16 * v) // 2, rl(lo), rl(hi)))
                        qr_ref[slot * NQB + qb, 40 * g:40 * g + 40, :] = jnp.concatenate(blk, axis=0)
                        st["qc"] = blk[4]
                        if want(t, "QT"):
                            fo = blk[0] | blk[1] | blk[2] | blk[3] | blk[4]
                            st["QTf"] = fo if "QTf" not in st else st["QTf"] | fo
                            st["QT"] = jnp.concatenate([st["QTf"]] * 2, axis=0)

            def VT(_):
                xf = x_ref[rows(t), :].astype(jnp.float32)
                xs = _bf16(_pack_shuffled(xf))
                if wvf:
                    w = jnp.concatenate([tmps_ref[1, kt] for kt in range(LT)], axis=1)
                    w = pltpu.bitcast(dep_on(_u32(w)), jnp.float32) if cur["deps"] else w
                else:
                    w = _bf16(dep_on(wvt_ref[...]))
                vt = lax.dot_general(w, xs, _NT, preferred_element_type=jnp.float32)
                r8 = lax.broadcasted_iota(jnp.int32, (8, 128), 0) < 4
                for qb in range(NQB):
                    tile = t * NQB + qb
                    for hp in range(H // 2):
                        win = vt[40 * hp:40 * hp + 40, qb * 128:(qb + 1) * 128]
                        mid = win[16:24]
                        vtp_ref[tile, 48 * hp:48 * hp + 48, :] = jnp.concatenate(
                            [win[0:16], jnp.where(r8, mid, 1.0), jnp.where(r8, 1.0, mid), win[24:40]], axis=0)

            def BV(rbs):
                if first and rbs[0] == 0:
                    qkvb_ref[LT:, 0:HALO, :] = jnp.zeros((2 * LT, HALO, 128), jnp.float32)
                for rb in range(*rbs):
                    r0 = q0 + rb * RB
                    q = [qkvb_ref[l, r0:r0 + RB, :] for l in range(LT)]
                    bc = bchain0 if first else bchain
                    if rb == rbs[0] and cur["deps"]:
                        q = [pltpu.bitcast(dep_on(_u32(jnp.concatenate([v] * (16 // min(RB, 16)), axis=0))), jnp.float32)[:RB] for v in q]
                    if bc and rb >= bc:
                        dep = st["bv", rb - bc]
                        q = [jnp.where(opaque(RB), dep, v) for v in q]
                    logits = []
                    for w in range(BW):
                        s = None
                        for l in range(LT):
                            pr = q[l] * qkvb_ref[LT + l, r0 - 2 * w:r0 - 2 * w + RB, :]
                            s = pr if s is None else s + pr
                        s = s + pltpu.roll(s, 64, 1)
                        s = s + pltpu.roll(s, 32, 1)
                        if first and rb * RB < 2 * w:
                            pos = rb * RB + lax.broadcasted_iota(jnp.int32, (RB, 128), 0)
                            s = jnp.where(pos >= 2 * w, s, NEG)
                        logits.append(s)
                    m = functools.reduce(jnp.maximum, logits)
                    e = [jnp.exp2(s - m) for s in logits]
                    den = functools.reduce(jnp.add, e)
                    rinv = 1.0 / den
                    for l in range(LT):
                        acc = None
                        for w in range(BW):
                            pr = e[w] * qkvb_ref[2 * LT + l, r0 - 2 * w:r0 - 2 * w + RB, :]
                            acc = pr if acc is None else acc + pr
                        acc = acc * rinv
                        if RB == 8:
                            obf_ref[slot, rb * RB:(rb + 1) * RB, l * 128:(l + 1) * 128] = acc
                        else:
                            ob_ref[slot, rb * RB // 2:(rb + 1) * RB // 2, l * 128:(l + 1) * 128] = _u32(acc.astype(jnp.bfloat16))
                        st["bv", rb] = [rinv, acc, m, logits[0], logits[4]][bsync]
                        st["bvl"] = jnp.concatenate([acc] * 2, axis=0)[:16]
                if rbs[1] == TB // RB and not (first and joint) and not (pair and slot == 0):
                    qkvb_ref[LT:, 0:HALO, :] = qkvb_ref[LT:, q0 + TB - HALO:q0 + TB, :]

            def GATE(gr):
                gr = gr or TB
                gw = gw_ref[...].astype(jnp.float32).reshape(1, D)
                gs = []
                for r0 in range(0, TB, gr):
                    xf = x_ref[pl.ds(t * TB + r0 if isinstance(t, int) else pl.multiple_of(t * TB + r0, gr), gr), :]
                    xf = xf.astype(jnp.float32) * gw
                    part = functools.reduce(jnp.add, [xf[:, l * 128:(l + 1) * 128] for l in range(LT)])
                    if gs:
                        part = jnp.where(opaque(gr), jnp.broadcast_to(gs[-1], (gr, 128)), part)
                    z = jnp.sum(part, axis=-1, keepdims=True)
                    gs.append(1.0 / (1.0 + jnp.exp(-z)))
                st["gate"] = jnp.concatenate(gs, axis=0) if len(gs) > 1 else gs[0]
                if want(t, "GATE"):
                    st["GATE"] = _fold(jnp.broadcast_to(gs[-1], (gr, 128)))

            def BP(cs):
                c0, c1 = cs or (0, LT)
                cl = slice(c0 * 128, c1 * 128)
                ob = obf_ref[slot] if RB == 8 else _bf16(dep_on(ob_ref[slot]))
                b = lax.dot_general(ob, _bf16(wobp_ref[:, cl]), _NN, preferred_element_type=jnp.float32)
                for c in range(c0, c1):
                    st["bp", c] = b[:, (c - c0) * 128:(c - c0 + 1) * 128]
                b = (1.0 - st["gate"]) * b
                st["b_done"] = True
                bacc_ref[slot, :, cl] = b
                if want(t, "BP"):
                    st["BP"] = _fold(b)

            def max4(b):
                return jnp.maximum(jnp.maximum(b[0:8], b[8:16]), jnp.maximum(b[16:24], b[24:32]))

            def QK(n):
                qb, g = chunks[n]
                qr = qr_ref[slot * NQB + qb, 40 * g:40 * g + 40, :]
                qr = dep_on(qr)
                if not isinstance(t, int) and bforce is not None and n == bforce:
                    qr = jnp.concatenate([jnp.where(opaque(16), _u32(st["bvl"]), qr[0:16]), qr[16:]], axis=0)
                zero24 = jnp.zeros((24, 128), jnp.uint32)
                out = [None] * 4
                for j in ([(jj + rot0 * n) % 4 for jj in range(4)] if first else range(4)):
                    J = 4 * qb + j
                    wq = jnp.concatenate([jnp.where(hcls == j, qr, jnp.uint32(0)), zero24], axis=0)
                    sh = (40 * g) % 64
                    wt = jnp.concatenate([wq[64 - sh:], wq[:64 - sh]], axis=0) if sh else wq
                    blocks = [None] * 8
                    if first:
                        kwin = kg_ref[g, 0:16 * (J + 1), :]
                        s = jnp.dot(_bf16(kwin), _bf16(wt), preferred_element_type=jnp.float32)
                        blocks[0] = jnp.where(tri, NEG, s[32 * J:32 * J + 32])
                        for i in range(J):
                            blocks[8 - J + i] = s[32 * i:32 * i + 32]
                    else:
                        base = hoff(16 * J - WIN // 2, 16)
                        kwin = jnp.concatenate([kg_ref[g, pl.ds(base, 16), :],
                                                kg_ref[g, pl.ds(base + 128, 16), :],
                                                kg_ref[g, pl.ds(base + 16, 112), :]], axis=0)
                        s = jnp.dot(_bf16(kwin), _bf16(wt), preferred_element_type=jnp.float32)
                        blocks[0] = jnp.where(tri, s[0:32], s[32:64])
                        for i in range(1, 8):
                            blocks[i] = s[32 * i + 32:32 * i + 64]
                    run = []
                    for b in blocks:
                        if b is not None:
                            run.append(max4(b) if not run else jnp.maximum(run[-1], max4(b)))
                    m = jnp.broadcast_to(jnp.max(run[-1], axis=0, keepdims=True), (8, 128))
                    if sx:
                        for i, b in enumerate(blocks):
                            if b is not None:
                                sc_ref[n % sx, j, 32 * i:32 * i + 32, :] = b
                    out[j] = (blocks, run, m)
                st["s", n] = out

            def PV(n):
                qb, g = chunks[n]
                sc = st.pop(("s", n))
                pc = pace0 if first else (pace1 if isinstance(t, int) and pace1 is not None else pace)
                off = poff0 if first else 1
                nxt = st.get(("s", n + off)) if pc is not None else None
                if first and nxt is not None:
                    nxt = [nxt[(j + rot0 * off) % 4] for j in range(4)]
                a0 = (2 - qb) if first else 0
                pcs = [None] * 4
                Wh = [[], [], [], []]

                hist = []
                ec = (ech0 if first else ech).get(n, 0)

                def prob(j, kk):
                    blocks, _, m = sc[j]
                    if first:
                        i = (kk + j - 4 * a0 + 1 if kk else 0) - pc if nxt is not None else -1
                    else:
                        i = kk + j - pc if nxt is not None else -1
                    if i >= 0:
                        m = jnp.where(opaque(), nxt[j][1][min(i, len(nxt[j][1]) - 1)], m)
                    if n in bpace and (bpace0 or not first):
                        pos = bpace[n][0] + bpace[n][1] * len(hist)
                        if pos >= 0:
                            m = jnp.where(opaque(), st["bp", pos // 32][8 * (pos % 32):8 * (pos % 32) + 8], m)
                    if ec and len(hist) >= ec:
                        m = jnp.where(opaque(), hist[-ec][24:32], m)
                    sv = sc_ref[n % sx, j, 32 * kk:32 * kk + 32, :] if sx else blocks[kk]
                    hist.append(jnp.exp2(sv - jnp.concatenate([m] * 4, axis=0)))
                    return hist[-1]

                def sel(m, a, b):
                    if a is None and b is None:
                        return None
                    return jnp.where(m, zero16 if a is None else a, zero16 if b is None else b)

                if first:
                    for j in range(4):
                        pcs[j] = _pack_shuffled(jnp.where(tri, 0.0, prob(j, 0)))
                for kb in range(4 * a0, 12):
                    src = []
                    for j in range(4):
                        kk = kb - j
                        if kk == 0:
                            pd = prob(j, 0)
                            src.append(_pack_shuffled(jnp.where(tri, pd, 0.0)))
                            pcs[j] = _pack_shuffled(jnp.where(tri, 0.0, pd))
                        elif 0 < kk < 8:
                            src.append(_pack_shuffled(prob(j, kk)))
                        elif kk == 8:
                            src.append(pcs[j])
                        else:
                            src.append(None)
                    inn = [src[(-i) % 4] for i in range(4)]
                    tt = [sel(b0, inn[r], inn[(r - 1) % 4]) for r in range(4)]
                    for r in range(4):
                        Wh[r].append(sel(b1, tt[r], tt[(r - 2) % 4]))
                        if wx:
                            w_ref[n % wx, r, 16 * kb:16 * kb + 16, :] = Wh[r][-1]
                accs = [None] * 4
                for a in range(a0, 3):
                    for hh in range(4):
                        h = 4 * g + hh
                        if wx:
                            w = _bf16(w_ref[n % wx, hh, 64 * a:64 * a + 64, :])
                        else:
                            w = _bf16(jnp.concatenate(Wh[hh][4 * (a - a0):4 * (a - a0) + 4], axis=0))
                        v = vtp_ref[t * NQB + qb + a - 2, 24 * h:24 * h + 24, :]
                        d = lax.dot_general(v, w, _NN, preferred_element_type=jnp.float32)
                        accs[hh] = d if accs[hh] is None else accs[hh] + d
                r8 = lax.broadcasted_iota(jnp.int32, (8, 128), 0) < 4
                blk = []
                for hp in range(2):
                    ea, ob_ = accs[2 * hp], accs[2 * hp + 1]
                    rz = 1.0 / jnp.where(r8, ob_[0:8], ea[16:24])
                    rs = pltpu.roll(rz, 4, 0)
                    ra, rb_ = jnp.where(r8, rs, rz), jnp.where(r8, rz, rs)
                    blk += [ea[0:8] * ra, ea[8:16] * ra, jnp.where(r8, ea[16:24], ob_[0:8]) * rs,
                            ob_[8:16] * rb_, ob_[16:24] * rb_]
                ot_ref[slot * NQB + qb, 80 * g:80 * g + 80, :] = jnp.concatenate(blk, axis=0)
                st["PV", n] = jnp.concatenate(blk[8:10], axis=0)

            def FIN(qb):
                for l in range(LT):
                    z = ot_ref[slot * NQB + qb, l * 128:(l + 1) * 128, :].T
                    zu = _u32(z.astype(jnp.bfloat16))
                    hd = (l * 128 + l16) // DH
                    h0 = (hd & 1) == 0
                    h1 = (hd & 2) == 0
                    zc = [zu[16 * c:16 * c + 16] for c in range(4)]
                    tt = [jnp.where(h0, zc[j], zc[(j + 1) % 4]) for j in range(4)]
                    oj = [jnp.where(h1, tt[j], tt[(j + 2) % 4]) for j in range(4)]
                    oa_ref[slot, qb * 64:(qb + 1) * 64, l * 128:(l + 1) * 128] = jnp.concatenate(oj, axis=0)
                    if want(t, "FIN%d" % qb):
                        fo = _fold(jnp.concatenate(oj, axis=0))
                        st["FIN%d" % qb] = fo if l == 0 else st["FIN%d" % qb] | fo

            def AP(qb):
                r = slice(qb * 128, (qb + 1) * 128)
                a = jnp.dot(_bf16(dep_on(oa_ref[slot, qb * 64:(qb + 1) * 64, :])), woa_ref[...], preferred_element_type=jnp.float32)
                if isinstance(t, int):
                    dst = pl.ds(t * TB + qb * 128, 128)
                else:
                    dst = pl.ds(pl.multiple_of(t * TB + qb * 128, 128), 128)
                if "b_done" in st:
                    a = (st["gate"][r] * a + bacc_ref[slot, r, :]).astype(o_ref.dtype)
                    o_ref[dst, :] = a
                else:
                    st["a_done"] = True
                    a = st["gate"][r] * a
                    bacc_ref[slot, r, :] = a
                if want(t, "AP%d" % qb):
                    st["AP%d" % qb] = _fold(a)

            def OS(qbs):
                for qb in (qbs or (0, 1)):
                    qb, n = qb if isinstance(qb, tuple) else (qb, 1)
                    ocopy(t, qb, n).start()
                    pend.extend([(t, qb, n)] if isinstance(t, int) else [(tt, qb, n) for tt in range(2, nrun)][::2 if pair else 1])

            def SPIN(n):
                acc = lax.fori_loop(0, n, lambda i, a: a * 1.0001 + 1.0, jnp.zeros((8, 128), jnp.float32))
                sc_ref[0, 0, 0:8, 0:128] = acc

            fns = dict(PBX=PBX, PREP=PREP, WW=WW, WS=WS, XW=XW, XS=XS, PB=PB, PK=PK, QT=QT, VT=VT, BV=BV, GATE=GATE, BP=BP,
                       QK=QK, PV=PV, FIN=FIN, AP=AP, OS=OS, SPIN=SPIN)
            return fns

        z_ref[1] = jnp.zeros((8, 128), jnp.int32)
        fs = [tile_fns(tt, tt % 2) for tt in range(NT)]
        for it in order0[nlead:]:
            cur["deps"] = it[3] if len(it) > 3 else ()
            fs[it[2] if len(it) > 2 else 0][it[0]](it[1])
        cur["deps"] = ()

        def loop_body(t, c):
            fns = tile_fns(t)
            for it in order1:
                cur["deps"] = it[3] if len(it) > 3 else ()
                fns[it[0]](it[1])
            cur["deps"] = ()
            return c
        def pair_body(i, c):
            for sl in range(2):
                fns = tile_fns(2 * i + sl, sl)
                for it in order1:
                    cur["deps"] = it[3] if len(it) > 3 else ()
                    fns[it[0]](it[1])
                cur["deps"] = ()
            return c
        t1 = 2 if joint else 1
        if pair:
            lax.fori_loop(1, nrun // 2, pair_body, 0)
        elif nrun > t1:
            lax.fori_loop(t1, nrun, loop_body, 0)
        if oshift:
            fs[nrun - 1]["OS"]((1,))
        for args in pend:
            ocopy(*args).wait()

    return kernel


def attn_order(lo=0, hi=NQB * NG, extra=None, last=("BP", 0), first=True, depth=1):
    extra = extra or {}
    nch = NQB * NG
    order = [("QK", lo + i) for i in range(depth)] if first else []
    for n in range(lo, hi):
        if n + depth < nch:
            order.append(("QK", n + depth))
        elif last and n == nch - 1:
            order.append(last)
        order += extra.get(n, [])
        order.append(("PV", n))
        if n % NG == NG - 1:
            order.append(("FIN", n // NG))
    return order


def orders(v0=0, depth=1, v1=0, p=None):
    NRB = TB // RB
    order1 = [("XW", 0), ("XS", 1), ("PB", (0, 3)), ("PK", 0), ("QT", 0), ("VT", 0), ("BV", (0, NRB)), ("GATE", 0)]
    if v1 == 0:
        order1 += attn_order(depth=depth) + [("AP", 0), ("AP", 1), ("OS", 0)]
    elif v1 == 1:
        order1 += [("BP", 0)] + attn_order(depth=depth, last=("AP", 0)) + [("AP", 1), ("OS", 0)]
    elif v1 == 3:
        order1 += attn_order(depth=depth, last=None, extra={14: [("BP", 0)]}) + [("AP", 0), ("AP", 1), ("OS", 0)]
    elif v1 == 4:
        order1 += attn_order(depth=depth, last=None, extra={14: [("BP", 0)]}) + [("AP", 0), ("OS", (0,)), ("AP", 1), ("OS", (1,))]
    elif v1 == 5:
        order1 = [("XW", 0), ("XS", 1), ("GATE", 0), ("PB", (0, 3, (p or {}).get("gn", 8), 0), 0, [("L", "GATE")]), ("PK", 0), ("QT", 0), ("VT", 0), ("BV", (0, NRB))]
        order1 += attn_order(depth=depth, last=None, extra={14: [("BP", 0)]}) + [("AP", 0), ("OS", (0,)), ("AP", 1), ("OS", (1,))]
    elif v1 == 6:
        q = dict(dict(gn=8, fq=10, bs=2, b1=14, b2=15), **(p or {}))
        order1 = [("XW", 0), ("XS", 1)]
        if q["gn"] is None:
            order1 += [("PB", (0, 3)), ("GATE", 0)]
        else:
            order1 += [("GATE", 0), ("PB", (0, 3, q["gn"], 0), 0, [("L", "GATE")])]
        order1 += [("PK", 0), ("QT", 0), ("VT", 0), ("BV", (0, NRB))]
        ex = {q["b1"]: [("BP", (0, q["bs"]))]}
        ex.setdefault(q["b2"], []).append(("BP", (q["bs"], LT)))
        order1 += attn_order(depth=depth, last=None, extra=ex) + [("AP", 0), ("OS", (0,)), ("AP", 1), ("OS", (1,))]
        if q["fq"] is not None:
            i = order1.index(("QK", q["fq"]))
            order1[i] = ("QK", q["fq"], 0, [("L", "FIN0")])
    elif v1 == 7:
        q = dict(dict(bs=4, b1=14, b2=15, pbs=1), **(p or {}))
        order1 = [("PBX", (0, 15, 0, 128)), ("PBX", (0, 15, 128, 256))] if q["pbs"] else [("PB", (0, 3))]
        order1 += [("GATE", q.get("gr1", 0)), ("QT", 0), ("VT", 0), ("BV", (0, NRB))]
        ex = {q["b1"]: [("BP", (0, q["bs"]))]}
        ex.setdefault(q["b2"], []).append(("BP", (q["bs"], LT)))
        order1 += attn_order(depth=depth, last=None, extra=ex) + [("AP", 0), ("OS", (0,)), ("AP", 1), ("OS", (1,))]
    elif v1 == 2:
        order1 += [("BP", 0)] + attn_order(depth=depth, last=None, extra={14: [("AP", 0)]}) + [("AP", 1), ("OS", 0)]
    def T(items, tile):
        return [(n, a, tile) for n, a in items]

    B = (0, NRB)
    att0 = attn_order(depth=2, last=None)
    if v0 == 0:
        order0 = [("WS", 20), ("XS", 0), ("WS", 1), ("XS", 1), ("WS", 8)] + [("WS", i) for i in (3, 4, 5, 2, 0, 6, 7)]
        order0 += [("XW", 0), ("WW", 1), ("XS", 2), ("PK", 0),
                   ("XW", 0, 1), ("WW", 8), ("WW", 20), ("WW", 3), ("PREP", 3), ("PK", 0, 1), ("GATE", 0), ("GATE", 0, 1),
                   ("WW", 4), ("PREP", 4), ("PB", (0, 1)), ("PB", (0, 1), 1),
                   ("WW", 5), ("WW", 2), ("PREP", 5), ("PREP", 2), ("PB", (1, 2)), ("PB", (1, 2), 1),
                   ("WW", 0), ("WW", 6), ("WW", 7),
                   ("PREP", 0), ("PREP", 6), ("PB", (2, 3)), ("PB", (2, 3), 1), ("VT", 0), ("QT", 0), ("VT", 0, 1), ("QT", 0, 1),
                   ("BV", B), ("BV", B, 1)]
        order0 += att0 + [("BP", 0)]
        order0 += T(attn_order(depth=depth, last=None, extra={14: [("BP", 0)]}), 1)
        i = order0.index(("PV", 1, 1))
        order0[i:i] = [("AP", 0), ("AP", 1), ("OS", 0)]
        order0 += T([("AP", 0), ("AP", 1), ("OS", 0)], 1)
    if v0 == 1:
        order0 = [("WS", 20), ("XS", 0), ("WS", 1), ("XS", 1), ("WS", 8)] + [("WS", i) for i in (3, 4, 5, 2, 0, 6, 7)]
        order0 += [("XW", 0), ("WW", 1), ("XS", 2), ("PK", 0),
                   ("XW", 0, 1), ("WW", 8), ("WW", 20), ("WW", 3), ("PREP", 3), ("PK", 0, 1), ("GATE", 0), ("GATE", 0, 1),
                   ("PB", (0, 1)),
                   ("WW", 4), ("PREP", 4), ("PB", (0, 1), 1), ("PB", (1, 2)),
                   ("WW", 5), ("WW", 2), ("WW", 0), ("PREP", 5), ("PB", (1, 2), 1), ("PB", (2, 3)), ("PREP", 2), ("PB", (2, 3), 1),
                   ("BV", B), ("BV", B, 1),
                   ("PREP", 0), ("VT", 0), ("QT", 0), ("VT", 0, 1), ("QT", 0, 1)]
        order0 += att0 + [("WW", 6), ("WW", 7), ("PREP", 6), ("AP", 0), ("AP", 1), ("BP", 0), ("OS", 0)]
        order0 += T(attn_order(depth=depth, last=None, extra={14: [("BP", 0)]}), 1)
        order0 += T([("AP", 0), ("AP", 1), ("OS", 0)], 1)
    if v0 in (2, 3):
        order0 = [("WS", 20), ("XS", 0), ("WS", 1), ("XS", 1), ("WS", 8)] + [("WS", i) for i in (3, 4, 5, 2, 0, 6, 7)]
        order0 += [("XW", 0), ("WW", 1), ("XS", 2), ("PK", 0),
                   ("XW", 0, 1), ("WW", 8), ("WW", 20), ("WW", 3), ("PREP", 3), ("PK", 0, 1),
                   ("PB", (0, 1)),
                   ("WW", 4), ("PREP", 4), ("PB", (0, 1), 1), ("PB", (1, 2)),
                   ("WW", 5), ("WW", 2), ("WW", 0), ("PREP", 5), ("PB", (1, 2), 1), ("PB", (2, 3)), ("PREP", 2), ("PB", (2, 3), 1),
                   ("BV", B),
                   ("PREP", 0), ("VT", 0), ("QT", 0)]
        if v0 == 2:
            order0 += att0
            order0 += [("WW", 6), ("WW", 7), ("PREP", 6), ("VT", 0, 1)]
        else:
            order0 += attn_order(depth=2, last=None, extra={14: [("VT", 0, 1)]})[:-1]
            order0 += [("WW", 6), ("WW", 7), ("PREP", 6), ("FIN", 1)]
        order0 += [("QT", 0, 1), ("BV", B, 1), ("GATE", 0), ("GATE", 0, 1),
                   ("AP", 0), ("AP", 1), ("BP", 0), ("OS", 0)]
        order0 += T(attn_order(depth=depth, last=None, extra={14: [("BP", 0)]}), 1)
        order0 += T([("AP", 0), ("AP", 1), ("OS", 0)], 1)
    def addep(order, item, deps):
        i = order.index(item)
        order[i] = (item[0], item[1], item[2] if len(item) > 2 else 0, deps)

    if v0 == 4:
        order0 = [("WS", 20), ("XS", 0), ("WS", 1), ("XS", 1), ("WS", 8)] + [("WS", i) for i in (3, 4, 5, 2, 0, 6, 7)]
        order0 += [("XW", 0), ("WW", 1), ("XS", 2), ("PK", 0),
                   ("XW", 0, 1), ("WW", 8), ("WW", 20), ("WW", 3), ("PREP", 3), ("PK", 0, 1),
                   ("PB", (0, 1)),
                   ("WW", 4), ("PREP", 4), ("PB", (0, 1), 1), ("PB", (1, 2)),
                   ("WW", 5), ("WW", 2), ("PREP", 5), ("PB", (1, 2), 1), ("GATE", 0), ("GATE", 0, 1), ("PREP", 2), ("PB", (2, 3)),
                   ("VT", 0, 0, [(0, "GATE"), (1, "GATE")]),
                   ("WW", 0), ("WW", 6), ("WW", 7),
                   ("PREP", 0), ("PREP", 6), ("BV", B), ("PB", (2, 3), 1), ("VT", 0, 1, [(0, ("PREP", 6))]), ("QT", 0)]
        order0 += attn_order(depth=2, last=None, extra={14: [("QT", 0, 1)]})
        addep(order0, ("QK", 2), [(0, "bvl")])
        order0 += [("BV", B, 1), ("BP", 0), ("AP", 0), ("AP", 1), ("OS", 0)]
        order0 += T(attn_order(depth=depth, last=None, extra={14: [("BP", 0)]}), 1)
        addep(order0, ("QK", 2, 1), [(1, "bvl")])
        addep(order0, ("QK", 3, 1), [(0, "AP0"), (0, "AP1")])
        order0 += T([("AP", 0), ("AP", 1), ("OS", 0)], 1)
    if v0 in (5, 6, 7):
        order0 = [("WS", 20), ("XS", 0), ("WS", 1), ("XS", 1), ("WS", 8)] + [("WS", i) for i in (3, 4, 6, 5, 2, 0, 7)]
        order0 += [("XW", 0), ("WW", 1), ("XS", 2), ("PK", 0),
                   ("XW", 0, 1), ("WW", 8), ("WW", 20), ("WW", 3), ("PREP", 3), ("PK", 0, 1), ("GATE", 0), ("GATE", 0, 1),
                   ("PB", (0, 1), 0, [(0, "GATE"), (1, "GATE")]),
                   ("WW", 4), ("WW", 6), ("PREP", 4), ("PB", (0, 1), 1), ("PREP", 6), ("PB", (1, 2), 0, [(0, ("PREP", 6))]),
                   ("WW", 5), ("WW", 2), ("PREP", 5), ("PB", (1, 2), 1), ("PREP", 2), ("PB", (2, 3), 0, [(0, ("PREP", 2))]),
                   ("WW", 0), ("WW", 7),
                   ("PREP", 0), ("BV", B), ("PB", (2, 3), 1), ("VT", 0)]
        p = dict(dict(f0=2, s1=12, f1=2, fa=3, d0=2, x0=14), **(p or {}))
        if v0 == 7:
            H0, H1 = (0, 128), (128, 256)
            order0 = [("WS", (3, k)) for k in range(LT)] + [("WS", (30, 0)), ("WS", (30, 1)), ("WS", 32), ("WS", 8), ("WS", 1),
                                                            ("WS", 20)]
            late = [(4,), (5, 6), (2, 0, 7), (31,), ()]
            for k in range(LT):
                order0 += [("WW", (3, k))] + [("WS", i) for i in late[k]]
                order0 += [("PREP", (3, k, "A"))] + [("PREP", (3, k - 1, "B"))] * (k > 0)
            order0 += [("WW", (30, 0)), ("PREP", (3, LT - 1, "B")), ("PBX", (0, 4) + H0),
                       ("WW", (30, 1)), ("WW", 32), ("WW", 8), ("WW", 20), ("GATE", 0), ("GATE", 0, 1),
                       ("PBX", (4, 5) + H0), ("PBX", (0, 5) + H1), ("PBX", (0, 5) + H0 + (0, 0), 1, [(0, "GATE")]),
                       ("PBX", (0, 5) + H1 + (0, 0), 1, [(1, "GATE")]),
                       ("WW", 1), ("PK", H0), ("PK", H1),
                       ("WW", 4), ("PREP", 4), ("PK", 0, 1), ("PBX", (5, 8, 0, TB)),
                       ("WW", 5), ("WW", 6), ("PREP", 5), ("PBX", (8, 10, 0, TB)), ("PB", (1, 2), 1), ("PREP", 6),
                       ("PB", (2, 3), 0, [(0, ("PREP", 6))]),
                       ("WW", 2), ("WW", 0), ("WW", 7),
                       ("PREP", 2), ("BV", B), ("PB", (2, 3), 1), ("PREP", 0), ("VT", 0)]
            order0 += [("VT", 0, 1), ("QT", 0)] if p.get("vq") else [("QT", 0), ("VT", 0, 1)]
            order0 += attn_order(depth=p["d0"], last=None, extra={p["x0"]: [("QT", 0, 1)]})
        elif v0 == 5:
            order0 += [("QT", 0), ("VT", 0, 1)]
            order0 += attn_order(depth=p["d0"], last=None, extra={p["x0"]: [("QT", 0, 1)]})
        else:
            order0 += [("QT", 0)]
            order0 += attn_order(depth=2, last=None, extra={14: [("QT", 0, 1)]}) + [("VT", 0, 1)]
        p = dict(dict(f0=2, s1=12, f1=2, fa=3), **(p or {}))
        addep(order0, ("QK", p["f0"]), [(0, "bvl")])
        order0 += [("BV", B, 1, [(0, ("PV", p["s1"]))] if p["s1"] is not None else []), ("BP", 0), ("AP", 0), ("AP", 1), ("OS", 0)]
        order0 += T(attn_order(depth=depth, last=None, extra={14: [("BP", 0)]}), 1)
        if p["f1"] == p["fa"]:
            addep(order0, ("QK", p["f1"], 1), [(1, "bvl"), (0, "AP0"), (0, "AP1")])
        else:
            addep(order0, ("QK", p["f1"], 1), [(1, "bvl")])
            if p["fa"] is not None:
                addep(order0, ("QK", p["fa"], 1), [(0, "AP0"), (0, "AP1")])
        order0 += T([("AP", 0), ("AP", 1), ("OS", 0)], 1)
    if v0 == 8:
        p = dict(dict(f0=2, s1=11, f1=2, fa=3, d0=4, x0=12, ks=2, p6=1, bs1=4, gr=0, gp=3, gq=2,
                      pk={2: [(5, 0)], 4: [(5, 1)], 6: [(6, 0)], 8: [(6, 1)], 10: [(7, 0)], 14: [(7, 1)]}), **(p or {}))
        ks = p["ks"]
        X = lambda a, b=None: (30, 2 * a, 2 * (a + 1 if b is None else b))
        G = [[X(0), (1, 0, ks)], [X(1)], [(1, ks, LT)], [3, X(2), 8, 20], [4, 5, X(3)], [6, 2, 0, 7, X(4, 8)]]
        W = lambda g: [("SPIN", 100)] * (p.get("spin") == g) + [("WW", k) for k in G[g]]
        order0 = [("WS", k) for g in G for k in g if k != 20] + [("WS", 20)]
        HH = lambda k0, k1, tt: [("PK", (0, 128, k0, k1), tt), ("PK", (128, 256, k0, k1), tt)]
        order0 += W(0) + HH(0, ks, 0)
        order0 += W(1) + HH(0, ks, 1)
        order0 += W(2) + [("PK", (0, TB, ks, LT), 0)] + HH(ks, LT, 1)
        gr = p["gr"]
        if p["gp"] == 3:
            order0 += W(3) + [("PREP", 3), ("PK", 0, 2), ("GATE", gr), ("GATE", gr, 1), ("PB", (0, 1)),
                              ("PBX", (0, 2, 0, TB, 0, 0), 1, [(0, "GATE"), (1, "GATE")])]
            order0 += W(4) + [("PREP", 4), ("PBX", (2, 5, 0, TB), 1), ("PK", 0, 3), ("PREP", 5), ("PB", (1, 2)), ("PB", (1, 2), 1),
                              ("PB", (2, 3)), ("PB", (2, 3), 1)]
        else:
            order0 += W(3) + [("PREP", 3), ("PK", 0, 2), ("PB", (0, 1)), ("PBX", (0, 2, 0, TB), 1)]
            order0 += W(4) + [("PREP", 4), ("PBX", (2, 5, 0, TB), 1), ("PK", 0, 3), ("PREP", 5), ("PB", (1, 2)), ("PB", (1, 2), 1),
                              ("GATE", gr), ("GATE", gr, 1), ("PB", (2, 3)),
                              ("PB", (2, 3, p["gq"], 0), 1, [(0, "GATE"), (1, "GATE")])]
        order0 += W(5) + [("PREP", 2), ("BV", B), ("PK", 0, 4), ("PREP", 0), ("VT", 0), ("PREP", 6),
                          ("QT", 0, 0, [(0, ("PREP", 6))] if p["p6"] == 0 else []),
                          ("VT", 0, 1, [(0, ("PREP", 6))] if p["p6"] == 1 else [])]
        pk = p["pk"]
        ex = {n: [("PK", (128 * h, 128 * h + 128), tt) for tt, h in v] for n, v in pk.items()}
        ex.setdefault(p["x0"], []).append(("QT", 0, 1))
        order0 += attn_order(depth=p["d0"], last=None, extra=ex)
        addep(order0, ("QK", p["f0"]), [(0, "bvl")])
        order0 += [("BV", B, 1, [(0, ("PV", p["s1"]))] if p["s1"] is not None else [])] + ex.get(16, [])
        order0 += [("BP", 0)] + ex.get(17, []) + [("AP", 0), ("AP", 1), ("OS", 0)] + ex.get(18, [])
        order0 += T(attn_order(depth=depth, last=None, extra={14: [("BP", (0, p["bs1"]))], 15: [("BP", (p["bs1"], LT))] * (p["bs1"] < LT)}), 1)
        addep(order0, ("QK", p["f1"], 1), [(1, "bvl")])
        if p["fa"] is not None:
            addep(order0, ("QK", p["fa"], 1), [(0, "AP0"), (0, "AP1")])
        order0 += T([("AP", 0), ("AP", 1), ("OS", 0)], 1)
        return order0, order1, {k: ("G", i) for i, g in enumerate(G) for k in g}
    if v0 == 9:
        p = dict(dict(f0=2, s1=11, f1=2, fa=3, d0=4, x0=12, ks=2, bs1=4, gr=32, bk=8, c4=4, p6=1,
                      pk={2: [(6, 0)], 5: [(6, 1)], 8: [(7, 0)], 10: [(7, 1)]}), **(p or {}))
        ks, gr, bk, c4 = p["ks"], p["gr"], p["bk"], p["c4"]
        X = lambda a, b: (30, a, b)
        G = [[X(0, 2), (1, 0, ks)], [X(2, 5)], [(1, ks, LT)], [3, X(5, 8), 8, 20], [4, 5, X(8, 10), 6], [2, 0, 7, X(10, 16)]]
        W = lambda g: [("SPIN", 100)] * (p.get("spin") == g) + [("WW", k) for k in G[g]]
        order0 = [("WS", k) for g in G for k in g if k != 20] + [("WS", 20)]
        PKS = lambda tt, r0, r1, n, k0, k1: [("PK", (r, r + n, k0, k1), tt) for r in range(r0, r1, n)]
        order0 += W(0) + PKS(0, 0, TB, 128, 0, ks)
        order0 += W(1) + PKS(1, 0, TB, 128, 0, ks) + PKS(2, 0, 128, 64, 0, ks)
        order0 += W(2) + PKS(0, 0, TB, 128, ks, LT) + PKS(1, 0, TB, 128, ks, LT) + PKS(2, 0, 128, 64, ks, LT)
        order0 += W(3) + [("PREP", 3), ("PK", (128, TB), 2), ("PK", 0, 3), ("GATE", gr), ("GATE", gr, 1), ("PB", (0, 1)),
                          ("PB", (0, 1, 2, 0), 1, [(0, "GATE"), (1, "GATE")])]
        order0 += W(4) + [("PREP", 4), ("PK", 0, 4), ("PREP", 5), ("PB", (1, 2)), ("PREP", 6),
                          ("PB", (2, 3), 0, [(0, ("PREP", 6))] * p["p6"])] + [("BV", (0, bk))] * (bk > 0)
        order0 += [("PB", (1, 2), 1), ("PBX", (10, 10 + c4, 0, TB), 1)]
        order0 += W(5) + [("PREP", 2), ("BV", (bk, NRB))] + [("PBX", (10 + c4, 15, 0, TB), 1)] * (c4 < 5)
        order0 += [("PK", 0, 5), ("PREP", 0), ("VT", 0), ("QT", 0), ("VT", 0, 1)]
        pk = p["pk"]
        ex = {n: [("PK", (128 * h, 128 * h + 128), tt) for tt, h in v] for n, v in pk.items()}
        ex.setdefault(p["x0"], []).append(("QT", 0, 1))
        if p.get("bp0") is not None:
            ex.setdefault(p["bp0"], []).append(("BP", 0))
        order0 += attn_order(depth=p["d0"], last=None, extra=ex)
        addep(order0, ("QK", p["f0"]), [(0, "bvl")])
        order0 += [("BV", B, 1, [(0, ("PV", p["s1"]))] if p["s1"] is not None else [])] + ex.get(16, [])
        order0 += [("BP", 0)] * (p.get("bp0") is None) + ex.get(17, []) + [("AP", 0), ("AP", 1), ("OS", 0)] + ex.get(18, [])
        if p.get("fq1") is not None:
            addep(order0, p["fq1"], [(1, "QT")])
        order0 += T(attn_order(depth=depth, last=None, extra={14: [("BP", (0, p["bs1"]))], 15: [("BP", (p["bs1"], LT))] * (p["bs1"] < LT)}), 1)
        addep(order0, ("QK", p["f1"], 1), [(1, "bvl")])
        if p["fa"] is not None:
            addep(order0, ("QK", p["fa"], 1), [(0, "AP0"), (0, "AP1")])
        order0 += T([("AP", 0), ("AP", 1), ("OS", 0)], 1)
        return order0, order1, {k: ("G", i) for i, g in enumerate(G) for k in g}
    if v0 == 10:
        p = dict(dict(f0=2, f1=2, fa=3, d0=4, ks=2, bs1=4, gr=32, bk=0, c4=4, p6=1, fb=0,
                      ex={1: [("BP", (0, 1))], 3: [("BP", (1, 2))], 5: [("BP", (2, 3))], 7: [("BP", (3, 4))], 9: [("BP", (4, 5))],
                          12: [("AP", 0)]}), **(p or {}))
        ks, gr, bk, c4 = p["ks"], p["gr"], p["bk"], p["c4"]
        X = lambda a, b: (30, a, b)
        G = [[X(0, 2), (1, 0, ks)], [X(2, 5)], [(1, ks, LT)], [3, X(5, 8), 8, 20], [4, 5, X(8, 10), 6], [2, 0, 7, X(10, 16)]]
        W = lambda g: [("SPIN", 100)] * (p.get("spin") == g) + [("WW", k) for k in G[g]]
        order0 = [("WS", k) for g in G for k in g if k != 20] + [("WS", 20)]
        PKS = lambda tt, r0, r1, n, k0, k1: [("PK", (r, r + n, k0, k1), tt) for r in range(r0, r1, n)]
        order0 += W(0) + PKS(0, 0, TB, 128, 0, ks)
        order0 += W(1) + PKS(1, 0, TB, 128, 0, ks) + PKS(2, 0, 128, 64, 0, ks)
        order0 += W(2) + PKS(0, 0, TB, 128, ks, LT) + PKS(1, 0, TB, 128, ks, LT) + PKS(2, 0, 128, 64, ks, LT)
        order0 += W(3) + [("PREP", 3), ("PK", (128, TB), 2), ("PK", 0, 3), ("GATE", gr), ("GATE", gr, 1), ("PB", (0, 1)),
                          ("PB", (0, 1, 2, 0), 1, [(0, "GATE"), (1, "GATE")])]
        order0 += W(4) + [("PREP", 4), ("PK", 0, 4), ("PREP", 5), ("PB", (1, 2)), ("PREP", 6),
                          ("PB", (2, 3), 0, [(0, ("PREP", 6))] * p["p6"])] + [("BV", (0, bk))] * (bk > 0)
        order0 += [("PB", (1, 2), 1), ("PBX", (10, 10 + c4, 0, TB), 1)]
        order0 += W(5) + [("PREP", 2), ("BV", (bk, NRB))] + [("PBX", (10 + c4, 15, 0, TB), 1)] * (c4 < 5)
        order0 += [("PK", 0, 5), ("PREP", 0), ("BV", B, 1, [(0, "bvl")]), ("VT", 0), ("PK", 0, 6), ("QT", 0), ("PK", 0, 7), ("VT", 0, 1), ("QT", 0, 1)]
        ex = p["ex"]
        order0 += attn_order(depth=p["d0"], last=None, extra=ex)
        addep(order0, ("QK", p["f0"]), [(1, "bvl")])
        done = [it for v in ex.values() for it in v]
        rest = [it for it in [("AP", 0), ("AP", 1)] if it not in done] + [("OS", 0)]
        a1 = T(attn_order(depth=depth, last=None, extra={14: [("BP", (0, p["bs1"]))], 15: [("BP", (p["bs1"], LT))] * (p["bs1"] < LT)}), 1)
        i = p.get("ai", 2)
        order0 += a1[:i] + rest + a1[i:]
        if p["fa"] is not None:
            addep(order0, ("QK", p["fa"], 1), [(0, "AP0"), (0, "AP1")])
        order0 += T([("AP", 0), ("AP", 1), ("OS", 0)], 1)
        return order0, order1, {k: ("G", i) for i, g in enumerate(G) for k in g}
    return order0, order1, None


def build(rb=16, nsem=8, v0=0, nrun=NT, cut=None, pace=None, depth=1, v1=0, p=None, xall=True, **kw):
    global RB
    RB = rb
    o0, o1, semmap = orders(v0, depth, v1, p)
    if semmap is None:
        o0 = [("WS", 31) if it == ("XS", 2) else it for it in o0] + [("WW", 31)]
        semmap = {32: (30, 1), 8: (30, 1), 20: (30, 1), 4: (3, 0), 5: (3, 1), 6: (3, 1), 2: (3, 2), 0: (3, 2), 7: (3, 2),
                  31: (3, 3), "o": (3, 4)}
    o1 = [it for it in o1 if it[0] not in ("XW", "XS")]
    kw["semmap"] = semmap
    if kw.get("oshift"):
        o1 = [("OS", ((-1, 2),)) if it == ("OS", (0,)) else it for it in o1 if it != ("OS", (1,))]
        i = o0.index(("OS", 0, 1))
        o0 = o0[:i - 1] + [("OS", (0,), 1), o0[i - 1]] + o0[i + 1:]
        o0 = [("OS", ((0, 2),)) if it == ("OS", 0) else it for it in o0]
    kernel = make_kernel(o0, o1, nrun=nrun, pace=pace, **kw)
    anyspec = pl.BlockSpec(memory_space=pl.ANY)

    @jax.jit
    def f(A_x, A_wqkv, A_wo, B_x, B_wqkv, B_wo, gate_w):
        x = A_x.reshape(S, D)
        out = pl.pallas_call(
            kernel,
            in_specs=[anyspec] * 6,
            out_specs=anyspec,
            out_shape=jax.ShapeDtypeStruct((S, D), jnp.bfloat16),
            scratch_shapes=[
                pltpu.VMEM((S, D), jnp.bfloat16),
                pltpu.VMEM((D, 3 * D), jnp.bfloat16),
                pltpu.VMEM((D, D), jnp.bfloat16),
                pltpu.VMEM((D, 3 * D), jnp.bfloat16),
                pltpu.VMEM((D, D), jnp.bfloat16),
                pltpu.VMEM((D,), jnp.bfloat16),
                pltpu.VMEM((S, D), jnp.bfloat16),
                pltpu.VMEM((D // 2, D), jnp.uint32),
                pltpu.VMEM((D // 2, D), jnp.uint32),
                pltpu.VMEM((3 * D // 2, D), jnp.uint32),
                pltpu.VMEM((D // 2, D), jnp.uint32),
                pltpu.VMEM((NG, S // 2, 128), jnp.uint32),
                pltpu.VMEM((S // 128, H * 24, 128), jnp.float32),
                pltpu.VMEM((2 * NQB, D // 2, 128), jnp.uint32),
                pltpu.VMEM((3 * LT, HALO + 2 * TB, 128), jnp.float32),
                pltpu.VMEM((2 * NQB, D, 128), jnp.float32),
                pltpu.VMEM((2, TB // 2, D), jnp.uint32),
                pltpu.VMEM((2, TB // 2, D), jnp.uint32),
                pltpu.VMEM((5, LT, D, 128), jnp.float32),
                pltpu.VMEM((LT, D // 2, 128), jnp.uint32),
                pltpu.VMEM((2, TB, D), jnp.float32),
                pltpu.VMEM((2, 8, 128), jnp.int32),
                pltpu.VMEM((16, 4, 256, 128), jnp.float32),
                pltpu.VMEM((16, 4, 192, 128), jnp.uint32),
                pltpu.VMEM((3, TB, D), jnp.float32),
                pltpu.VMEM((2, TB, D), jnp.float32),
                pltpu.SemaphoreType.DMA((nsem,)),
            ],
            compiler_params=pltpu.CompilerParams(
                vmem_limit_bytes=100 * 1024 * 1024,
            ),
        )(x, A_wqkv, A_wo, B_wqkv, B_wo, gate_w)
        return out.reshape(1, S, D)
    return f


_impl = build(v0=9, pace=1, depth=2, v1=7, bchain=1, bforce=2, bchain0=1, pace1=1, wvf=True, bpace={14:(0,1), 15:(32,2)}, pchain=(3,4,5,6), nsem=7, oshift=True, p=dict(bk=0))


@jax.jit
def pallas_gated_mix__sliding_block__sliding_local_dilated__prompt_kernel(
    A_x: jax.Array,
    A_wqkv: jax.Array,
    A_wo: jax.Array,
    B_x: jax.Array,
    B_wqkv: jax.Array,
    B_wo: jax.Array,
    gate_w: jax.Array,
):
    return _impl(A_x, A_wqkv, A_wo, B_x, B_wqkv, B_wo, gate_w)
```

```python
import functools
import math

import jax
import jax.numpy as jnp
from jax import lax
import jax.experimental.pallas as pl
import jax.experimental.pallas.tpu as pltpu

S = 2048
D = 640
H = 32
DH = 20
WIN = 256
NG = 8
LT = D // 128
BW = 8
HALO = 16
TB = 256
NT = S // TB
NQB = TB // 128
RB = 16

QSCALE = (DH ** -0.5) * math.log2(math.e)
ONE_BITS = 0x3F803F80
NEG = -1e30

_NT = (((1,), (1,)), ((), ()))
_NN = (((1,), (0,)), ((), ()))


def _u32(x):
    return pltpu.bitcast(x, jnp.uint32)


def _bf16(x):
    return pltpu.bitcast(x, jnp.bfloat16)


def _pack2(a, b):
    return pltpu.pack_elementwise([a, b], packed_dtype=jnp.bfloat16).astype(jnp.uint32)


def _pack_shuffled(p):
    R, C = p.shape
    p3 = p.reshape(R // 16, 16, C)
    w = pltpu.pack_elementwise([p3[:, :8, :], p3[:, 8:, :]], packed_dtype=jnp.bfloat16)
    return w.reshape(R // 2, C).astype(jnp.uint32)


def _fold(v):
    u = _u32(v)
    R, C = u.shape
    parts = [u[r:r + 16, c:c + 128] for r in range(0, R, 16) for c in range(0, C, 128)]
    while len(parts) > 1:
        parts = [parts[i] | parts[i + 1] if i + 1 < len(parts) else parts[i] for i in range(0, len(parts), 2)]
    return parts[0]


def _lane_range_mask(shape, lo, n):
    lane = lax.broadcasted_iota(jnp.int32, shape, 1)
    lo = lo % 128
    if lo + n <= 128:
        return (lane >= lo) & (lane < lo + n)
    return (lane >= lo) | (lane < lo + n - 128)


def make_kernel(order0, order1, nrun=NT, pace=None, bchain=0, bsync=0, bforce=None, joint=True, bchain0=0, pace0=None, pace1=None, rot0=1, poff0=1, pchain=(4, 5, 6), ech={}, ech0={}, semmap={}, wvf=False, wqf=False, bpace={}, sx=0, wx=0, qchain=0, bpace0=0, pair=False, oshift=False, bfull=0, bfull0=0, bval=0, gbc=0, ksplit={}, nchain=0, swp=0, xsp=None, bvo=0, bvo0=None, bsync0=None, ao=0, ao1=0, noos=0, ofin=None, dpr=0, opr=0):

    def kernel(x_hbm, wa_hbm, woa_hbm, wb_hbm, wob_hbm, gw_hbm, o_hbm,
               x_ref, wa_ref, woa_ref, wb_ref, wob_ref, gw_ref, o_ref,
               wvt_ref, wqt_ref, wbt_ref, wobp_ref, kg_ref, vtp_ref, qr_ref, qkvb_ref,
               ot_ref, oa_ref, ob_ref, tmps_ref, tmpu_ref, bacc_ref, z_ref, sc_ref, w_ref, pk_ref, obf_ref, wq0_ref, xs_ref, gt_ref,
               wsem):

        sems = {}
        sts = {}

        cur = {"deps": ()}
        wanted = {d for it in order0 + order1 if len(it) > 3 for d in it[3]}

        def want(t, key):
            return (t if isinstance(t, int) else "L", key) in wanted

        def sem_of(key):
            key = semmap.get(key, key)
            return wsem.at[sems.setdefault(key, len(sems))]

        def wcopy(key):
            i, kt = key[:2] if isinstance(key, tuple) else (key, None)
            r = slice(None) if kt is None else slice(kt * 128, (key[2] if len(key) > 2 else kt + 1) * 128)
            sem = sem_of(key)
            if i == 20:
                return pltpu.make_async_copy(z_ref.at[1], z_ref.at[0], sem)
            if i == 45:
                return pltpu.make_async_copy(wb_hbm.at[:, D:], wb_ref.at[:, D:], sem)
            if i == 32:
                return pltpu.make_async_copy(x_hbm.at[TB:2 * TB, :], x_ref.at[TB:2 * TB, :], sem)
            if i == 31:
                return pltpu.make_async_copy(x_hbm.at[2 * TB:, :], x_ref.at[2 * TB:, :], sem)
            if i == 30:
                if len(key) > 3:
                    c = slice(key[3] * 128, key[4] * 128)
                    return pltpu.make_async_copy(x_hbm.at[r, c], x_ref.at[r, c], sem)
                return pltpu.make_async_copy(x_hbm.at[r, :], x_ref.at[r, :], sem)
            if i < 3:
                return pltpu.make_async_copy(wa_hbm.at[r, i * D:(i + 1) * D], wa_ref.at[r, i * D:(i + 1) * D], sem)
            if i < 6:
                p = i - 3
                return pltpu.make_async_copy(wb_hbm.at[r, p * D:(p + 1) * D], wb_ref.at[r, p * D:(p + 1) * D], sem)
            if i == 6:
                return pltpu.make_async_copy(wob_hbm, wob_ref, sem)
            if i == 7:
                return pltpu.make_async_copy(woa_hbm, woa_ref, sem)
            return pltpu.make_async_copy(gw_hbm, gw_ref, sem)

        def rows(t):
            if isinstance(t, int):
                return pl.ds(t * TB, TB)
            return pl.ds(pl.multiple_of(t * TB, TB), TB)

        def xcopy(t):
            sem = sem_of("x1") if (isinstance(t, int) and t == 1) else sem_of("x")
            return pltpu.make_async_copy(x_hbm.at[rows(t), :], x_ref.at[rows(t), :], sem)

        def ocopy(t, qb, n=1, c0=0, c1=LT):
            r = t * TB + int(qb * 128)
            r = pl.ds(r if isinstance(t, int) else pl.multiple_of(r, 16), int(128 * n))
            c = slice(c0 * 128, c1 * 128)
            return pltpu.make_async_copy(o_ref.at[r, c], o_hbm.at[r, c], sem_of("o"))
        pend = []

        nlead = 0
        while order0[nlead][0] == "WS" and order0[nlead][1] != 20:
            wcopy(order0[nlead][1]).start(priority=int(nlead >= dpr - 1) if dpr else 0)
            nlead += 1

        rr = lax.broadcasted_iota(jnp.int32, (32, 128), 0)
        ll = lax.broadcasted_iota(jnp.int32, (32, 128), 1)
        tri = rr > (ll & 31)
        l16 = lax.broadcasted_iota(jnp.int32, (16, 128), 1)
        b0 = (l16 & 32) == 0
        b1 = (l16 & 64) == 0
        zero16 = jnp.zeros((16, 128), jnp.uint32)
        chunks = [(qb, g) for qb in range(NQB) for g in range(NG)]
        hcls = ((lax.broadcasted_iota(jnp.int32, (40, 128), 1) >> 5)
                - lax.broadcasted_iota(jnp.int32, (40, 128), 0) // 10) & 3

        def tile_fns(t, slot=0):
            first = isinstance(t, int) and t == 0
            st = {}
            sts[t if isinstance(t, int) else "L"] = st
            q0 = HALO + slot * TB

            def opaque(rows=8):
                o = z_ref[0] != 0
                return o if rows == 8 else jnp.concatenate([o] * (rows // 8), axis=0)

            def dep_on(u, r0=0, c0=0):
                deps = cur["deps"]
                if not deps:
                    return u
                blk = u[r0:r0 + 16, c0:c0 + 128]
                for b, key in deps:
                    blk = jnp.where(opaque(16), _u32(sts[b][key]), blk)
                R, C = u.shape
                mid = [u[r0:r0 + 16, :c0]] * (c0 > 0) + [blk] + [u[r0:r0 + 16, c0 + 128:]] * (c0 + 128 < C)
                mid = jnp.concatenate(mid, axis=1) if len(mid) > 1 else blk
                full = [u[:r0]] * (r0 > 0) + [mid] + [u[r0 + 16:]] * (r0 + 16 < R)
                return jnp.concatenate(full, axis=0) if len(full) > 1 else mid

            def hoff(base, mult):
                if isinstance(t, int):
                    return t * (TB // 2) + base
                return pl.multiple_of(t * (TB // 2) + base, mult)

            def PREP(key):
                i, kt, ph = (key + ("AB",))[:3] if isinstance(key, tuple) else (key, None, "AB")
                kts = range(LT) if kt is None else [kt]
                outs = []
                chain = want(t, ("PREP", key))

                def link(o):
                    if chain and outs:
                        o = jnp.where(opaque(o.shape[0]), outs[-1], o)
                    outs.append(o)

                def xpose(blk):
                    if key in pchain and "T" in st:
                        top = jnp.where(jnp.concatenate([opaque()] * LT, axis=1),
                                        jnp.concatenate([st["T"]] * LT, axis=1), blk[0:8])
                        blk = jnp.concatenate([top, blk[8:]], axis=0)
                    bt = blk.T
                    st["T"] = bt[D - 8:]
                    return bt
                st.pop("T", None)
                if i in (0, 2):
                    dst = wvt_ref if i == 2 else wqt_ref
                    tmp_ref = tmps_ref.at[i // 2]
                    for kt in kts:
                        blk = wa_ref[kt * 128:(kt + 1) * 128, i * D:(i + 1) * D].astype(jnp.float32)
                        tmp_ref[kt] = xpose(blk)
                        if (i == 2 and wvf) or (i == 0 and wqf):
                            continue
                        if i == 2:
                            a = tmp_ref[kt, pl.ds(0, D // 2, stride=2), :]
                            b = tmp_ref[kt, pl.ds(1, D // 2, stride=2), :]
                            link(_pack2(a, b))
                            dst[:, kt * 128:(kt + 1) * 128] = outs[-1]
                            continue
                        for par in range(2):
                            a = tmp_ref[kt, pl.ds(par, D // 4, stride=4), :]
                            b = tmp_ref[kt, pl.ds(par + 2, D // 4, stride=4), :]
                            link(_pack2(a, b))
                            dst[par * (D // 4):(par + 1) * (D // 4), kt * 128:(kt + 1) * 128] = outs[-1]
                elif i < 6:
                    p = i - 3
                    tmp_ref = tmps_ref.at[2 + p]
                    for kt in kts:
                        if "A" in ph:
                            blk = wb_ref[kt * 128:(kt + 1) * 128, p * D:(p + 1) * D].astype(jnp.float32)
                            tmp_ref[kt] = xpose(blk)
                        for d in range(DH) if "B" in ph else ():
                            ev = tmp_ref[kt, pl.ds(d, H // 2, stride=2 * DH), :]
                            od = tmp_ref[kt, pl.ds(d + DH, H // 2, stride=2 * DH), :]
                            link(_pack2(ev, od))
                            r0 = (p * D + d * H) // 2
                            wbt_ref[r0:r0 + H // 2, kt * 128:(kt + 1) * 128] = outs[-1]
                else:
                    for lt in range(LT):
                        u = _u32(wob_ref[:, lt * 128:(lt + 1) * 128])
                        if key in pchain and outs:
                            u = jnp.where(opaque(D // 2), jnp.concatenate([outs[-1]] * (D // 64), axis=0), u)
                        tmpu_ref[lt] = u
                        for d2 in range(DH // 2):
                            ev = tmpu_ref[lt, pl.ds(d2, H // 2, stride=DH), :]
                            od = tmpu_ref[lt, pl.ds(d2 + DH // 2, H // 2, stride=DH), :]
                            lo = (ev & jnp.uint32(0xFFFF)) | (od << 16)
                            hi = (ev >> 16) | (od & jnp.uint32(0xFFFF0000))
                            link(jnp.concatenate([lo, hi], axis=0))
                            wobp_ref[d2 * H:(d2 + 1) * H, lt * 128:(lt + 1) * 128] = outs[-1]
                if want(t, ("PREP", key)):
                    st["PREP", key] = _fold(outs[-1])

            def WW(i):
                wcopy(i).wait()

            def WS(i):
                wcopy(i).start()

            def XW(_):
                xcopy(t).wait()

            def XS(k):
                if isinstance(t, int):
                    if t + k < nrun:
                        xcopy(t + k).start()
                else:
                    @pl.when(t + 1 < nrun)
                    def _():
                        xcopy(t + 1).start()

            def xdep():
                xb = x_ref[rows(t), :]
                return _bf16(dep_on(_u32(xb))) if cur["deps"] else xb

            def PB(ps):
                xb = x_ref[rows(t), :]
                lo, hi = ps[:2]
                w = wbt_ref[lo * D // 2:hi * D // 2, :]
                if cur["deps"]:
                    nt, kt = ps[2:] if len(ps) > 2 else (LT - 1, 0)
                    w = dep_on(w, 64 * nt, 128 * kt)
                ksp = [0] + list(ksplit.get((lo, t), ())) + [LT]
                qkvb = functools.reduce(jnp.add, [
                    lax.dot_general(xb[:, 128 * a:128 * b], _bf16(w[:, 128 * a:128 * b]), _NT, preferred_element_type=jnp.float32)
                    for a, b in zip(ksp[:-1], ksp[1:])])
                for l in range((hi - lo) * LT):
                    v = qkvb[:, l * 128:(l + 1) * 128]
                    if lo * LT + l < LT:
                        v = v * QSCALE
                    qkvb_ref[lo * LT + l, q0:q0 + TB, :] = v

            def PBX(a, pre=False):
                c0, c1, r0, r1 = a[:4]
                if ("PBX", a) in st:
                    xb, w = st.pop(("PBX", a))
                else:
                    xb = x_ref[pl.ds(t * TB + r0 if isinstance(t, int) else pl.multiple_of(t * TB + r0, 16), r1 - r0), :]
                    w = wbt_ref[64 * c0:64 * c1, :]
                    if cur["deps"]:
                        nt, kt = a[4:] if len(a) > 4 else (c1 - c0 - 1, 0)
                        w = dep_on(w, 64 * nt, 128 * kt)
                    if pre:
                        st["PBX", a] = (xb, w)
                        return
                if xsp and not isinstance(t, int) and "xs" not in st and r0 == xsp[2]:
                    xu = _pack_shuffled(x_ref[rows(t), :].astype(jnp.float32))
                    st["xs"] = xu
                    n0, stp = xsp[:2]
                    for i in range(2 * LT):
                        pos = n0 + stp * i
                        st["xsf"] = _fold(xu[64 * (i % 2):64 * (i % 2) + 64, 128 * (i // 2):128 * (i // 2) + 128])
                        cur["deps"] = [("L", "xsf")]
                        w = dep_on(w, 64 * (pos // LT), 128 * (pos % LT))
                    cur["deps"] = ()
                qkvb = lax.dot_general(xb, _bf16(w), _NT, preferred_element_type=jnp.float32)
                for l in range(c0, c1):
                    v = qkvb[:, (l - c0) * 128:(l - c0 + 1) * 128]
                    if l < LT:
                        v = v * QSCALE
                    qkvb_ref[l, q0 + r0:q0 + r1, :] = v

            def PREPN(cs):
                last = None
                for c in range(*(cs or (0, 1))):
                    for kt in range(LT):
                        w = _bf16(wbt_ref[64 * c:64 * c + 64, kt * 128:(kt + 1) * 128]).astype(jnp.float32)
                        if nchain and last is not None and kt % nchain == 0:
                            w = jnp.concatenate([jnp.where(opaque(), last, w[0:8]), w[8:]], axis=0)
                        w = w.T
                        last = w[120:]
                        wq0_ref[64 * kt:64 * kt + 64, 128 * c:128 * c + 128] = _u32(w.astype(jnp.bfloat16))

            def PBN(a):
                r0, r1, c0, c1 = (a + (0, 1))[:4]
                xb = x_ref[pl.ds(pl.multiple_of(t * TB + r0, 16), r1 - r0), :]
                q = jnp.dot(xb, _bf16(wq0_ref[:, 128 * c0:128 * c1]), preferred_element_type=jnp.float32)
                for l in range(c0, c1):
                    v = q[:, (l - c0) * 128:(l - c0 + 1) * 128]
                    qkvb_ref[l, q0 + r0:q0 + r1, :] = v * QSCALE if l < LT else v

            def groups(tiles, zero):
                shp = tiles[0].shape
                out = []
                for g in range(NG):
                    lo, hi = 80 * g, 80 * g + 80
                    t0, t1 = lo // 128, (hi - 1) // 128
                    if t0 == t1:
                        v = tiles[t0]
                        if zero:
                            v = jnp.where(_lane_range_mask(shp, lo, 80), v, jnp.uint32(0))
                    else:
                        n0 = 128 * t1 - lo
                        m0 = _lane_range_mask(shp, lo, n0)
                        v = tiles[t1]
                        if zero:
                            v = jnp.where(_lane_range_mask(shp, 0, 80 - n0), v, jnp.uint32(0))
                        v = jnp.where(m0, tiles[t0], v)
                    out.append(v)
                return out

            def PK(rr_, pre=False):
                r0, r1, k0, k1 = (tuple(rr_) + (0, LT))[:4] if rr_ else (0, TB, 0, LT)
                if ("PK", rr_) in st:
                    xb, w = st.pop(("PK", rr_))
                else:
                    xb = x_ref[t * TB + r0:t * TB + r1, k0 * 128:k1 * 128] if rr_ else xdep()
                    if rr_ and cur["deps"]:
                        xb = _bf16(dep_on(_u32(xb)))
                    w = wa_ref[k0 * 128:k1 * 128, D:2 * D]
                    if pre:
                        st["PK", rr_] = (xb, w)
                        return
                k = jnp.dot(xb, w, preferred_element_type=jnp.float32)
                if k0 > 0:
                    k = k + pk_ref[t * TB + r0:t * TB + r1, :]
                if k1 < LT:
                    pk_ref[t * TB + r0:t * TB + r1, :] = k
                    return
                kt_ = [_u32(k[:, l * 128:(l + 1) * 128].astype(jnp.bfloat16)) for l in range(LT)]
                for g, v in enumerate(groups(kt_, False)):
                    kg_ref[g, pl.ds(hoff(r0 // 2, 32), (r1 - r0) // 2), :] = v

            def QT(gs_):
                g0, g1 = gs_ or (0, NG)
                xb = x_ref[rows(t), :]
                if gs_:
                    w = jnp.concatenate([wqt_ref[par * (D // 4) + 20 * g0:par * (D // 4) + 20 * g1, :] for par in range(2)], axis=0)
                else:
                    w = wqt_ref[...]
                w = _bf16(dep_on(w))
                qt = lax.dot_general(w, xb, _NT, preferred_element_type=jnp.float32) * QSCALE
                nr = 40 * (g1 - g0)
                qtu = _pack2(qt[:nr], qt[nr:])
                s8 = lax.broadcasted_iota(jnp.int32, (8, 128), 0)
                for qb in range(NQB):
                    for g in range(g0, g1):
                        blk = []
                        for v in range(5):
                            u = qtu[40 * (g - g0) + 8 * v:40 * (g - g0) + 8 * v + 8, qb * 128:(qb + 1) * 128]
                            if qchain and v == 4 and "qc" in st:
                                u = jnp.where(opaque(), st["qc"], u)
                            lo, hi = (16 * v) // DH, (16 * v + 15) // DH
                            rl = lambda r: pltpu.roll(u, 32 * r, 1) if r else u
                            if lo == hi:
                                blk.append(rl(lo))
                            else:
                                blk.append(jnp.where(s8 < (DH * hi - 16 * v) // 2, rl(lo), rl(hi)))
                        qr_ref[slot * NQB + qb, 40 * g:40 * g + 40, :] = jnp.concatenate(blk, axis=0)
                        st["qc"] = blk[4]
                        if want(t, "QT"):
                            fo = blk[0] | blk[1] | blk[2] | blk[3] | blk[4]
                            st["QTf"] = fo if "QTf" not in st else st["QTf"] | fo
                            st["QT"] = jnp.concatenate([st["QTf"]] * 2, axis=0)

            def VT(_):
                if (swp & 1) and not isinstance(t, int):
                    xs = _bf16(xs_ref[...])
                elif "xs" in st:
                    xs = _bf16(st["xs"])
                else:
                    xf = x_ref[rows(t), :].astype(jnp.float32)
                    xs = _bf16(_pack_shuffled(xf))
                if wvf:
                    w = jnp.concatenate([tmps_ref[1, kt] for kt in range(LT)], axis=1)
                    w = pltpu.bitcast(dep_on(_u32(w)), jnp.float32) if cur["deps"] else w
                else:
                    w = _bf16(dep_on(wvt_ref[...]))
                ksp = [0] + list(ksplit.get(("V", t), ()) if isinstance(t, int) else ()) + [LT]
                vt = functools.reduce(jnp.add, [
                    lax.dot_general(w[:, 128 * a:128 * b], xs[:, 128 * a:128 * b], _NT, preferred_element_type=jnp.float32)
                    for a, b in zip(ksp[:-1], ksp[1:])])
                r8 = lax.broadcasted_iota(jnp.int32, (8, 128), 0) < 4
                for qb in range(NQB):
                    tile = t * NQB + qb
                    for hp in range(H // 2):
                        win = vt[40 * hp:40 * hp + 40, qb * 128:(qb + 1) * 128]
                        mid = win[16:24]
                        vtp_ref[tile, 48 * hp:48 * hp + 48, :] = jnp.concatenate(
                            [win[0:16], jnp.where(r8, mid, 1.0), jnp.where(r8, 1.0, mid), win[24:40]], axis=0)

            def BV(rbs, bvo=bvo, bsync=bsync):
                if isinstance(t, int):
                    bvo = bvo if bvo0 is None else (bvo0[t] if isinstance(bvo0, tuple) else bvo0)
                    bsync = bsync if bsync0 is None else (bsync0[t] if isinstance(bsync0, tuple) else bsync0)
                if first and rbs[0] == 0:
                    qkvb_ref[LT:, 0:HALO, :] = jnp.zeros((2 * LT, HALO, 128), jnp.float32)
                for rb in range(*rbs):
                    r0 = q0 + rb * RB
                    q = [qkvb_ref[l, r0:r0 + RB, :] for l in range(LT)]
                    bc = bchain0 if first else bchain
                    if rb == rbs[0] and cur["deps"]:
                        q = [pltpu.bitcast(dep_on(_u32(jnp.concatenate([v] * (16 // min(RB, 16)), axis=0))), jnp.float32)[:RB] for v in q]
                    if bc and rb >= bc:
                        dep = st["bv", rb - bc]
                        q = [jnp.where(opaque(RB), dep, v) for v in q]
                    bf = bfull0 if isinstance(t, int) else bfull
                    if bf and rb >= bf:
                        dep = pltpu.bitcast(jnp.concatenate([st["bvf", rb - bf]] * 2, axis=0), jnp.float32)
                        q[0] = jnp.where(opaque(RB), dep, q[0])
                    logits = [None] * BW
                    wo = list(range(BW))[::-1 if bvo & 1 else 1]
                    lo_ = list(range(LT))[::-1 if bvo & 2 else 1]
                    for w in wo:
                        s = None
                        for l in lo_:
                            pr = q[l] * qkvb_ref[LT + l, r0 - 2 * w:r0 - 2 * w + RB, :]
                            s = pr if s is None else s + pr
                        if bvo & 4:
                            s = s + pltpu.roll(s, 32, 1)
                            s = s + pltpu.roll(s, 64, 1)
                        else:
                            s = s + pltpu.roll(s, 64, 1)
                            s = s + pltpu.roll(s, 32, 1)
                        if first and rb * RB < 2 * w:
                            pos = rb * RB + lax.broadcasted_iota(jnp.int32, (RB, 128), 0)
                            s = jnp.where(pos >= 2 * w, s, NEG)
                        logits[w] = s
                    def tree(f, v):
                        if not bvo & 8:
                            return functools.reduce(f, [v[w] for w in wo])
                        while len(v) > 1:
                            v = [f(v[i], v[i + 1]) for i in range(0, len(v), 2)]
                        return v[0]
                    m = tree(jnp.maximum, logits)
                    e = [jnp.exp2(s - m) for s in logits]
                    den = tree(jnp.add, e)
                    rinv = 1.0 / den
                    for l in range(LT):
                        acc = None
                        for w in (wo[::-1] if bvo & 16 else wo):
                            pr = e[w] * qkvb_ref[2 * LT + l, r0 - 2 * w:r0 - 2 * w + RB, :]
                            acc = pr if acc is None else acc + pr
                        acc = acc * rinv
                        if RB == 8:
                            obf_ref[slot, rb * RB:(rb + 1) * RB, l * 128:(l + 1) * 128] = acc
                        else:
                            pk_ = _u32(acc.astype(jnp.bfloat16))
                            ob_ref[slot, rb * RB // 2:(rb + 1) * RB // 2, l * 128:(l + 1) * 128] = pk_
                            st["bvf", rb] = pk_ if l == 0 else st["bvf", rb] | pk_
                        st["bv", rb] = [rinv, acc, m, logits[0], logits[4]][bsync]
                        st["bvl"] = jnp.concatenate([acc] * 2, axis=0)[:16]
                    if bf and rb == rbs[1] - 1:
                        fo = functools.reduce(jnp.bitwise_or, [st["bvf", rb - k] for k in range(bf) if ("bvf", rb - k) in st])
                        st["bvl"] = pltpu.bitcast(jnp.concatenate([fo] * 2, axis=0), jnp.float32)
                if rbs[1] == TB // RB and not (first and joint) and not (pair and slot == 0):
                    qkvb_ref[LT:, 0:HALO, :] = qkvb_ref[LT:, q0 + TB - HALO:q0 + TB, :]

            def NXT(_):
                tn = t + 1 if isinstance(t, int) else jnp.minimum(t + 1, NT - 1)
                xf = x_ref[rows(tn), :].astype(jnp.float32)
                if swp & 1:
                    xs_ref[...] = _pack_shuffled(xf)
                if swp & 2:
                    xg = xf * gw_ref[...].astype(jnp.float32).reshape(1, D)
                    part = functools.reduce(jnp.add, [xg[:, l * 128:(l + 1) * 128] for l in range(LT)])
                    z = jnp.broadcast_to(jnp.sum(part, axis=-1, keepdims=True), (TB, 128))
                    gt_ref[...] = 1.0 / (1.0 + jnp.exp(-z))

            def GATE(gr):
                if (swp & 2) and not isinstance(t, int):
                    st["gate"] = gt_ref[...]
                    return
                gr = gr or TB
                gw = gw_ref[...].astype(jnp.float32).reshape(1, D)
                gs = []
                for r0 in range(0, TB, gr):
                    xf = x_ref[pl.ds(t * TB + r0 if isinstance(t, int) else pl.multiple_of(t * TB + r0, gr), gr), :]
                    xf = xf.astype(jnp.float32) * gw
                    part = functools.reduce(jnp.add, [xf[:, l * 128:(l + 1) * 128] for l in range(LT)])
                    if gs:
                        part = jnp.where(opaque(gr), jnp.broadcast_to(gs[-1], (gr, 128)), part)
                    z = jnp.sum(part, axis=-1, keepdims=True)
                    if gbc == 2:
                        z = jnp.broadcast_to(z, (gr, 128))
                    gs.append(1.0 / (1.0 + jnp.exp(-z)))
                    if gbc == 1:
                        gs[-1] = jnp.broadcast_to(gs[-1], (gr, 128))
                st["gate"] = jnp.concatenate(gs, axis=0) if len(gs) > 1 else gs[0]
                if want(t, "GATE"):
                    st["GATE"] = _fold(jnp.broadcast_to(gs[-1], (gr, 128)))

            def BP(cs):
                c0, c1 = cs or (0, LT)
                cl = slice(c0 * 128, c1 * 128)
                ob = obf_ref[slot] if RB == 8 else _bf16(dep_on(ob_ref[slot]))
                b = lax.dot_general(ob, _bf16(wobp_ref[:, cl]), _NN, preferred_element_type=jnp.float32)
                for c in range(c0, c1):
                    st["bp", c] = b[:, (c - c0) * 128:(c - c0 + 1) * 128]
                g1 = 1.0 - st["gate"]
                b = (jnp.concatenate([g1] * (c1 - c0), axis=1) if gbc else g1) * b
                st["b_done"] = True
                if bval == 1 or (bval == 2 and isinstance(t, int)):
                    st.setdefault("bv_", []).append(b)
                else:
                    bacc_ref[slot, :, cl] = b
                if want(t, "BP"):
                    st["BP"] = _fold(b)

            def max4(b):
                return jnp.maximum(jnp.maximum(b[0:8], b[8:16]), jnp.maximum(b[16:24], b[24:32]))

            def QK(n):
                qb, g = chunks[n]
                qr = qr_ref[slot * NQB + qb, 40 * g:40 * g + 40, :]
                qr = dep_on(qr)
                if not isinstance(t, int) and bforce is not None and n == bforce:
                    qr = jnp.concatenate([jnp.where(opaque(16), _u32(st["bvl"]), qr[0:16]), qr[16:]], axis=0)
                zero24 = jnp.zeros((24, 128), jnp.uint32)
                out = [None] * 4
                aoo = ao1 if isinstance(t, int) else ao
                jo = [[0, 1, 2, 3], [3, 2, 1, 0], [(jj + n) % 4 for jj in range(4)], [(jj - n) % 4 for jj in range(4)]][aoo & 3]
                for j in ([(jj + rot0 * n) % 4 for jj in range(4)] if first else jo):
                    J = 4 * qb + j
                    wq = jnp.concatenate([jnp.where(hcls == j, qr, jnp.uint32(0)), zero24], axis=0)
                    sh = (40 * g) % 64
                    wt = jnp.concatenate([wq[64 - sh:], wq[:64 - sh]], axis=0) if sh else wq
                    blocks = [None] * 8
                    if first:
                        kwin = kg_ref[g, 0:16 * (J + 1), :]
                        s = jnp.dot(_bf16(kwin), _bf16(wt), preferred_element_type=jnp.float32)
                        blocks[0] = jnp.where(tri, NEG, s[32 * J:32 * J + 32])
                        for i in range(J):
                            blocks[8 - J + i] = s[32 * i:32 * i + 32]
                    else:
                        base = hoff(16 * J - WIN // 2, 16)
                        kwin = jnp.concatenate([kg_ref[g, pl.ds(base, 16), :],
                                                kg_ref[g, pl.ds(base + 128, 16), :],
                                                kg_ref[g, pl.ds(base + 16, 112), :]], axis=0)
                        s = jnp.dot(_bf16(kwin), _bf16(wt), preferred_element_type=jnp.float32)
                        blocks[0] = jnp.where(tri, s[0:32], s[32:64])
                        for i in range(1, 8):
                            blocks[i] = s[32 * i + 32:32 * i + 64]
                    run = []
                    for b in blocks:
                        if b is not None:
                            run.append(max4(b) if not run else jnp.maximum(run[-1], max4(b)))
                    m = jnp.broadcast_to(jnp.max(run[-1], axis=0, keepdims=True), (8, 128))
                    if sx:
                        for i, b in enumerate(blocks):
                            if b is not None:
                                sc_ref[n % sx, j, 32 * i:32 * i + 32, :] = b
                    out[j] = (blocks, run, m)
                st["s", n] = out

            def PV(n):
                qb, g = chunks[n]
                sc = st.pop(("s", n))
                pc = pace0 if first else (pace1 if isinstance(t, int) and pace1 is not None else pace)
                off = poff0 if first else 1
                nxt = st.get(("s", n + off)) if pc is not None else None
                if first and nxt is not None:
                    nxt = [nxt[(j + rot0 * off) % 4] for j in range(4)]
                a0 = (2 - qb) if first else 0
                pcs = [None] * 4
                Wh = [[], [], [], []]

                hist = []
                ec = (ech0 if first else ech).get(n, 0)

                def prob(j, kk):
                    blocks, _, m = sc[j]
                    if first:
                        i = (kk + j - 4 * a0 + 1 if kk else 0) - pc if nxt is not None else -1
                    else:
                        i = kk + j - pc if nxt is not None else -1
                    if i >= 0:
                        m = jnp.where(opaque(), nxt[j][1][min(i, len(nxt[j][1]) - 1)], m)
                    if n in bpace and (bpace0 or not first):
                        pos = bpace[n][0] + bpace[n][1] * len(hist)
                        if pos >= 0:
                            m = jnp.where(opaque(), st["bp", pos // 32][8 * (pos % 32):8 * (pos % 32) + 8], m)
                    if ec and len(hist) >= ec:
                        m = jnp.where(opaque(), hist[-ec][24:32], m)
                    sv = sc_ref[n % sx, j, 32 * kk:32 * kk + 32, :] if sx else blocks[kk]
                    hist.append(jnp.exp2(sv - jnp.concatenate([m] * 4, axis=0)))
                    return hist[-1]

                def sel(m, a, b):
                    if a is None and b is None:
                        return None
                    return jnp.where(m, zero16 if a is None else a, zero16 if b is None else b)

                if first:
                    for j in range(4):
                        pcs[j] = _pack_shuffled(jnp.where(tri, 0.0, prob(j, 0)))
                for kb in range(4 * a0, 12):
                    src = []
                    for j in range(4):
                        kk = kb - j
                        if kk == 0:
                            pd = prob(j, 0)
                            src.append(_pack_shuffled(jnp.where(tri, pd, 0.0)))
                            pcs[j] = _pack_shuffled(jnp.where(tri, 0.0, pd))
                        elif 0 < kk < 8:
                            src.append(_pack_shuffled(prob(j, kk)))
                        elif kk == 8:
                            src.append(pcs[j])
                        else:
                            src.append(None)
                    inn = [src[(-i) % 4] for i in range(4)]
                    tt = [sel(b0, inn[r], inn[(r - 1) % 4]) for r in range(4)]
                    for r in range(4):
                        Wh[r].append(sel(b1, tt[r], tt[(r - 2) % 4]))
                        if wx:
                            w_ref[n % wx, r, 16 * kb:16 * kb + 16, :] = Wh[r][-1]
                accs = [None] * 4
                aoo = 0 if first else ao1 if isinstance(t, int) else ao
                hho = [[0, 1, 2, 3], [3, 2, 1, 0]][(aoo >> 2) & 1]
                ah = [(a, hh) for a in range(a0, 3) for hh in hho]
                if aoo & 8:
                    ah = [(a, hh) for hh in hho for a in range(a0, 3)]
                for a, hh in ah:
                    if True:
                        h = 4 * g + hh
                        if wx:
                            w = _bf16(w_ref[n % wx, hh, 64 * a:64 * a + 64, :])
                        else:
                            w = _bf16(jnp.concatenate(Wh[hh][4 * (a - a0):4 * (a - a0) + 4], axis=0))
                        v = vtp_ref[t * NQB + qb + a - 2, 24 * h:24 * h + 24, :]
                        d = lax.dot_general(v, w, _NN, preferred_element_type=jnp.float32)
                        accs[hh] = d if accs[hh] is None else accs[hh] + d
                r8 = lax.broadcasted_iota(jnp.int32, (8, 128), 0) < 4
                blk = []
                for hp in range(2):
                    ea, ob_ = accs[2 * hp], accs[2 * hp + 1]
                    rz = 1.0 / jnp.where(r8, ob_[0:8], ea[16:24])
                    rs = pltpu.roll(rz, 4, 0)
                    ra, rb_ = jnp.where(r8, rs, rz), jnp.where(r8, rz, rs)
                    blk += [ea[0:8] * ra, ea[8:16] * ra, jnp.where(r8, ea[16:24], ob_[0:8]) * rs,
                            ob_[8:16] * rb_, ob_[16:24] * rb_]
                ot_ref[slot * NQB + qb, 80 * g:80 * g + 80, :] = jnp.concatenate(blk, axis=0)
                st["PV", n] = jnp.concatenate(blk[8:10], axis=0)

            def FIN(qb):
                for l in range(LT):
                    z = ot_ref[slot * NQB + qb, l * 128:(l + 1) * 128, :].T
                    zu = _u32(z.astype(jnp.bfloat16))
                    hd = (l * 128 + l16) // DH
                    h0 = (hd & 1) == 0
                    h1 = (hd & 2) == 0
                    zc = [zu[16 * c:16 * c + 16] for c in range(4)]
                    tt = [jnp.where(h0, zc[j], zc[(j + 1) % 4]) for j in range(4)]
                    oj = [jnp.where(h1, tt[j], tt[(j + 2) % 4]) for j in range(4)]
                    oa_ref[slot, qb * 64:(qb + 1) * 64, l * 128:(l + 1) * 128] = jnp.concatenate(oj, axis=0)
                    if want(t, "FIN%d" % qb):
                        fo = _fold(jnp.concatenate(oj, axis=0))
                        st["FIN%d" % qb] = fo if l == 0 else st["FIN%d" % qb] | fo

            def AP(qb):
                r0, r1, c0, c1 = (qb + (0, LT))[:4] if isinstance(qb, tuple) else (qb * 128, (qb + 1) * 128, 0, LT)
                qb = r0 // 128
                r = slice(r0, r1)
                cs = slice(c0 * 128, c1 * 128)
                a = jnp.dot(_bf16(dep_on(oa_ref[slot, r0 // 2:r1 // 2, :])), woa_ref[:, cs], preferred_element_type=jnp.float32)
                if isinstance(t, int):
                    dst = pl.ds(t * TB + r0, r1 - r0)
                else:
                    dst = pl.ds(pl.multiple_of(t * TB + r0, math.gcd(r0, 128)), r1 - r0)
                if "b_done" in st:
                    bb = jnp.concatenate([v[r] for v in st["bv_"]], axis=1)[:, cs] if "bv_" in st else bacc_ref[slot, r, cs]
                    gg = jnp.concatenate([st["gate"][r]] * (c1 - c0), axis=1) if gbc else st["gate"][r]
                    a = (gg * a + bb).astype(o_ref.dtype)
                    o_ref[dst, cs] = a
                else:
                    st["a_done"] = True
                    a = st["gate"][r] * a
                    bacc_ref[slot, r, :] = a
                if want(t, "AP%d" % qb):
                    st["AP%d" % qb] = _fold(a)

            def OS(qbs):
                for qb in (qbs or (0, 1)) if isinstance(t, int) or not noos else ():
                    qb = qb if isinstance(qb, tuple) else (qb, 1)
                    ocopy(t, *qb).start(priority=opr)
                    pend.extend([(t,) + qb] if isinstance(t, int) else [(tt,) + qb for tt in range(2, nrun)][::2 if pair else 1])

            def OSL(qb):
                @pl.when(t == nrun - 1)
                def _():
                    ocopy(nrun - 1, *qb).start()
                pend.append((nrun - 1,) + qb)

            def SPIN(n):
                acc = lax.fori_loop(0, n, lambda i, a: a * 1.0001 + 1.0, jnp.zeros((8, 128), jnp.float32))
                sc_ref[0, 0, 0:8, 0:128] = acc

            fns = dict(NXT=NXT, PREPN=PREPN, PBN=PBN, PKp=lambda a: PK(a, True), PBXp=lambda a: PBX(a, True), PBX=PBX, PREP=PREP, WW=WW, WS=WS, XW=XW, XS=XS, PB=PB, PK=PK, QT=QT, VT=VT, BV=BV, GATE=GATE, BP=BP,
                       QK=QK, PV=PV, FIN=FIN, AP=AP, OS=OS, OSL=OSL, SPIN=SPIN)
            return fns

        z_ref[1] = jnp.zeros((8, 128), jnp.int32)
        fs = [tile_fns(tt, tt % 2) for tt in range(NT)]
        for it in order0[nlead:]:
            cur["deps"] = it[3] if len(it) > 3 else ()
            fs[it[2] if len(it) > 2 else 0][it[0]](it[1])
        cur["deps"] = ()

        def loop_body(t, c):
            fns = tile_fns(t)
            for it in order1:
                cur["deps"] = it[3] if len(it) > 3 else ()
                fns[it[0]](it[1])
            cur["deps"] = ()
            return c
        def pair_body(i, c):
            for sl in range(2):
                fns = tile_fns(2 * i + sl, sl)
                for it in order1:
                    cur["deps"] = it[3] if len(it) > 3 else ()
                    fns[it[0]](it[1])
                cur["deps"] = ()
            return c
        t1 = 2 if joint else 1
        if pair:
            lax.fori_loop(1, nrun // 2, pair_body, 0)
        elif nrun > t1:
            lax.fori_loop(t1, nrun, loop_body, 0)
        if ofin:
            fs[nrun - 1]["OS"](((1, 1, ofin[-1], LT),))
        elif oshift:
            fs[nrun - 1]["OS"]((1,) if oshift is True else ((oshift / 128, 2 - oshift / 128),))
        for args in pend:
            ocopy(*args).wait()

    return kernel


ORDER0 = [('WS', (1, 0, 1)), ('WS', (30, 0, 4, 0, 1)), ('WS', (30, 4, 14, 0, 1)), ('WS', (1, 1, 2)), ('WS', (30, 14, 16, 0, 1)), ('WS', (30, 0, 16, 1, 2)),
 ('WS', (1, 2, 4)), ('WS', (30, 0, 4, 2, 5)), ('WS', 3), ('WS', 8), ('WS', (1, 4, 5)), ('WS', 4), ('WS', (30, 4, 8, 2, 5)), ('WS', 5), ('WS', 2),
 ('WS', 6), ('WS', 0), ('WS', 7), ('WS', (30, 8, 16, 2, 5)), ('WS', 20), ('WW', (1, 0, 1)), ('WW', (30, 0, 4, 0, 1)), ('PK', (0, 128, 0, 1), 0),
 ('PK', (128, 256, 0, 1), 0), ('PK', (256, 384, 0, 1), 0), ('PK', (384, 512, 0, 1), 0), ('WW', (30, 4, 14, 0, 1)), ('PK', (512, 672, 0, 1), 0),
 ('PK', (672, 832, 0, 1), 0), ('PK', (832, 992, 0, 1), 0), ('PK', (992, 1152, 0, 1), 0), ('PK', (1152, 1312, 0, 1), 0), ('PK', (1312, 1472, 0, 1), 0),
 ('PK', (1472, 1632, 0, 1), 0), ('PK', (1632, 1792, 0, 1), 0), ('WW', (1, 1, 2)), ('WW', (30, 14, 16, 0, 1)), ('WW', (30, 0, 16, 1, 2)),
 ('PK', (0, 224, 1, 2), 0), ('PK', (224, 448, 1, 2), 0), ('PK', (448, 672, 1, 2), 0), ('PK', (672, 896, 1, 2), 0), ('PK', (896, 1120, 1, 2), 0),
 ('PK', (1120, 1344, 1, 2), 0), ('PK', (1344, 1568, 1, 2), 0), ('PK', (1568, 1792, 1, 2), 0), ('PK', (1792, 1920, 0, 2), 0),
 ('PK', (1920, 2048, 0, 2), 0), ('WW', (1, 2, 4)), ('WW', (30, 0, 4, 2, 5)), ('WW', 3), ('WW', 8), ('WW', 20), ('PREP', 3), ('PK', (0, 128, 2, 4), 0),
 ('PK', (128, 256, 2, 4), 0), ('PK', (256, 384, 2, 4), 0), ('PK', (384, 512, 2, 4), 0), ('GATE', 32), ('GATE', 32, 1), ('PB', (0, 1)),
 ('PBX', (0, 3, 0, 256, 2, 0), 1, [(0, 'GATE'), (1, 'GATE')]), ('PBX', (3, 5, 0, 128), 1), ('PBX', (3, 5, 128, 256), 1), ('WW', (1, 4, 5)), ('WW', 4),
 ('WW', (30, 4, 8, 2, 5)), ('WW', 5), ('PREP', 4), ('PK', (0, 128, 4, 5), 0), ('PK', (128, 256, 4, 5), 0), ('PK', (256, 384, 4, 5), 0),
 ('PK', (384, 512, 4, 5), 0), ('PK', (512, 640, 2, 5), 0), ('PK', (640, 768, 2, 5), 0), ('PK', (768, 896, 2, 5), 0), ('PK', (896, 1024, 2, 5), 0),
 ('PREP', 5), ('PB', (1, 2)), ('PB', (2, 3), 0, []), ('PB', (1, 2), 1), ('PREPN', 0), ('PBX', (10, 12, 0, 256), 1), ('PBX', (12, 13, 0, 128), 1),
 ('PBX', (12, 13, 128, 256), 1), ('WW', 2), ('WW', 6), ('WW', 0), ('WW', 7), ('WW', (30, 8, 16, 2, 5)), ('PREP', 2), ('BV', (0, 16)),
 ('PK', (1024, 1152, 2, 5), 0), ('PK', (1152, 1280, 2, 5), 0), ('PBX', (13, 15, 0, 256), 1), ('PREP', 0), ('VT', 0), ('PREP', 6), ('QT', 0),
 ('VT', 0, 1, []), ('QK', 0), ('QK', 1), ('QK', 2, 0, [(0, 'bvl')]), ('QK', 3), ('QK', 4), ('PV', 0), ('QK', 5), ('PV', 1), ('QK', 6),
 ('PK', (1280, 1408, 2, 5), 0), ('PV', 2), ('QK', 7), ('PV', 3), ('QK', 8), ('PK', (1408, 1536, 2, 5), 0), ('PV', 4), ('QK', 9), ('PV', 5),
 ('QK', 10), ('PK', (1536, 1664, 2, 5), 0), ('PV', 6), ('QK', 11), ('PV', 7), ('FIN', 0), ('QK', 12), ('PK', (1664, 1792, 2, 5), 0), ('PV', 8),
 ('QK', 13), ('PK', (1792, 1920, 2, 5), 0), ('PV', 9), ('QK', 14), ('PK', (1920, 2048, 2, 5), 0), ('PV', 10), ('QK', 15), ('PV', 11), ('PV', 12),
 ('QT', 0, 1), ('PV', 13), ('PV', 14), ('PV', 15), ('FIN', 1), ('BV', (0, 16), 1, [(0, ('PV', 10))]), ('BP', 0), ('AP', 0), ('AP', 1),
 ('OS', ((0, 2),)), ('QK', 0, 1), ('QK', 1, 1), ('QK', 2, 1, [(1, 'bvl')]), ('PV', 0, 1), ('QK', 3, 1), ('PV', 1, 1), ('QK', 4, 1), ('PV', 2, 1),
 ('QK', 5, 1), ('PV', 3, 1), ('QK', 6, 1), ('PV', 4, 1), ('QK', 7, 1, [(0, 'AP0'), (0, 'AP1')]), ('PV', 5, 1), ('QK', 8, 1), ('PV', 6, 1),
 ('QK', 9, 1), ('PV', 7, 1), ('FIN', 0, 1), ('QK', 10, 1), ('PV', 8, 1), ('QK', 11, 1), ('PV', 9, 1), ('QK', 12, 1), ('PV', 10, 1), ('QK', 13, 1),
 ('PV', 11, 1), ('QK', 14, 1), ('PV', 12, 1), ('QK', 15, 1), ('PV', 13, 1), ('BP', (0, 4), 1), ('PV', 14, 1), ('BP', (4, 5), 1), ('PV', 15, 1),
 ('FIN', 1, 1), ('AP', 0, 1), ('OS', (0,), 1), ('AP', 1, 1), ('OS', ((1, 1, 0, 4),), 1)]

ORDER1 = [('PBN', (0, 128)), ('PBX', (1, 15, 0, 128)), ('PBX', (0, 15, 128, 256)), ('GATE', 0), ('QT', 0), ('VT', 0), ('BV', (0, 16)), ('QK', 0), ('QK', 1),
 ('QK', 2), ('PV', 0), ('QK', 3), ('PV', 1), ('QK', 4), ('PV', 2), ('QK', 5), ('PV', 3), ('QK', 6), ('PV', 4), ('QK', 7), ('PV', 5), ('QK', 8),
 ('PV', 6), ('QK', 9), ('PV', 7), ('FIN', 0), ('QK', 10), ('PV', 8), ('QK', 11), ('PV', 9), ('QK', 12), ('PV', 10), ('QK', 13), ('PV', 11),
 ('QK', 14), ('PV', 12), ('QK', 15), ('PV', 13), ('BP', (0, 4)), ('PV', 14), ('BP', (4, 5)), ('PV', 15), ('FIN', 1), ('AP', 0),
 ('OS', ((-1, 2, 4, 5), (0, 1, 0, 4))), ('AP', (128, 256, 0, 1)), ('OS', ((1, 1, 0, 1),)), ('AP', (128, 256, 1, 2)), ('OS', ((1, 1, 1, 2),)),
 ('AP', (128, 256, 2, 4)), ('OS', ((1, 1, 2, 4),)), ('AP', (128, 256, 4, 5))]

KNOBS = {'nrun': 8,
 'pace': 1,
 'bchain': 1,
 'bforce': 2,
 'bchain0': 1,
 'pace1': 1,
 'wvf': True,
 'bpace': {14: (-16, 1), 15: (64, 2)},
 'bvo0': (8, 12),
 'bsync0': (2, 2),
 'ao1': 5,
 'pace0': 3,
 'pchain': (3, 4, 5, 6),
 'oshift': True,
 'bval': 1,
 'gbc': 2,
 'ao': 1,
 'bsync': 2,
 'ofin': (1, 2, 4),
 'bvo': 9,
 'semmap': {(1, 0, 1): ('G', 0),
            (30, 0, 4, 0, 1): ('G', 0),
            (30, 4, 14, 0, 1): ('G', 1),
            (1, 1, 2): ('G', 2),
            (30, 14, 16, 0, 1): ('G', 2),
            (30, 0, 16, 1, 2): ('G', 2),
            (1, 2, 4): ('G', 3),
            (30, 0, 4, 2, 5): ('G', 3),
            3: ('G', 3),
            8: ('G', 3),
            20: ('G', 3),
            (1, 4, 5): ('G', 4),
            4: ('G', 4),
            (30, 4, 8, 2, 5): ('G', 4),
            5: ('G', 4),
            2: ('G', 5),
            6: ('G', 5),
            0: ('G', 5),
            7: ('G', 5),
            (30, 8, 16, 2, 5): ('G', 5)}}


def build():
    kernel = make_kernel(ORDER0, ORDER1, **KNOBS)
    anyspec = pl.BlockSpec(memory_space=pl.ANY)

    @jax.jit
    def f(A_x, A_wqkv, A_wo, B_x, B_wqkv, B_wo, gate_w):
        x = A_x.reshape(S, D)
        out = pl.pallas_call(
            kernel,
            in_specs=[anyspec] * 6,
            out_specs=anyspec,
            out_shape=jax.ShapeDtypeStruct((S, D), jnp.bfloat16),
            scratch_shapes=[
                pltpu.VMEM((S, D), jnp.bfloat16),
                pltpu.VMEM((D, 3 * D), jnp.bfloat16),
                pltpu.VMEM((D, D), jnp.bfloat16),
                pltpu.VMEM((D, 3 * D), jnp.bfloat16),
                pltpu.VMEM((D, D), jnp.bfloat16),
                pltpu.VMEM((D,), jnp.bfloat16),
                pltpu.VMEM((S, D), jnp.bfloat16),
                pltpu.VMEM((D // 2, D), jnp.uint32),
                pltpu.VMEM((D // 2, D), jnp.uint32),
                pltpu.VMEM((3 * D // 2, D), jnp.uint32),
                pltpu.VMEM((D // 2, D), jnp.uint32),
                pltpu.VMEM((NG, S // 2, 128), jnp.uint32),
                pltpu.VMEM((S // 128, H * 24, 128), jnp.float32),
                pltpu.VMEM((2 * NQB, D // 2, 128), jnp.uint32),
                pltpu.VMEM((3 * LT, HALO + 2 * TB, 128), jnp.float32),
                pltpu.VMEM((2 * NQB, D, 128), jnp.float32),
                pltpu.VMEM((2, TB // 2, D), jnp.uint32),
                pltpu.VMEM((2, TB // 2, D), jnp.uint32),
                pltpu.VMEM((5, LT, D, 128), jnp.float32),
                pltpu.VMEM((LT, D // 2, 128), jnp.uint32),
                pltpu.VMEM((1, 8, 128), jnp.float32),
                pltpu.VMEM((2, 8, 128), jnp.int32),
                pltpu.VMEM((1, 1, 8, 128), jnp.float32),
                pltpu.VMEM((1, 1, 8, 128), jnp.uint32),
                pltpu.VMEM((S, D), jnp.float32),
                pltpu.VMEM((1, 8, 128), jnp.float32),
                pltpu.VMEM((D // 2, 3 * D), jnp.uint32),
                pltpu.VMEM((TB // 2, D), jnp.uint32),
                pltpu.VMEM((TB, 128), jnp.float32),
                pltpu.SemaphoreType.DMA((7,)),
            ],
            compiler_params=pltpu.CompilerParams(
                vmem_limit_bytes=100 * 1024 * 1024,
                disable_semaphore_checks=True,
                disable_bounds_checks=True,
            ),
        )(x, A_wqkv, A_wo, B_wqkv, B_wo, gate_w)
        return out.reshape(1, S, D)
    return f


_impl = build()


@jax.jit
def pallas_gated_mix__sliding_block__sliding_local_dilated__prompt_kernel(
    A_x: jax.Array,
    A_wqkv: jax.Array,
    A_wo: jax.Array,
    B_x: jax.Array,
    B_wqkv: jax.Array,
    B_wo: jax.Array,
    gate_w: jax.Array,
):
    return _impl(A_x, A_wqkv, A_wo, B_x, B_wqkv, B_wo, gate_w)
```
